```python
import os as _os
_os.environ.setdefault("JAX_PLATFORMS", "cpu")
import jax
import jax.numpy as jnp

def _softmax(x, axis=-1):
    return jax.nn.softmax(x, axis=axis)
def _gelu(x):
    return jax.nn.gelu(x, approximate=True)
def _silu(x):
    return jax.nn.silu(x)
def _sigmoid(x):
    return jax.nn.sigmoid(x)
def _layernorm(x, axis=-1, eps=1e-5):
    m = jnp.mean(x, axis=axis, keepdims=True)
    v = jnp.var(x, axis=axis, keepdims=True)
    return (x - m) / jnp.sqrt(v + eps)
def _scatter_add(tgt, idx, src, axis=0):
    return tgt.at[idx].add(src)
def _segment_sum(src, seg, n):
    return jax.ops.segment_sum(src, seg, n)
class _Rng:
    def __init__(self, key):
        self._k = key
    def _next(self):
        self._k, sub = jax.random.split(self._k)
        return sub
    def normal(self, shape):
        return jax.random.normal(self._next(), shape, dtype=jnp.bfloat16)
    def randint(self, lo, hi, shape):
        return jax.random.randint(self._next(), shape, lo, hi, dtype=jnp.int32)
    def uniform(self, shape, lo=0.0, hi=1.0):
        return jax.random.uniform(self._next(), shape, jnp.bfloat16, lo, hi)
    def permutation(self, n):
        return jax.random.permutation(self._next(), n)


kernel_name = 'gated_mix__compressed_kv_cla__ssm_conv_h3__prompt'

def setup_inputs():
    _rng = _Rng(jax.random.key(int.from_bytes(__import__("os").urandom(4), "little")))
    _w = (lambda a: (lambda t: t.astype(jnp.bfloat16) if jnp.issubdtype(t.dtype, jnp.floating) else t)(jnp.asarray(a)))
    def _A_setup():
        B, H, Sq, Sk, D, M = 1, 32, 2048, 2048, 128, 1024
        Dc = 4 * D
        return {
            "x": _w((lambda *s: _rng.normal(s) * 0.05)(B, Sq, M)),
            "c_kv": _w((lambda *s: _rng.normal(s) * 0.8)(B, Sk, Dc)),
            "w_q": _w((lambda *s: _rng.normal(s) * 3.2)(M, H, D) * (M ** -0.5)),
            "w_uk": _w((lambda *s: _rng.normal(s) * 3.2)(Dc, H, D) * (Dc ** -0.5)),
            "w_uv": _w((lambda *s: _rng.normal(s) * 0.8)(Dc, H, D) * (Dc ** -0.5)),
            "w_o": _w((lambda *s: _rng.normal(s) * 0.8)(H, D, M) * ((H * D) ** -0.5)),
        }
    _A_in = _A_setup()

    def _B_setup():
        B, S, D = 1, 2048, 1024
        ks = 4
        return {
            "q": _w((lambda *s: _rng.normal(s) * 0.05)(B, S, D)),
            "k": _w((lambda *s: _rng.normal(s) * 0.8)(B, S, D)),
            "v": _w((lambda *s: _rng.normal(s) * 0.8)(B, S, D)),
            "shift_k": _w((lambda *s: _rng.normal(s) * 0.8)(D, ks) * 0.5),
            "ssm_k": _w((lambda *s: _rng.normal(s) * 0.8)(D, S) * (1.0 / S ** 0.5)),
            "ssm_D": _w((lambda *s: _rng.normal(s) * 0.8)(D)),
        }
    _B_in = _B_setup()

    return {
        "A_x": _A_in["x"],
        "A_c_kv": _A_in["c_kv"],
        "A_w_q": _A_in["w_q"],
        "A_w_uk": _A_in["w_uk"],
        "A_w_uv": _A_in["w_uv"],
        "A_w_o": _A_in["w_o"],
        "B_q": _B_in["q"],
        "B_k": _B_in["k"],
        "B_v": _B_in["v"],
        "B_shift_k": _B_in["shift_k"],
        "B_ssm_k": _B_in["ssm_k"],
        "B_ssm_D": _B_in["ssm_D"],
        "gate_w": _w((lambda *s: _rng.normal(s) * 0.05)(1024) * 16.0),
    }

def reference(A_x, A_c_kv, A_w_q, A_w_uk, A_w_uv, A_w_o, B_q, B_k, B_v, B_shift_k, B_ssm_k, B_ssm_D, gate_w):
    def _A_ref(x, c_kv, w_q, w_uk, w_uv, w_o):
        B, Sq, M = x.shape[0], x.shape[1], x.shape[2]
        Sk = c_kv.shape[1]
        H, D = w_q.shape[1], w_q.shape[2]
        q = jnp.einsum("bqm,mhd->bhqd", x, w_q)
        k = jnp.einsum("bkc,chd->bhkd", c_kv, w_uk)
        v = jnp.einsum("bkc,chd->bhkd", c_kv, w_uv)
        scores = jnp.einsum("bhqd,bhkd->bhqk", q, k) * (D ** -0.5)
        off = Sk - Sq
        qi = jnp.arange(Sq)[:, None]
        kj = jnp.arange(Sk)[None, :]
        cmask = kj <= (qi + off)
        scores = jnp.where(cmask[None, None], scores, -1e9)
        p = _softmax(scores, axis=-1)
        ctx = jnp.einsum("bhqk,bhkd->bhqd", p, v)
        return jnp.einsum("bhqd,hdm->bqm", ctx, w_o)

    def _B_ref(q, k, v, shift_k, ssm_k, ssm_D):
        B, S, D = q.shape
        ks = shift_k.shape[-1]
        k_pad = jnp.pad(k, ((0, 0), (ks - 1, 0), (0, 0)))
        k_shift = jnp.zeros_like(k)
        for t in range(ks):
            k_shift = k_shift + k_pad[:, t:t + S, :] * shift_k[:, ks - 1 - t][None, None, :]
        kv = k_shift * v
        L = 2 * S
        kv_pad = jnp.pad(kv, ((0, 0), (0, S), (0, 0)))
        kf_pad = jnp.pad(ssm_k, ((0, 0), (0, S)))
        kv_f = (lambda x, axes=(-2,-1): jnp.fft.rfft2(x.astype(jnp.float32), axes=axes))(kv_pad[:, None, :, :], axes=(1, 2))
        kf_f = (lambda x, axes=(-2,-1): jnp.fft.rfft2(x.astype(jnp.float32), axes=axes))(kf_pad[:, None, :], axes=(1, 2))
        kf_f = (lambda x, *d: x.transpose(*d))(kf_f, 1, 2, 0)
        y_f = kv_f * kf_f[None, :, :, :]
        y = (lambda x, s, axes=(-2,-1): jnp.fft.irfft2(x, s=s, axes=axes).astype(jnp.bfloat16))(y_f, (1, L), axes=(1, 2))[:, 0, :S, :]
        y = y + kv * ssm_D[None, None, :]
        return q * y

    x = A_x
    g = _sigmoid((x * gate_w).sum(-1, keepdims=True))
    a = _A_ref(x, A_c_kv, A_w_q, A_w_uk, A_w_uv, A_w_o)
    b = _B_ref(x, B_k, B_v, B_shift_k, B_ssm_k, B_ssm_D)
    return g * a + (1 - g) * b
```

```python
import collections
import functools
import numpy as np
import jax
import jax.numpy as jnp
import jax.experimental.pallas as pl
import jax.experimental.pallas.tpu as pltpu

f32, bf16 = jnp.float32, jnp.bfloat16
NT = (((1,), (1,)), ((), ()))

S = 2048
M = 1024
DC = 512
H = 32
D = 128
HP = 2
NSTEP = H // HP
BQ = 256
NB = S // BQ
NU = 2 * NB
C = 128
NCH = S // C
HB = 8
SPB = HB // HP
LOG2E = 1.4426950408889634

CFG = {}
KC = CFG.get("kc", 4)
RATE = CFG.get("rate", 2.0)


def _dft_consts():
    n = np.arange(C)
    Fs, Gs = [], []
    for p in range(2):
        ks = np.arange(p * 64, (p + 1) * 64)
        ks = np.concatenate([ks[ks % 2 == 0], ks[ks % 2 == 1]])
        th = np.pi * (2 * ks[:, None] + 1) * n[None, :] / (2 * C)
        F = np.concatenate([np.cos(th), -np.sin(th)], axis=0)
        G = np.concatenate([np.cos(th), -np.sin(th)], axis=0).T / C
        Fs.append(F); Gs.append(G)
    return np.stack(Fs).astype(np.float32), np.stack(Gs).astype(np.float32)


def _kernel(x_ref, c_ref, wq0_ref, wk0_ref, wv0_ref, wqn_ref, wkn_ref, wvn_ref, wo_ref,
            xt_ref, kt_ref, vt_ref, ht_ref, par_ref, gw_ref, f_ref, g_ref,
            o_ref,
            acc_ref, q_s, k_s, v_s, wq_st, wk_st, wv_st, wq_b, wk_b, wv_b, gate_s, kpad_s, u_s, ub_s, W_s, ctx_s):
    step = pl.program_id(0)
    ct = step // 2
    P = functools.partial

    @pl.when(step == 0)
    def _():
        acc_ref[...] = jnp.zeros_like(acc_ref)
        wq_st[0] = wq0_ref[...].astype(f32).reshape(M * HB, D)
        wk_st[0] = wk0_ref[...].astype(f32).reshape(DC * HB, D)
        wv_st[0] = wv0_ref[...].astype(f32).reshape(DC * HB, D)
        for st_, wb, rows in ((wq_st, wq_b, M), (wk_st, wk_b, DC), (wv_st, wv_b, DC)):
            wb[...] = jnp.concatenate([st_[0, pl.ds(hh, rows, stride=HB), :] for hh in range(HP)], axis=1).astype(bf16)
        gw = gw_ref[...].astype(f32)
        for i in range(NB):
            xs = x_ref[i * BQ:(i + 1) * BQ, :].astype(f32) * gw
            z = jnp.sum(xs, axis=1, keepdims=True)
            gate_s[i * BQ:(i + 1) * BQ, :] = jnp.broadcast_to(jax.nn.sigmoid(z), (BQ, D))
        kpad_s[0:8, :] = jnp.zeros((8, D), f32)

    scale = (D ** -0.5) * LOG2E
    row = jax.lax.broadcasted_iota(jnp.int32, (128, 128), 0)
    col = jax.lax.broadcasted_iota(jnp.int32, (128, 128), 1)
    mask = col <= row
    par = par_ref[...].astype(f32)
    never8 = jnp.broadcast_to(par[7:8, :], (8, 128)) != 0.0
    never = jnp.broadcast_to(par[7:8, :], (128, 128)) != 0.0

    side = collections.deque()
    budget = [0.0]

    def pin(arr, spacing):
        R = arr.shape[0]
        out, last = [], 0
        for g in range(R // 8):
            budget[0] = min(budget[0] + RATE * spacing, 64.0)
            if side and budget[0] >= side[0][0]:
                cost, fn = side.popleft()
                budget[0] -= cost
                v = fn()
                if g * 8 > last:
                    out.append(arr[last:g * 8])
                out.append(jnp.where(never8, v, arr[g * 8:(g + 1) * 8]))
                last = (g + 1) * 8
        if last == 0:
            return arr
        if last < R:
            out.append(arr[last:])
        return jnp.concatenate(out, axis=0)

    def flush():
        while side:
            side.popleft()[1]()

    def pq(i, hh):
        r0 = i * BQ; r1 = r0 + BQ
        hs = slice(hh * D, (hh + 1) * D)
        r = jnp.dot(x_ref[r0:r1, :], wq_b[:, hs], preferred_element_type=f32)
        q_s[r0:r1, hs] = (pin(r, 8) * scale).astype(bf16)

    def pk(i, hh):
        r0 = i * BQ; r1 = r0 + BQ
        hs = slice(hh * D, (hh + 1) * D)
        r = jnp.dot(c_ref[r0:r1, :], wk_b[:, hs], preferred_element_type=f32)
        k_s[r0:r1, hs] = pin(r, 8).astype(bf16)

    def pvv(i, hh):
        r0 = i * BQ; r1 = r0 + BQ
        hs = slice(hh * D, (hh + 1) * D)
        r = jnp.dot(c_ref[r0:r1, :], wv_b[:, hs], preferred_element_type=f32)
        v_s[r0:r1, hs] = pin(r, 8).astype(bf16)

    def chunks(i):
        nt = 2 * i + 1
        out, t = [], 0
        while t < nt:
            n = min(KC, nt - t)
            out.append((0, t * 128, (t + n) * 128))
            t += n
        out.append((128, nt * 128, (nt + 1) * 128))
        return out

    st = {}

    def qk_atom(i, hh, ch):
        rl, kl, kh = ch
        r0 = i * BQ
        hs = slice(hh * D, (hh + 1) * D)
        s = jax.lax.dot_general(q_s[r0 + rl:r0 + BQ, hs], k_s[kl:kh, hs], NT, preferred_element_type=f32)
        nt = (kh - kl) // 128
        tiles = [s[:, t * 128:(t + 1) * 128] for t in range(nt)]
        if kh > r0 + rl:
            d = tiles[-1]
            dm = jnp.where(mask, d[:128], -1e30)
            tiles[-1] = dm if rl == 128 else jnp.concatenate([dm, d[128:]], axis=0)
        u = st.setdefault((i, hh), {"m": [None, None], "l": [None, None], "o": [None, None]})
        u[("s", ch)] = tiles
        mm = functools.reduce(jnp.maximum, tiles)
        for g in range(rl // 128, 2):
            a = mm[g * 128 - rl:(g + 1) * 128 - rl]
            u["m"][g] = a if u["m"][g] is None else jnp.maximum(u["m"][g], a)

    def maxfin(i, hh):
        u = st[(i, hh)]
        u["M"] = [jnp.broadcast_to(jnp.max(u["m"][g], axis=1, keepdims=True), (128, 128)) for g in range(2)]

    def pv_atom(i, hh, ch):
        rl, kl, kh = ch
        hs = slice(hh * D, (hh + 1) * D)
        u = st[(i, hh)]
        m = u["M"][1] if rl == 128 else jnp.concatenate(u["M"], axis=0)
        ps = [jnp.exp2(t - m) for t in u[("s", ch)]]
        lp = functools.reduce(jnp.add, ps)
        ls = []
        for g in range(rl // 128, 2):
            a = lp[g * 128 - rl:(g + 1) * 128 - rl]
            u["l"][g] = a if u["l"][g] is None else u["l"][g] + a
            ls.append(u["l"][g])
        ps[-1] = jnp.minimum(ps[-1], jnp.concatenate(ls, axis=0) if len(ls) > 1 else ls[0])
        pb = (jnp.concatenate(ps, axis=1) if len(ps) > 1 else ps[0]).astype(bf16)
        o = jnp.dot(pb, v_s[kl:kh, hs], preferred_element_type=f32)
        for g in range(rl // 128, 2):
            a = o[g * 128 - rl:(g + 1) * 128 - rl]
            u["o"][g] = a if u["o"][g] is None else u["o"][g] + a

    def norm(i, hh):
        u = st[(i, hh)]
        r0 = i * BQ
        hs = slice(hh * D, (hh + 1) * D)
        for g in range(2):
            l = jnp.where(never, u["o"][g], u["l"][g])
            r = gate_s[r0 + g * 128: r0 + (g + 1) * 128, :] / jnp.sum(l, axis=1, keepdims=True)
            ctx_s[g * 128:(g + 1) * 128, hs] = (u["o"][g] * r).astype(bf16)

    def oproj_atom(i, a):
        r0 = i * BQ; r1 = r0 + BQ
        r = jnp.dot(ctx_s[...], wo_ref[:, a * 256:(a + 1) * 256], preferred_element_type=f32)
        acc_ref[2 * a, r0:r1, :] += pin(r[:, :128], 8)
        acc_ref[2 * a + 1, r0:r1, :] += r[:, 128:]

    cv = {}

    def u_piece(r):
        j = r // C
        ks = kpad_s[8 + r:24 + r, :] * par[0:1]
        for t in range(1, 4):
            ks = ks + kpad_s[8 - t + r:24 - t + r, :] * par[t:t + 1]
        u = ks * vt_ref[r:r + 16, :].astype(f32)
        ub_s[r - j * C:r - j * C + 16, j * 128:(j + 1) * 128] = u.astype(bf16)
        u_s[r:r + 16, :] = u * (0.5 * par[4:5])
        return jnp.maximum(u[:8], u[8:])

    def fwdu(half):
        lo, hi = half * NCH // 2, (half + 1) * NCH // 2
        U = jnp.dot(f_ref[0], ub_s[:, lo * 128:hi * 128], preferred_element_type=f32)
        for j in range(lo, hi):
            ur = U[0:64, (j - lo) * 128:(j - lo + 1) * 128]
            ui = U[64:128, (j - lo) * 128:(j - lo + 1) * 128]
            cv[("ur", j)], cv[("ui", j)] = ur, ui
            if j == 0:
                vr, vi = ur, ui
            else:
                pr, pi = cv[("ur", j - 1)], cv[("ui", j - 1)]
                vr = jnp.concatenate([ur[:32] - pi[:32], ur[32:] + pi[32:]], axis=0)
                vi = jnp.concatenate([ui[:32] + pr[:32], ui[32:] - pr[32:]], axis=0)
            cv[("V", 0, j)], cv[("V", 1, j)], cv[("V", 2, j)] = vr, vi, vr + vi

    def fwdh(half):
        lo, hi = half * NCH // 2, (half + 1) * NCH // 2
        hcat = jnp.concatenate([ht_ref[:, j * C:(j + 1) * C] for j in range(lo, hi)], axis=0)
        Hf = jax.lax.dot_general(f_ref[0], hcat, NT, preferred_element_type=f32)
        for j in range(lo, hi):
            hr = Hf[0:64, (j - lo) * 128:(j - lo + 1) * 128]
            hi_ = Hf[64:128, (j - lo) * 128:(j - lo + 1) * 128]
            cv[("H", 0, j)], cv[("H", 1, j)], cv[("H", 2, j)] = hi_ - hr, hr + hi_, hr

    def mac_piece(i, r, a):
        rs = slice(r, r + 8)
        s = functools.reduce(jnp.add, [cv[("H", a, i - j)][rs] * cv[("V", a, j)][rs] for j in range(i + 1)])
        cv[("S", a, i, r)] = s
        if a == 2:
            W_s[r:r + 8, i * 128:(i + 1) * 128] = s - cv[("S", 1, i, r)]
            W_s[64 + r:64 + r + 8, i * 128:(i + 1) * 128] = s + cv[("S", 0, i, r)]
        return s

    def inv(half):
        lo, hi = half * NCH // 2, (half + 1) * NCH // 2
        Y = jnp.dot(g_ref[0], W_s[:, lo * 128:hi * 128].astype(bf16), preferred_element_type=f32)
        for j in range(lo, hi):
            a, b = j * C, (j + 1) * C
            y = Y[:, (j - lo) * 128:(j - lo + 1) * 128]
            bb = xt_ref[a:b, :].astype(f32) * (y + u_s[a:b, :])
            acc_ref[ct, a:b, :] += (1.0 - gate_s[a:b, :]) * bb

    nslot = (step // SPB + 1) % 2
    qtr = step % SPB
    nstep = step + 1
    eslot = (nstep // SPB) % 2
    ehead = (nstep % SPB) * HP

    def stage_piece(src, st_, rows, m0):
        n = rows // SPB * HB
        w = src[m0:m0 + 4].astype(f32).reshape(4 * HB, D)
        st_[nslot, pl.ds(pl.multiple_of(qtr * n + m0 * HB, 8), 4 * HB), :] = w
        return functools.reduce(jnp.maximum, [w[k * 8:(k + 1) * 8] for k in range(4)])

    def extract_piece(st_, wb, m0):
        ws = [st_[eslot, pl.ds(ehead + hh + m0 * HB, 8, stride=HB), :] for hh in range(HP)]
        wb[m0:m0 + 8, :] = jnp.concatenate(ws, axis=1).astype(bf16)
        return ws[0]

    wsets = ((wqn_ref, wq_st, wq_b, M), (wkn_ref, wk_st, wk_b, DC), (wvn_ref, wv_st, wv_b, DC))
    units = [(u // 2, u % 2) for u in range(NU)]

    kpad_s[8:8 + S, :] = kt_ref[...].astype(f32)
    for r in range(0, S, 16):
        side.append((28, P(u_piece, r)))
    pq(0, 0); pk(0, 0); pq(0, 1); pk(0, 1)
    for ch in chunks(0): qk_atom(0, 0, ch)
    maxfin(0, 0)
    pvv(0, 0); pvv(0, 1)
    fwdh(0); fwdh(1)
    FW = CFG.get("fw", 2)
    for s in range(NU):
        i, hh = units[s]
        if s == FW:
            flush()
            fwdu(0); fwdu(1)
            order = sorted(range(NCH), key=lambda k: (k % 2, k) if CFG.get("macsort", 0) else k)
            for ii in range(NCH // 2):
                for i2 in (ii, NCH - 1 - ii):
                    for r in range(0, 64, 8):
                        for a in range(3):
                            side.append((2 * (i2 + 1) + 2, P(mac_piece, i2, r, a)))
            for src, st_, wb, rows in wsets:
                for m0 in range(0, rows // SPB, 4):
                    side.append((12, P(stage_piece, src, st_, rows, m0)))
        if s == NU - 2:
            flush()
            for src, st_, wb, rows in wsets:
                for m0 in range(0, rows, 8):
                    side.append((8, P(extract_piece, st_, wb, m0)))
        if s >= 2 and hh == 0:
            for a in range(4): oproj_atom(i - 1, a)
        if i + 1 < NB:
            pq(i + 1, hh); pk(i + 1, hh); pvv(i + 1, hh)
        if s == NU - 1:
            inv(0)
        for ch in chunks(i): pv_atom(i, hh, ch)
        norm(i, hh)
        if s + 1 < NU:
            i1, h1 = units[s + 1]
            for ch in chunks(i1): qk_atom(i1, h1, ch)
            maxfin(i1, h1)
    inv(1)
    for a in range(4): oproj_atom(NB - 1, a)
    flush()

    @pl.when(step == NSTEP - 1)
    def _():
        for j in range(M // 256):
            o_ref[:, j * 256:(j + 1) * 256] = jnp.concatenate([acc_ref[2 * j], acc_ref[2 * j + 1]], axis=1).astype(o_ref.dtype)


@jax.jit
def pallas_gated_mix__compressed_kv_cla__ssm_conv_h3__prompt_kernel(A_x, A_c_kv, A_w_q, A_w_uk, A_w_uv, A_w_o, B_q, B_k, B_v, B_shift_k, B_ssm_k, B_ssm_D, gate_w):
    x = A_x.reshape(S, M)
    c = A_c_kv.reshape(S, DC)
    wo = A_w_o.reshape(H * D, M)
    k = B_k.reshape(S, M)
    v = B_v.reshape(S, M)
    par = jnp.concatenate([B_shift_k.T, B_ssm_D[None, :], jnp.zeros((3, M), bf16)], axis=0)
    gw = gate_w.reshape(1, M)
    Fc, Gc = _dft_consts()
    Fc = jnp.asarray(Fc, bf16); Gc = jnp.asarray(Gc, bf16)
    nblk = H // HB
    nxt = lambda s: (s % SPB, jnp.minimum(s // SPB + 1, nblk - 1), 0)
    in_specs = [
        pl.BlockSpec((S, M), lambda s: (0, 0)),
        pl.BlockSpec((S, DC), lambda s: (0, 0)),
        pl.BlockSpec((M, HB, D), lambda s: (0, 0, 0)),
        pl.BlockSpec((DC, HB, D), lambda s: (0, 0, 0)),
        pl.BlockSpec((DC, HB, D), lambda s: (0, 0, 0)),
        pl.BlockSpec((M // SPB, HB, D), nxt),
        pl.BlockSpec((DC // SPB, HB, D), nxt),
        pl.BlockSpec((DC // SPB, HB, D), nxt),
        pl.BlockSpec((HP * D, M), lambda s: (s, 0)),
        pl.BlockSpec((S, 128), lambda s: (0, s // 2)),
        pl.BlockSpec((S, 128), lambda s: (0, s // 2)),
        pl.BlockSpec((S, 128), lambda s: (0, s // 2)),
        pl.BlockSpec((128, S), lambda s: (s // 2, 0)),
        pl.BlockSpec((8, 128), lambda s: (0, s // 2)),
        pl.BlockSpec((1, M), lambda s: (0, 0)),
        pl.BlockSpec((1, 128, C), lambda s: (s % 2, 0, 0)),
        pl.BlockSpec((1, C, 128), lambda s: (s % 2, 0, 0)),
    ]
    scratch = [
        pltpu.VMEM((M // 128, S, 128), f32),
        pltpu.VMEM((S, HP * D), bf16),
        pltpu.VMEM((S, HP * D), bf16),
        pltpu.VMEM((S, HP * D), bf16),
        pltpu.VMEM((2, M * HB, D), f32),
        pltpu.VMEM((2, DC * HB, D), f32),
        pltpu.VMEM((2, DC * HB, D), f32),
        pltpu.VMEM((M, HP * D), bf16),
        pltpu.VMEM((DC, HP * D), bf16),
        pltpu.VMEM((DC, HP * D), bf16),
        pltpu.VMEM((S, 128), f32),
        pltpu.VMEM((S + 8, 128), f32),
        pltpu.VMEM((S, 128), f32),
        pltpu.VMEM((C, NCH * 128), bf16),
        pltpu.VMEM((128, NCH * 128), f32),
        pltpu.VMEM((BQ, HP * D), bf16),
    ]
    out = pl.pallas_call(
        _kernel,
        out_shape=jax.ShapeDtypeStruct((S, M), bf16),
        grid=(NSTEP,),
        in_specs=in_specs,
        out_specs=pl.BlockSpec((S, M), lambda s: (0, 0)),
        scratch_shapes=scratch,
        compiler_params=pltpu.CompilerParams(vmem_limit_bytes=110 * 1024 * 1024, dimension_semantics=("arbitrary",)),
    )(x, c, A_w_q, A_w_uk, A_w_uv, A_w_q, A_w_uk, A_w_uv, wo, x, k, v, B_ssm_k, par, gw, Fc, Gc)
    return out.reshape(1, S, M)
```

```python
import collections
import functools
import numpy as np
import jax
import jax.numpy as jnp
import jax.experimental.pallas as pl
import jax.experimental.pallas.tpu as pltpu

f32, bf16 = jnp.float32, jnp.bfloat16
NT = (((1,), (1,)), ((), ()))

S = 2048
M = 1024
DC = 512
H = 32
D = 128
HP = 2
NSTEP = H // HP
BQ = 256
NB = S // BQ
NU = 2 * NB
C = 128
NCH = S // C
HB = 8
SPB = HB // HP
NBLK = H // HB
GR = S // NSTEP
LOG2E = 1.4426950408889634

CFG = {}
KC = CFG.get("kc", 4)
RATE = CFG.get("rate", 2.0)
MACW = CFG.get("macw", 2.25)
FW = CFG.get("fw", 4)
NP0 = FW // 2 + 1

SEM_WQ, SEM_WK, SEM_WV, SEM_WO, SEM_KT, SEM_VT, SEM_HT = range(7)
SEM_W0 = 7
SEM_C = 10
SEM_X = 12
SEM_OUT = 14
SEM_SM = 15
NSEM = 20


def _dft_consts():
    n = np.arange(C)
    Fs, Gs = [], []
    for p in range(2):
        ks = np.arange(p * 64, (p + 1) * 64)
        ks = np.concatenate([ks[ks % 2 == 0], ks[ks % 2 == 1]])
        th = np.pi * (2 * ks[:, None] + 1) * n[None, :] / (2 * C)
        F = np.stack([np.cos(th).reshape(8, 8, C), -np.sin(th).reshape(8, 8, C)], axis=1).reshape(128, C)
        Fs.append(F); Gs.append(F.T / C)
    return np.stack(Fs).astype(np.float32), np.stack(Gs).astype(np.float32)


def _kernel(x_h, c_h, wq_h, wk_h, wv_h, wo_h, k_h, v_h, h_h,
            skt_h, dd_h, gw_h, f_h, g_h,
            o_h,
            skt_ref, dd_ref, gw_ref, f_ref, g_ref,
            x_v, c_v, wq_l, wk_l, wv_l, wq_0, wk_0, wv_0, wq_st, wk_st, wv_st, wq_b, wk_b, wv_b, wo_l,
            kt_l, vt_l, ht_l, acc, b_s, out_v, q_s, k_s, v_s, ctx_s, gate_s, par_s, kpad_s, u_s, ub_s,
            V_s, H_s, W_s, sems):
    step = pl.program_id(0)
    P = functools.partial
    wsets = ((wq_h, wq_l, wq_0, wq_st, wq_b, M, SEM_WQ), (wk_h, wk_l, wk_0, wk_st, wk_b, DC, SEM_WK),
             (wv_h, wv_l, wv_0, wv_st, wv_b, DC, SEM_WV))

    def late_copies():
        q = step % SPB
        blk = jnp.minimum(step // SPB + 1, NBLK - 1)
        cps = [pltpu.make_async_copy(wo_h.at[pl.ds(pl.multiple_of(step * 256, 256), 256), :], wo_l, sems.at[SEM_WO])]
        for (wh, wl, w0, st_, wb, rows, sem) in wsets:
            nr = rows // SPB
            cps.append(pltpu.make_async_copy(
                wh.at[pl.ds(pl.multiple_of(q * nr, nr), nr), pl.ds(pl.multiple_of(blk * HB, HB), HB), :], wl, sems.at[sem]))
        return cps

    def early_copies(n):
        col = pl.multiple_of((jnp.minimum(n, NSTEP - 1) // 2) * 128, 128)
        return [pltpu.make_async_copy(k_h.at[:, pl.ds(col, 128)], kt_l, sems.at[SEM_KT]),
                pltpu.make_async_copy(v_h.at[:, pl.ds(col, 128)], vt_l, sems.at[SEM_VT]),
                pltpu.make_async_copy(h_h.at[pl.ds(col, 128), :], ht_l, sems.at[SEM_HT])]

    def part_copies(p):
        a, b = (0, NP0 * BQ) if p == 0 else (NP0 * BQ, S)
        return [pltpu.make_async_copy(c_h.at[a:b, :], c_v.at[a:b, :], sems.at[SEM_C + p]),
                pltpu.make_async_copy(x_h.at[a:b, :], x_v.at[a:b, :], sems.at[SEM_X + p])]

    @pl.when(step == 0)
    def _():
        w0 = [pltpu.make_async_copy(ws[0].at[:, 0:HB, :], ws[2], sems.at[SEM_W0 + n]) for n, ws in enumerate(wsets)]
        sm = [pltpu.make_async_copy(a, b, sems.at[SEM_SM + n]) for n, (a, b) in enumerate(
            ((skt_h, skt_ref), (dd_h, dd_ref), (gw_h, gw_ref), (f_h, f_ref), (g_h, g_ref)))]
        for cp in w0 + sm + part_copies(0) + early_copies(step) + part_copies(1): cp.start()

        def zero(i, c):
            rs = pl.ds(pl.multiple_of(i * 64, 64), 64)
            acc[rs, :] = jnp.zeros((64, M), f32)
            b_s[rs, :] = jnp.zeros((64, M), f32)
            return c
        jax.lax.fori_loop(0, S // 64, zero, 0)
        for cp in sm: cp.wait()
        par_s[0:4, :] = skt_ref[...].astype(f32)
        par_s[4:5, :] = 0.5 * dd_ref[...].astype(f32).reshape(1, M)
        par_s[5:6, :] = gw_ref[...].astype(f32).reshape(1, M)
        par_s[6:8, :] = jnp.zeros((2, M), f32)
        kpad_s[0:8, :] = jnp.zeros((8, D), f32)
        for n, (wh, wl, wz, st_, wb, rows, sem) in enumerate(wsets):
            w0[n].wait()

            def stg(i, c, wz=wz, st_=st_, wb=wb):
                m0 = pl.multiple_of(i * 64, 64)
                st_[0, pl.ds(pl.multiple_of(m0 * HB, 64), 64 * HB), :] = wz[pl.ds(m0, 64)].astype(f32).reshape(64 * HB, D)
                ws = [st_[0, pl.ds(hh + m0 * HB, 64, stride=HB), :] for hh in range(HP)]
                wb[pl.ds(m0, 64), :] = jnp.concatenate(ws, axis=1).astype(bf16)
                return c
            jax.lax.fori_loop(0, rows // 64, stg, 0)
        for cp in part_copies(0): cp.wait()

    for cp in late_copies(): cp.start()
    for cp in early_copies(step): cp.wait()

    ct = step // 2
    half = step % 2
    ccol = pl.ds(pl.multiple_of(ct * 128, 128), 128)
    scale = (D ** -0.5) * LOG2E
    row = jax.lax.broadcasted_iota(jnp.int32, (128, 128), 0)
    col = jax.lax.broadcasted_iota(jnp.int32, (128, 128), 1)
    mask = col <= row
    never8 = f_ref[0, 0:8, :].astype(f32) > 2.0
    never = jnp.concatenate([never8] * 16, axis=0)

    side = collections.deque()
    budget = [0.0]

    def pin(arr, spacing):
        R = arr.shape[0]
        out, lastr = [], 0
        for g in range(R // 8):
            budget[0] = min(budget[0] + RATE * spacing, 80.0)
            if side and budget[0] >= side[0][0]:
                cost, fn = side.popleft()
                budget[0] -= cost
                v = fn()
                if g * 8 > lastr:
                    out.append(arr[lastr:g * 8])
                out.append(jnp.where(never8, v, arr[g * 8:(g + 1) * 8]))
                lastr = (g + 1) * 8
        if lastr == 0:
            return arr
        if lastr < R:
            out.append(arr[lastr:])
        return jnp.concatenate(out, axis=0)

    def flush():
        if side and CFG.get("dbg"): print("flush leftover", len(side))
        while side:
            side.popleft()[1]()

    def pq(i, hh):
        r0 = i * BQ; r1 = r0 + BQ
        hs = slice(hh * D, (hh + 1) * D)
        r = jnp.dot(x_v[r0:r1, :], wq_b[:, hs], preferred_element_type=f32)
        q_s[r0:r1, hs] = (pin(r, 8) * scale).astype(bf16)

    def pk(i, hh):
        r0 = i * BQ; r1 = r0 + BQ
        hs = slice(hh * D, (hh + 1) * D)
        r = jnp.dot(c_v[r0:r1, :], wk_b[:, hs], preferred_element_type=f32)
        k_s[r0:r1, hs] = pin(r, 8).astype(bf16)

    def pvv(i, hh):
        r0 = i * BQ; r1 = r0 + BQ
        hs = slice(hh * D, (hh + 1) * D)
        r = jnp.dot(c_v[r0:r1, :], wv_b[:, hs], preferred_element_type=f32)
        v_s[r0:r1, hs] = pin(r, 8).astype(bf16)

    def chunks(i):
        nt = 2 * i + 1
        out, t = [], 0
        while t < nt:
            n = min(KC, nt - t)
            out.append((0, t * 128, (t + n) * 128))
            t += n
        out.append((128, nt * 128, (nt + 1) * 128))
        return out

    st = {}

    def qk_atom(i, hh, ch):
        rl, kl, kh = ch
        r0 = i * BQ
        hs = slice(hh * D, (hh + 1) * D)
        s = jax.lax.dot_general(q_s[r0 + rl:r0 + BQ, hs], k_s[kl:kh, hs], NT, preferred_element_type=f32)
        nt = (kh - kl) // 128
        tiles = [s[:, t * 128:(t + 1) * 128] for t in range(nt)]
        if kh > r0 + rl:
            d = tiles[-1]
            dm = jnp.where(mask, d[:128], -1e30)
            tiles[-1] = dm if rl == 128 else jnp.concatenate([dm, d[128:]], axis=0)
        u = st.setdefault((i, hh), {"m": [None, None], "l": [None, None], "o": [None, None]})
        u[("s", ch)] = tiles
        mm = functools.reduce(jnp.maximum, tiles)
        for g in range(rl // 128, 2):
            a = mm[g * 128 - rl:(g + 1) * 128 - rl]
            u["m"][g] = a if u["m"][g] is None else jnp.maximum(u["m"][g], a)

    def qk(i, hh):
        for ch in chunks(i): qk_atom(i, hh, ch)
        u = st[(i, hh)]
        u["M"] = [jnp.broadcast_to(jnp.max(u["m"][g], axis=1, keepdims=True), (128, 128)) for g in range(2)]

    def pv_atom(i, hh, ch):
        rl, kl, kh = ch
        hs = slice(hh * D, (hh + 1) * D)
        u = st[(i, hh)]
        m = u["M"][1] if rl == 128 else jnp.concatenate(u["M"], axis=0)
        ps = [jnp.exp2(t - m) for t in u[("s", ch)]]
        lp = functools.reduce(jnp.add, ps)
        ls = []
        for g in range(rl // 128, 2):
            a = lp[g * 128 - rl:(g + 1) * 128 - rl]
            u["l"][g] = a if u["l"][g] is None else u["l"][g] + a
            ls.append(u["l"][g])
        ps[-1] = jnp.minimum(ps[-1], jnp.concatenate(ls, axis=0) if len(ls) > 1 else ls[0])
        pb = (jnp.concatenate(ps, axis=1) if len(ps) > 1 else ps[0]).astype(bf16)
        o = jnp.dot(pb, v_s[kl:kh, hs], preferred_element_type=f32)
        for g in range(rl // 128, 2):
            a = o[g * 128 - rl:(g + 1) * 128 - rl]
            u["o"][g] = a if u["o"][g] is None else u["o"][g] + a

    def recip(l):
        if CFG.get("exactdiv"):
            return 1.0 / l
        r = pl.reciprocal(l, approx=True)
        return r * (2.0 - l * r)

    def norm_piece(i, hh, g, r):
        u = st[(i, hh)]
        hs = slice(hh * D, (hh + 1) * D)
        o = u["o"][g][r:r + 16]
        c = o * recip(u["L"][g][r:r + 16])
        ctx_s[i, g * 128 + r:g * 128 + r + 16, hs] = c.astype(bf16)
        return jnp.maximum(c[:8], c[8:])

    def pv(i, hh, defer):
        for ch in chunks(i): pv_atom(i, hh, ch)
        u = st[(i, hh)]
        u["L"] = [jnp.sum(jnp.where(never, u["o"][g], u["l"][g]), axis=1, keepdims=True) for g in range(2)]
        pieces = [(CFG.get("normc", 32), P(norm_piece, i, hh, g, r)) for g in range(2) for r in range(0, 128, 16)]
        if defer:
            side.extendleft(reversed(pieces))
            u["left"] = len(side) - len(pieces)
        else:
            for _, fn in pieces: fn()

    def oproj(i, atoms=range(4)):
        r0 = i * BQ; r1 = r0 + BQ
        for a in atoms:
            cs = slice(a * 256, (a + 1) * 256)
            r = jnp.dot(ctx_s[i], wo_l[:, cs], preferred_element_type=f32)
            r = jnp.concatenate([pin(r[:, :128], 8), r[:, 128:]], axis=1)
            acc[r0:r1, cs] += r

    cv = {}

    def u_piece(r):
        j = r // C
        par = cv["par"]
        ks = kpad_s[8 + r:24 + r, :] * par[0:1]
        for t in range(1, 4):
            ks = ks + kpad_s[8 - t + r:24 - t + r, :] * par[t:t + 1]
        u = ks * vt_l[r:r + 16, :].astype(f32)
        ub_s[r - j * C:r - j * C + 16, j * 128:(j + 1) * 128] = u.astype(bf16)
        u_s[r:r + 16, :] = u * par[4:5]
        return jnp.maximum(u[:8], u[8:])

    def queue_u():
        cv["par"] = par_s[:, ccol]
        kpad_s[8:8 + S, :] = kt_l[...].astype(f32)
        for r in range(0, S, 16):
            side.append((28, P(u_piece, r)))

    def split(T, j):
        t = T[:, j * 128:(j + 1) * 128]
        re = jnp.concatenate([t[16 * g:16 * g + 8] for g in range(8)], axis=0)
        im = jnp.concatenate([t[16 * g + 8:16 * g + 16] for g in range(8)], axis=0)
        return re, im

    def fwdu(hf):
        lo, hi = hf * NCH // 2, (hf + 1) * NCH // 2
        U = jnp.dot(f_ref[half], ub_s[:, lo * 128:hi * 128], preferred_element_type=f32)
        for j in range(lo, hi):
            re, im = split(U, j - lo)
            V_s[0, j] = re
            V_s[1, j] = im
            V_s[2, j] = re + im

    def fwdh(hf):
        lo, hi = hf * NCH // 2, (hf + 1) * NCH // 2
        hcat = jnp.concatenate([ht_l[:, j * C:(j + 1) * C] for j in range(lo, hi)], axis=0)
        Hf = jax.lax.dot_general(f_ref[half], hcat, NT, preferred_element_type=f32)
        for j in range(lo, hi):
            re, im = split(Hf, j - lo)
            H_s[0, j] = im - re
            H_s[1, j] = re + im
            H_s[2, j] = re

    def mac_piece(i, r, a):
        rs = slice(r, r + 8)
        s = functools.reduce(jnp.add, [H_s[a, i - j, rs, :] * V_s[a, j, rs, :] for j in range(i + 1)])
        cv[a] = s
        if a == 2:
            yr, yi = s - cv[1], s + cv[0]
            wr, wi = yr, yi
            if i > 0:
                pr, pi = cv[("y", r)]
                wr, wi = (yr - pi, yi + pr) if r < 32 else (yr + pi, yi - pr)
            cv[("y", r)] = (yr, yi)
            W_s[2 * r:2 * r + 16, i * 128:(i + 1) * 128] = jnp.concatenate([wr, wi], axis=0)
        return s

    def queue_mac():
        for i2 in range(NCH):
            for r in range(0, 64, 8):
                for a in range(3):
                    side.append((MACW * (2 * (i2 + 1) + 3), P(mac_piece, i2, r, a)))

    def inv(hf):
        lo, hi = hf * NCH // 2, (hf + 1) * NCH // 2
        Y = jnp.dot(g_ref[half], W_s[:, lo * 128:hi * 128].astype(bf16), preferred_element_type=f32)
        for j in range(lo, hi):
            a, b = j * C, (j + 1) * C
            y = Y[:, (j - lo) * 128:(j - lo + 1) * 128]
            b_s[a:b, ccol] += x_v[a:b, ccol].astype(f32) * (y + u_s[a:b, :])

    def gate_piece(r):
        rs = pl.ds(pl.multiple_of(step * GR + r, 16), 16)
        xs = x_v[rs, :].astype(f32) * par_s[5:6, :]
        z = jnp.sum(xs, axis=1, keepdims=True)
        g = jnp.broadcast_to(jax.nn.sigmoid(z), (16, 128))
        gate_s[rs, :] = g
        return jnp.maximum(g[:8], g[8:])

    def stage_piece(src, st_, slot, dst0, m0):
        w = src[m0:m0 + 4].astype(f32).reshape(4 * HB, D)
        st_[slot, pl.ds(dst0, 4 * HB), :] = w
        return functools.reduce(jnp.maximum, [w[k * 8:(k + 1) * 8] for k in range(4)])

    def extract_piece(st_, wb, slot, head, m0):
        ws = [st_[slot, pl.ds(head + hh + m0 * HB, 8, stride=HB), :] for hh in range(HP)]
        wb[m0:m0 + 8, :] = jnp.concatenate(ws, axis=1).astype(bf16)
        return ws[0]

    def queue_stage():
        nslot = (step // SPB + 1) % 2
        qtr = step % SPB
        for (wh, wl, wz, st_, wb, rows, sem) in wsets:
            nr = rows // SPB
            for m0 in range(0, nr, 4):
                side.append((12, P(stage_piece, wl, st_, nslot, pl.multiple_of((qtr * nr + m0) * HB, 8), m0)))

    def queue_extract():
        nstep = step + 1
        for (wh, wl, wz, st_, wb, rows, sem) in wsets:
            for m0 in range(0, rows, 8):
                side.append((8, P(extract_piece, st_, wb, (nstep // SPB) % 2, (nstep % SPB) * HP, m0)))

    units = [(u // 2, u % 2) for u in range(NU)]

    queue_u()
    pq(0, 0); pk(0, 0); pq(0, 1); pk(0, 1)
    qk(0, 0)
    pvv(0, 0); pvv(0, 1)
    fwdh(0); fwdh(1)
    odone = 0
    ND = CFG.get("normdefer", 1)
    for s in range(NU):
        i, hh = units[s]
        if s == FW:
            flush()
            fwdu(0); fwdu(1)
            for cp in early_copies(step + 1): cp.start()
            for cp in late_copies(): cp.wait()

            @pl.when(step == 0)
            def _():
                for cp in part_copies(1): cp.wait()
            for r in range(0, GR, 16):
                side.append((70, P(gate_piece, r)))
            queue_mac()
            queue_stage()
        if s == NU - 2:
            flush()
            queue_extract()
        if i + 1 < NB:
            pk(i + 1, hh); pq(i + 1, hh); pvv(i + 1, hh)
            if s >= 1 and "left" in st[units[s - 1]]:
                assert len(side) <= max(st[units[s - 1]]["left"], 0) or s == FW, (s, len(side))
        if s >= FW and odone < i and s < NU - 2:
            oproj(odone); odone += 1
        if s == NU - 2:
            oproj(NB - 2, (0, 1))
        if s == NU - 1:
            oproj(NB - 2, (2, 3))
        pv(i, hh, ND and s + 1 < NU - 2 and s + 1 != FW)
        if s + 1 < NU:
            qk(*units[s + 1])
    inv(0); inv(1)
    assert odone == NB - 2
    oproj(NB - 1)
    flush()

    @pl.when(step == NSTEP - 1)
    def _():
        RC = 128

        def fin(i, c):
            rs = pl.ds(pl.multiple_of(i * RC, RC), RC)
            g = gate_s[rs, :]
            g = jnp.concatenate([g] * (M // 128), axis=1)
            out_v[rs, :] = (g * acc[rs, :] + (1.0 - g) * b_s[rs, :]).astype(bf16)
            pltpu.make_async_copy(out_v.at[rs, :], o_h.at[rs, :], sems.at[SEM_OUT]).start()
            return c
        jax.lax.fori_loop(0, S // RC, fin, 0)
        for cp in early_copies(step + 1): cp.wait()
        pltpu.make_async_copy(out_v, o_h, sems.at[SEM_OUT]).wait()


@jax.jit
def pallas_gated_mix__compressed_kv_cla__ssm_conv_h3__prompt_kernel(A_x, A_c_kv, A_w_q, A_w_uk, A_w_uv, A_w_o, B_q, B_k, B_v, B_shift_k, B_ssm_k, B_ssm_D, gate_w):
    x = A_x.reshape(S, M)
    c = A_c_kv.reshape(S, DC)
    wo = A_w_o.reshape(H * D, M)
    k = B_k.reshape(S, M)
    v = B_v.reshape(S, M)
    Fc, Gc = _dft_consts()
    Fc = jnp.asarray(Fc, bf16); Gc = jnp.asarray(Gc, bf16)
    hbm = pl.BlockSpec(memory_space=pl.ANY)
    vm = pl.BlockSpec(memory_space=pltpu.VMEM)
    scratch = [
        pltpu.VMEM((4, M), bf16), pltpu.VMEM((M,), bf16), pltpu.VMEM((M,), bf16),
        pltpu.VMEM((2, 128, C), bf16), pltpu.VMEM((2, C, 128), bf16),
        pltpu.VMEM((S, M), bf16),
        pltpu.VMEM((S, DC), bf16),
        pltpu.VMEM((M // SPB, HB, D), bf16),
        pltpu.VMEM((DC // SPB, HB, D), bf16),
        pltpu.VMEM((DC // SPB, HB, D), bf16),
        pltpu.VMEM((M, HB, D), bf16),
        pltpu.VMEM((DC, HB, D), bf16),
        pltpu.VMEM((DC, HB, D), bf16),
        pltpu.VMEM((2, M * HB, D), f32),
        pltpu.VMEM((2, DC * HB, D), f32),
        pltpu.VMEM((2, DC * HB, D), f32),
        pltpu.VMEM((M, HP * D), bf16),
        pltpu.VMEM((DC, HP * D), bf16),
        pltpu.VMEM((DC, HP * D), bf16),
        pltpu.VMEM((HP * D, M), bf16),
        pltpu.VMEM((S, 128), bf16),
        pltpu.VMEM((S, 128), bf16),
        pltpu.VMEM((128, S), bf16),
        pltpu.VMEM((S, M), f32),
        pltpu.VMEM((S, M), f32),
        pltpu.VMEM((S, M), bf16),
        pltpu.VMEM((S, HP * D), bf16),
        pltpu.VMEM((S, HP * D), bf16),
        pltpu.VMEM((S, HP * D), bf16),
        pltpu.VMEM((NB, BQ, HP * D), bf16),
        pltpu.VMEM((S, 128), f32),
        pltpu.VMEM((8, M), f32),
        pltpu.VMEM((S + 8, 128), f32),
        pltpu.VMEM((S, 128), f32),
        pltpu.VMEM((C, NCH * 128), bf16),
        pltpu.VMEM((3, NCH, 64, 128), f32),
        pltpu.VMEM((3, NCH, 64, 128), f32),
        pltpu.VMEM((128, NCH * 128), f32),
        pltpu.SemaphoreType.DMA((NSEM,)),
    ]
    out = pl.pallas_call(
        _kernel,
        out_shape=jax.ShapeDtypeStruct((S, M), bf16),
        grid=(NSTEP,),
        in_specs=[hbm] * 14,
        out_specs=hbm,
        scratch_shapes=scratch,
        compiler_params=pltpu.CompilerParams(vmem_limit_bytes=120 * 1024 * 1024, dimension_semantics=("arbitrary",),
                                             disable_bounds_checks=True),
    )(x, c, A_w_q, A_w_uk, A_w_uv, wo, k, v, B_ssm_k, B_shift_k.T, B_ssm_D, gate_w, Fc, Gc)
    return out.reshape(1, S, M)
```

```python
import collections
import functools
import numpy as np
import jax
import jax.numpy as jnp
import jax.experimental.pallas as pl
import jax.experimental.pallas.tpu as pltpu

f32, bf16 = jnp.float32, jnp.bfloat16
NT = (((1,), (1,)), ((), ()))

S = 2048
M = 1024
DC = 512
H = 32
D = 128
HP = 2
NSTEP = H // HP
BQ = 256
NB = S // BQ
NU = 2 * NB
C = 128
NCH = S // C
HB = 8
SPB = HB // HP
NBLK = H // HB
GR = S // NSTEP
LOG2E = 1.4426950408889634

CFG = {}
KC = CFG.get("kc", 4)
RATE = CFG.get("rate", 2.0)
MACW = CFG.get("macw", 2.25)
FW = CFG.get("fw", 4)
NP0 = FW // 2 + 1

SEM_WQ, SEM_WK, SEM_WV, SEM_WO, SEM_KT, SEM_VT, SEM_HT = range(7)
SEM_W0 = 7
SEM_C = 10
SEM_X = 12
SEM_OUT = 14
SEM_SM = 15
NSEM = 20


def _dft_consts():
    n = np.arange(C)
    Fs, Gs = [], []
    for p in range(2):
        ks = np.arange(p * 64, (p + 1) * 64)
        ks = np.concatenate([ks[ks % 2 == 0], ks[ks % 2 == 1]])
        th = np.pi * (2 * ks[:, None] + 1) * n[None, :] / (2 * C)
        F = np.stack([np.cos(th).reshape(8, 8, C), -np.sin(th).reshape(8, 8, C)], axis=1).reshape(128, C)
        Fs.append(F); Gs.append(F.T / C)
    return np.stack(Fs).astype(np.float32), np.stack(Gs).astype(np.float32)


def _kernel(x_h, c_h, wq_h, wk_h, wv_h, wo_h, k_h, v_h, h_h,
            skt_h, dd_h, gw_h, f_h, g_h,
            o_h,
            skt_ref, dd_ref, gw_ref, f_ref, g_ref,
            x_v, c_v, wq_l, wk_l, wv_l, wq_0, wk_0, wv_0, wq_st, wk_st, wv_st, wq_b, wk_b, wv_b, wo_l,
            kt_l, vt_l, ht_l, acc, b_s, out_v, q_s, k_s, v_s, ctx_s, gate_s, par_s, ub_s,
            V_s, H_s, W_s, s_a, s_b, sems):
    s_s = (s_a, s_b)
    step = pl.program_id(0)
    P = functools.partial
    wsets = ((wq_h, wq_l, wq_0, wq_st, wq_b, M, SEM_WQ), (wk_h, wk_l, wk_0, wk_st, wk_b, DC, SEM_WK),
             (wv_h, wv_l, wv_0, wv_st, wv_b, DC, SEM_WV))

    def late_copies():
        q = step % SPB
        blk = jnp.minimum(step // SPB + 1, NBLK - 1)
        cps = [pltpu.make_async_copy(wo_h.at[pl.ds(pl.multiple_of(step * 256, 256), 256), :], wo_l, sems.at[SEM_WO])]
        for (wh, wl, w0, st_, wb, rows, sem) in wsets:
            nr = rows // SPB
            cps.append(pltpu.make_async_copy(
                wh.at[pl.ds(pl.multiple_of(q * nr, nr), nr), pl.ds(pl.multiple_of(blk * HB, HB), HB), :], wl, sems.at[sem]))
        return cps

    def early_copies(n):
        col = pl.multiple_of((jnp.minimum(n, NSTEP - 1) // 2) * 128, 128)
        return [pltpu.make_async_copy(k_h.at[:, pl.ds(col, 128)], kt_l, sems.at[SEM_KT]),
                pltpu.make_async_copy(v_h.at[:, pl.ds(col, 128)], vt_l, sems.at[SEM_VT]),
                pltpu.make_async_copy(h_h.at[pl.ds(col, 128), :], ht_l, sems.at[SEM_HT])]

    def part_copies(p):
        a, b = (0, NP0 * BQ) if p == 0 else (NP0 * BQ, S)
        return [pltpu.make_async_copy(c_h.at[a:b, :], c_v.at[a:b, :], sems.at[SEM_C + p]),
                pltpu.make_async_copy(x_h.at[a:b, :], x_v.at[a:b, :], sems.at[SEM_X + p])]

    @pl.when(step == 0)
    def _():
        w0 = [pltpu.make_async_copy(ws[0].at[:, 0:HB, :], ws[2], sems.at[SEM_W0 + n]) for n, ws in enumerate(wsets)]
        sm = [pltpu.make_async_copy(a, b, sems.at[SEM_SM + n]) for n, (a, b) in enumerate(
            ((skt_h, skt_ref), (dd_h, dd_ref), (gw_h, gw_ref), (f_h, f_ref), (g_h, g_ref)))]
        P1 = CFG.get('p1', 0)
        for cp in w0 + sm + part_copies(0) + early_copies(step) + (part_copies(1) if P1 == 0 else []): cp.start()

        def zero(i, c):
            rs = pl.ds(pl.multiple_of(i * 64, 64), 64)
            acc[rs, :] = jnp.zeros((64, M), f32)
            b_s[rs, :] = jnp.zeros((64, M), f32)
            return c
        jax.lax.fori_loop(0, S // 64, zero, 0)
        for cp in sm: cp.wait()
        par_s[0:4, :] = skt_ref[...].astype(f32)
        par_s[4:5, :] = 0.5 * dd_ref[...].astype(f32).reshape(1, M)
        par_s[5:6, :] = gw_ref[...].astype(f32).reshape(1, M)
        par_s[6:8, :] = jnp.zeros((2, M), f32)
        for n, (wh, wl, wz, st_, wb, rows, sem) in enumerate(wsets):
            w0[n].wait()
            if P1 == n + 1:
                for cp in part_copies(1): cp.start()

            def stg(i, c, wz=wz, st_=st_, wb=wb):
                m0 = pl.multiple_of(i * 64, 64)
                st_[0, pl.ds(pl.multiple_of(m0 * HB, 64), 64 * HB), :] = wz[pl.ds(m0, 64)].astype(f32).reshape(64 * HB, D)
                ws = [st_[0, pl.ds(hh + m0 * HB, 64, stride=HB), :] for hh in range(HP)]
                wb[pl.ds(m0, 64), :] = jnp.concatenate(ws, axis=1).astype(bf16)
                return c
            jax.lax.fori_loop(0, rows // 64, stg, 0)
        if P1 == 4:
            for cp in part_copies(1): cp.start()
        for cp in part_copies(0): cp.wait()
        if P1 == 5:
            for cp in part_copies(1): cp.start()

    for cp in late_copies(): cp.start()
    for cp in early_copies(step): cp.wait()

    ct = step // 2
    half = step % 2
    ccol = pl.ds(pl.multiple_of(ct * 128, 128), 128)
    scale = (D ** -0.5) * LOG2E
    row = jax.lax.broadcasted_iota(jnp.int32, (128, 128), 0)
    col = jax.lax.broadcasted_iota(jnp.int32, (128, 128), 1)
    mask = col <= row
    never8 = f_ref[0, 0:8, :].astype(f32) > 2.0
    never = jnp.concatenate([never8] * 16, axis=0)

    side = collections.deque()
    budget = [0.0]

    def pin(arr, spacing):
        R = arr.shape[0]
        out, lastr = [], 0
        for g in range(R // 8):
            budget[0] = min(budget[0] + RATE * spacing, 80.0)
            if side and budget[0] >= side[0][0]:
                cost, fn = side.popleft()
                budget[0] -= cost
                v = fn()
                if g * 8 > lastr:
                    out.append(arr[lastr:g * 8])
                out.append(jnp.where(never8, v, arr[g * 8:(g + 1) * 8]))
                lastr = (g + 1) * 8
        if lastr == 0:
            return arr
        if lastr < R:
            out.append(arr[lastr:])
        return jnp.concatenate(out, axis=0)

    def flush():
        if side and CFG.get("dbg"): print("flush leftover", len(side))
        while side:
            side.popleft()[1]()

    def pq(i, hh):
        r0 = i * BQ; r1 = r0 + BQ
        hs = slice(hh * D, (hh + 1) * D)
        r = jnp.dot(x_v[r0:r1, :], wq_b[:, hs], preferred_element_type=f32)
        q_s[r0:r1, hs] = (pin(r, 8) * scale).astype(bf16)

    def pk(i, hh):
        r0 = i * BQ; r1 = r0 + BQ
        hs = slice(hh * D, (hh + 1) * D)
        r = jnp.dot(c_v[r0:r1, :], wk_b[:, hs], preferred_element_type=f32)
        k_s[r0:r1, hs] = pin(r, 8).astype(bf16)

    def pvv(i, hh):
        r0 = i * BQ; r1 = r0 + BQ
        hs = slice(hh * D, (hh + 1) * D)
        r = jnp.dot(c_v[r0:r1, :], wv_b[:, hs], preferred_element_type=f32)
        v_s[r0:r1, hs] = pin(r, 8).astype(bf16)

    def chunks(i):
        nt = 2 * i + 1
        out, t = [], 0
        while t < nt:
            n = min(KC, nt - t)
            out.append((0, t * 128, (t + n) * 128))
            t += n
        out.append((128, nt * 128, (nt + 1) * 128))
        return out

    st = {}

    def qk_atom(i, hh, ch):
        rl, kl, kh = ch
        r0 = i * BQ
        hs = slice(hh * D, (hh + 1) * D)
        s = jax.lax.dot_general(q_s[r0 + rl:r0 + BQ, hs], k_s[kl:kh, hs], NT, preferred_element_type=f32)
        nt = (kh - kl) // 128
        tiles = [s[:, t * 128:(t + 1) * 128] for t in range(nt)]
        if kh > r0 + rl:
            d = tiles[-1]
            dm = jnp.where(mask, d[:128], -1e30)
            tiles[-1] = dm if rl == 128 else jnp.concatenate([dm, d[128:]], axis=0)
        u = st.setdefault((i, hh), {"m": [None, None], "l": [None, None], "o": [None, None]})
        u[("s", ch)] = tiles
        if CFG.get("smem", 1):
            for t in range(nt):
                s_s[hh][rl:BQ, kl + t * 128:kl + (t + 1) * 128] = tiles[t]
        mm = functools.reduce(jnp.maximum, tiles)
        for g in range(rl // 128, 2):
            a = mm[g * 128 - rl:(g + 1) * 128 - rl]
            u["m"][g] = a if u["m"][g] is None else jnp.maximum(u["m"][g], a)

    def qk(i, hh):
        for ch in chunks(i): qk_atom(i, hh, ch)
        u = st[(i, hh)]
        u["M"] = [jnp.broadcast_to(jnp.max(u["m"][g], axis=1, keepdims=True), (128, 128)) for g in range(2)]
        if CFG.get("smem", 1):
            s_s[hh][pl.ds(pl.multiple_of(BQ + (step >> 8) * 8, 8), 8), 0:128] = u["m"][1][120:128]

    def pv_atom(i, hh, ch):
        rl, kl, kh = ch
        hs = slice(hh * D, (hh + 1) * D)
        u = st[(i, hh)]
        m = u["M"][1] if rl == 128 else jnp.concatenate(u["M"], axis=0)
        if CFG.get("smem", 1):
            ps = [jnp.exp2(s_s[hh][rl:BQ, k0:k0 + 128] - m) for k0 in range(kl, kh, 128)]
        else:
            ps = [jnp.exp2(t - m) for t in u[("s", ch)]]
        lp = functools.reduce(jnp.add, ps)
        ls = []
        for g in range(rl // 128, 2):
            a = lp[g * 128 - rl:(g + 1) * 128 - rl]
            u["l"][g] = a if u["l"][g] is None else u["l"][g] + a
            ls.append(u["l"][g])
        ps[-1] = jnp.minimum(ps[-1], jnp.concatenate(ls, axis=0) if len(ls) > 1 else ls[0])
        pb = (jnp.concatenate(ps, axis=1) if len(ps) > 1 else ps[0]).astype(bf16)
        o = jnp.dot(pb, v_s[kl:kh, hs], preferred_element_type=f32)
        for g in range(rl // 128, 2):
            a = o[g * 128 - rl:(g + 1) * 128 - rl]
            u["o"][g] = a if u["o"][g] is None else u["o"][g] + a

    def recip(l):
        if CFG.get("exactdiv"):
            return 1.0 / l
        r = pl.reciprocal(l, approx=True)
        return r * (2.0 - l * r)

    def norm_piece(i, hh, g, r):
        u = st[(i, hh)]
        hs = slice(hh * D, (hh + 1) * D)
        o = u["o"][g][r:r + 16]
        c = o * recip(u["L"][g][r:r + 16])
        ctx_s[i, g * 128 + r:g * 128 + r + 16, hs] = c.astype(bf16)
        return jnp.maximum(c[:8], c[8:])

    def pv(i, hh, defer):
        for ch in chunks(i): pv_atom(i, hh, ch)
        u = st[(i, hh)]
        u["L"] = [jnp.sum(jnp.where(never, u["o"][g], u["l"][g]), axis=1, keepdims=True) for g in range(2)]
        pieces = [(CFG.get("normc", 32), P(norm_piece, i, hh, g, r)) for g in range(2) for r in range(0, 128, 16)]
        if defer:
            side.extendleft(reversed(pieces))
            u["left"] = len(side) - len(pieces)
        else:
            for _, fn in pieces: fn()

    def oproj(i, atoms=range(4)):
        r0 = i * BQ; r1 = r0 + BQ
        for a in atoms:
            cs = slice(a * 256, (a + 1) * 256)
            r = jnp.dot(ctx_s[i], wo_l[:, cs], preferred_element_type=f32)
            r = jnp.concatenate([pin(r[:, :128], 8), r[:, 128:]], axis=1)
            acc[r0:r1, cs] += r

    cv = {}

    UR = CFG.get("ur", 16)

    def u_piece(r):
        j = r // C
        par = cv["par"]
        if r == 0:
            kf = jnp.concatenate([jnp.zeros((8, 128), f32), kt_l[0:UR, :].astype(f32)], axis=0)
        else:
            kf = kt_l[r - 16:r + UR, :].astype(f32)[8:]
        ks = kf[8:] * par[0:1]
        for t in range(1, 4):
            ks = ks + kf[8 - t:8 - t + UR] * par[t:t + 1]
        u = ks * vt_l[r:r + UR, :].astype(f32)
        ub_s[r - j * C:r - j * C + UR, j * 128:(j + 1) * 128] = u.astype(bf16)
        b_s[r:r + UR, ccol] += u * par[4:5]
        return functools.reduce(jnp.maximum, [u[k:k + 8] for k in range(0, UR, 8)])

    def queue_u():
        cv["par"] = par_s[:, ccol]
        for r in range(0, S, UR):
            side.append((CFG.get("uc", 2.5) * UR, P(u_piece, r)))

    def split(T, j):
        t = T[:, j * 128:(j + 1) * 128]
        re = jnp.concatenate([t[16 * g:16 * g + 8] for g in range(8)], axis=0)
        im = jnp.concatenate([t[16 * g + 8:16 * g + 16] for g in range(8)], axis=0)
        return re, im

    def fwdu(hf):
        lo, hi = hf * NCH // 2, (hf + 1) * NCH // 2
        U = jnp.dot(f_ref[half], ub_s[:, lo * 128:hi * 128], preferred_element_type=f32)
        for j in range(lo, hi):
            re, im = split(U, j - lo)
            V_s[0, j] = re
            V_s[1, j] = im
            V_s[2, j] = re + im

    def fwdh(hf):
        lo, hi = hf * NCH // 2, (hf + 1) * NCH // 2
        hcat = jnp.concatenate([ht_l[:, j * C:(j + 1) * C] for j in range(lo, hi)], axis=0)
        Hf = jax.lax.dot_general(f_ref[half], hcat, NT, preferred_element_type=f32)
        for j in range(lo, hi):
            re, im = split(Hf, j - lo)
            H_s[0, j] = im - re
            H_s[1, j] = re + im
            H_s[2, j] = re

    def mac_piece(i, r, a):
        rs = slice(r, r + 8)
        s = functools.reduce(jnp.add, [H_s[a, i - j, rs, :] * V_s[a, j, rs, :] for j in range(i + 1)])
        cv[a] = s
        if a == 2:
            yr, yi = s - cv[1], s + cv[0]
            wr, wi = yr, yi
            if i > 0:
                pr, pi = cv[("y", r)]
                wr, wi = (yr - pi, yi + pr) if r < 32 else (yr + pi, yi - pr)
            cv[("y", r)] = (yr, yi)
            W_s[2 * r:2 * r + 16, i * 128:(i + 1) * 128] = jnp.concatenate([wr, wi], axis=0).astype(W_s.dtype)
        return s

    def queue_mac():
        for i2 in range(NCH):
            for r in range(0, 64, 8):
                for a in range(3):
                    side.append((MACW * (2 * (i2 + 1) + 3), P(mac_piece, i2, r, a)))

    def inv(hf):
        lo, hi = hf * NCH // 2, (hf + 1) * NCH // 2
        Y = jnp.dot(g_ref[half], W_s[:, lo * 128:hi * 128].astype(bf16), preferred_element_type=f32)
        for j in range(lo, hi):
            a, b = j * C, (j + 1) * C
            y = Y[:, (j - lo) * 128:(j - lo + 1) * 128]
            b_s[a:b, ccol] += y

    def gate_piece(r):
        rs = pl.ds(pl.multiple_of(step * GR + r, 8), 8)
        xs = x_v[rs, :].astype(f32) * par_s[5:6, :]
        z = functools.reduce(jnp.add, [xs[:, t * 128:(t + 1) * 128] for t in range(M // 128)])
        gate_s[rs, :] = z
        return z

    def stage_piece(src, st_, slot, dst0, m0):
        w = src[m0:m0 + 4].astype(f32).reshape(4 * HB, D)
        st_[slot, pl.ds(dst0, 4 * HB), :] = w
        return functools.reduce(jnp.maximum, [w[k * 8:(k + 1) * 8] for k in range(4)])

    def extract_piece(st_, wb, slot, head, m0):
        ws = [st_[slot, pl.ds(head + hh + m0 * HB, 8, stride=HB), :] for hh in range(HP)]
        wb[m0:m0 + 8, :] = jnp.concatenate(ws, axis=1).astype(bf16)
        return ws[0]

    def queue_stage():
        nslot = (step // SPB + 1) % 2
        qtr = step % SPB
        for (wh, wl, wz, st_, wb, rows, sem) in wsets:
            nr = rows // SPB
            for m0 in range(0, nr, 4):
                side.append((12, P(stage_piece, wl, st_, nslot, pl.multiple_of((qtr * nr + m0) * HB, 8), m0)))

    def queue_extract():
        nstep = step + 1
        for (wh, wl, wz, st_, wb, rows, sem) in wsets:
            for m0 in range(0, rows, 8):
                side.append((8, P(extract_piece, st_, wb, (nstep // SPB) % 2, (nstep % SPB) * HP, m0)))

    units = [(u // 2, u % 2) for u in range(NU)]

    queue_u()
    pq(0, 0); pk(0, 0); pq(0, 1); pk(0, 1)
    qk(0, 0)
    pvv(0, 0); pvv(0, 1)
    fwdh(0); fwdh(1)
    odone = 0
    ND = CFG.get("normdefer", 1)
    for s in range(NU):
        i, hh = units[s]
        if s == FW:
            flush()
            fwdu(0); fwdu(1)
            for cp in early_copies(step + 1): cp.start()
            for cp in late_copies(): cp.wait()

            @pl.when(step == 0)
            def _():
                for cp in part_copies(1): cp.wait()
            for r in range(0, GR, 8):
                side.append((32, P(gate_piece, r)))
            queue_mac()
            queue_stage()
        if s == NU - 2:
            flush()
            queue_extract()
        if i + 1 < NB:
            pk(i + 1, hh); pq(i + 1, hh); pvv(i + 1, hh)
            if s >= 1 and "left" in st[units[s - 1]]:
                assert len(side) <= max(st[units[s - 1]]["left"], 0) or s == FW, (s, len(side))
        if s >= FW and odone < i and s < NU - 2:
            oproj(odone); odone += 1
        if s == NU - 2:
            oproj(NB - 2, (0, 1))
        if s == NU - 1:
            oproj(NB - 2, (2, 3))
        pv(i, hh, ND and s + 1 < NU - 2 and s + 1 != FW)
        if s + 1 < NU:
            qk(*units[s + 1])
    inv(0); inv(1)
    assert odone == NB - 2
    oproj(NB - 1)
    flush()

    @pl.when(step == NSTEP - 1)
    def _():
        RC = 128

        def fin(i, c):
            rs = pl.ds(pl.multiple_of(i * RC, RC), RC)
            g = jax.nn.sigmoid(jnp.sum(gate_s[rs, :], axis=1, keepdims=True))
            out_v[rs, :] = (g * acc[rs, :] + (1.0 - g) * (x_v[rs, :].astype(f32) * b_s[rs, :])).astype(bf16)
            pltpu.make_async_copy(out_v.at[rs, :], o_h.at[rs, :], sems.at[SEM_OUT]).start()
            return c
        jax.lax.fori_loop(0, S // RC, fin, 0)
        for cp in early_copies(step + 1): cp.wait()
        pltpu.make_async_copy(out_v, o_h, sems.at[SEM_OUT]).wait()


@jax.jit
def pallas_gated_mix__compressed_kv_cla__ssm_conv_h3__prompt_kernel(A_x, A_c_kv, A_w_q, A_w_uk, A_w_uv, A_w_o, B_q, B_k, B_v, B_shift_k, B_ssm_k, B_ssm_D, gate_w):
    x = A_x.reshape(S, M)
    c = A_c_kv.reshape(S, DC)
    wo = A_w_o.reshape(H * D, M)
    k = B_k.reshape(S, M)
    v = B_v.reshape(S, M)
    Fc, Gc = _dft_consts()
    Fc = jnp.asarray(Fc, bf16); Gc = jnp.asarray(Gc, bf16)
    hbm = pl.BlockSpec(memory_space=pl.ANY)
    vm = pl.BlockSpec(memory_space=pltpu.VMEM)
    scratch = [
        pltpu.VMEM((4, M), bf16), pltpu.VMEM((M,), bf16), pltpu.VMEM((M,), bf16),
        pltpu.VMEM((2, 128, C), bf16), pltpu.VMEM((2, C, 128), bf16),
        pltpu.VMEM((S, M), bf16),
        pltpu.VMEM((S, DC), bf16),
        pltpu.VMEM((M // SPB, HB, D), bf16),
        pltpu.VMEM((DC // SPB, HB, D), bf16),
        pltpu.VMEM((DC // SPB, HB, D), bf16),
        pltpu.VMEM((M, HB, D), bf16),
        pltpu.VMEM((DC, HB, D), bf16),
        pltpu.VMEM((DC, HB, D), bf16),
        pltpu.VMEM((2, M * HB, D), f32),
        pltpu.VMEM((2, DC * HB, D), f32),
        pltpu.VMEM((2, DC * HB, D), f32),
        pltpu.VMEM((M, HP * D), bf16),
        pltpu.VMEM((DC, HP * D), bf16),
        pltpu.VMEM((DC, HP * D), bf16),
        pltpu.VMEM((HP * D, M), bf16),
        pltpu.VMEM((S, 128), bf16),
        pltpu.VMEM((S, 128), bf16),
        pltpu.VMEM((128, S), bf16),
        pltpu.VMEM((S, M), f32),
        pltpu.VMEM((S, M), f32),
        pltpu.VMEM((S, M), bf16),
        pltpu.VMEM((S, HP * D), bf16),
        pltpu.VMEM((S, HP * D), bf16),
        pltpu.VMEM((S, HP * D), bf16),
        pltpu.VMEM((NB, BQ, HP * D), bf16),
        pltpu.VMEM((S, 128), f32),
        pltpu.VMEM((8, M), f32),
        pltpu.VMEM((C, NCH * 128), bf16),
        pltpu.VMEM((3, NCH, 64, 128), f32),
        pltpu.VMEM((3, NCH, 64, 128), f32),
        pltpu.VMEM((128, NCH * 128), bf16 if CFG.get('wbf', 1) else f32),
        pltpu.VMEM((BQ + 8, S), f32),
        pltpu.VMEM((BQ + 8, S), f32),
        pltpu.SemaphoreType.DMA((NSEM,)),
    ]
    out = pl.pallas_call(
        _kernel,
        out_shape=jax.ShapeDtypeStruct((S, M), bf16),
        grid=(NSTEP,),
        in_specs=[hbm] * 14,
        out_specs=hbm,
        scratch_shapes=scratch,
        compiler_params=pltpu.CompilerParams(vmem_limit_bytes=120 * 1024 * 1024, dimension_semantics=("arbitrary",),
                                             disable_bounds_checks=True),
    )(x, c, A_w_q, A_w_uk, A_w_uv, wo, k, v, B_ssm_k, B_shift_k.T, B_ssm_D, gate_w, Fc, Gc)
    return out.reshape(1, S, M)
```

```python
import collections
import functools
import numpy as np
import jax
import jax.numpy as jnp
import jax.experimental.pallas as pl
import jax.experimental.pallas.tpu as pltpu

f32, bf16 = jnp.float32, jnp.bfloat16
NT = (((1,), (1,)), ((), ()))

S = 2048
M = 1024
DC = 512
H = 32
D = 128
HP = 2
NSTEP = H // HP
BQ = 256
NB = S // BQ
NU = 2 * NB
C = 128
NCH = S // C
HB = 8
SPB = HB // HP
NBLK = H // HB
GR = S // NSTEP
WR = M + 2 * DC
LOG2E = 1.4426950408889634

CFG = {}
KC = CFG.get("kc", 4)
RATE = CFG.get("rate", 2.0)
MACW = CFG.get("macw", 2.25)
FW = CFG.get("fw", 4)
NP0 = (FW - 1) // 2 + 2

SEM_WQ, SEM_WK, SEM_WV, SEM_WO, SEM_KT, SEM_VT, SEM_HT = range(7)
SEM_W0 = 7
SEM_C = 10
SEM_X = 12
SEM_OUT = 14
SEM_SM = 15
NSEM = 20


def _dft_consts():
    n = np.arange(C)
    Fs, Gs = [], []
    for p in range(2):
        ks = np.arange(p * 64, (p + 1) * 64)
        ks = np.concatenate([ks[ks % 2 == 0], ks[ks % 2 == 1]])
        th = np.pi * (2 * ks[:, None] + 1) * n[None, :] / (2 * C)
        F = np.stack([np.cos(th).reshape(8, 8, C), -np.sin(th).reshape(8, 8, C)], axis=1).reshape(128, C)
        Fs.append(F); Gs.append(F.T / C)
    return np.stack(Fs).astype(np.float32), np.stack(Gs).astype(np.float32)


def _kernel(x_h, c_h, wq_h, wk_h, wv_h, wo_h, k_h, v_h, h_h,
            skt_h, dd_h, gw_h, f_h, g_h,
            o_h,
            skt_ref, dd_ref, gw_ref, f_ref, g_ref,
            x_v, c_v, w_l, w_0, w_st, wq_b, wk_b, wv_b, wo_l,
            kv_l, ht_l, acc, b_s, out_v, q_s, k_s, v_s, ctx_s, gate_s, par_s, ub_s,
            V_s, H_s, W_s, s_a, s_b, sems):
    s_s = (s_a, s_b)
    kt_l, vt_l = kv_l.at[0], kv_l.at[1]
    step = pl.program_id(0)
    P = functools.partial
    wsets = ((wq_h, wq_b, M, 0), (wk_h, wk_b, DC, M), (wv_h, wv_b, DC, M + DC))

    def pair_copies(n, land, sem):
        h0 = pl.multiple_of(n * HP, HP)
        return [pltpu.make_async_copy(wh.at[:, j, pl.ds(h0, HP), :],
                                      land.at[off // 4:(off + rows) // 4, HP * j:HP * (j + 1), :], sems.at[sem])
                for (wh, wb, rows, off) in wsets for j in range(4)]

    def late_copies(n):
        return ([pltpu.make_async_copy(wo_h.at[pl.ds(pl.multiple_of(n * 256, 256), 256), :], wo_l, sems.at[SEM_WO])]
                + pair_copies(jnp.minimum(n + 1, NSTEP - 1), w_l, SEM_WQ))

    def late_wait():
        pltpu.make_async_copy(wo_l, wo_l, sems.at[SEM_WO]).wait()
        pltpu.make_async_copy(w_l, w_l, sems.at[SEM_WQ]).wait()

    def early_copies(n):
        col = pl.multiple_of((jnp.minimum(n, NSTEP - 1) // 2) * 128, 128)
        return [pltpu.make_async_copy(k_h.at[:, pl.ds(col, 128)], kt_l, sems.at[SEM_KT]),
                pltpu.make_async_copy(v_h.at[:, pl.ds(col, 128)], vt_l, sems.at[SEM_KT]),
                pltpu.make_async_copy(h_h.at[pl.ds(col, 128), :], ht_l, sems.at[SEM_HT])]

    def early_wait():
        pltpu.make_async_copy(kv_l, kv_l, sems.at[SEM_KT]).wait()
        pltpu.make_async_copy(ht_l, ht_l, sems.at[SEM_HT]).wait()

    def part_copies(p):
        a, b = (0, NP0 * BQ) if p == 0 else (NP0 * BQ, S)
        return [pltpu.make_async_copy(c_h.at[a:b, :], c_v.at[a:b, :], sems.at[SEM_C + p]),
                pltpu.make_async_copy(x_h.at[a:b, :], x_v.at[a:b, :], sems.at[SEM_X + p])]

    @pl.when(step == 0)
    def _():
        w0 = pair_copies(step, w_0, SEM_W0)
        sm = [pltpu.make_async_copy(a, b, sems.at[SEM_SM + n]) for n, (a, b) in enumerate(
            ((skt_h, skt_ref), (dd_h, dd_ref), (gw_h, gw_ref), (f_h, f_ref), (g_h, g_ref)))]
        P1 = CFG.get('p1', 0)
        for cp in w0 + sm + part_copies(0) + early_copies(step) + (part_copies(1) if P1 == 0 else []) + late_copies(step): cp.start()

        def zero(i, c):
            rs = pl.ds(pl.multiple_of(i * 64, 64), 64)
            acc[rs, :] = jnp.zeros((64, M), f32)
            b_s[rs, :] = jnp.zeros((64, M), f32)
            return c
        jax.lax.fori_loop(0, S // 64, zero, 0)
        for cp in sm: cp.wait()
        par_s[0:4, :] = skt_ref[...].astype(f32)
        par_s[4:5, :] = 0.5 * dd_ref[...].astype(f32).reshape(1, M)
        par_s[5:6, :] = gw_ref[...].astype(f32).reshape(1, M)
        par_s[6:8, :] = jnp.zeros((2, M), f32)
        pltpu.make_async_copy(w_0, w_0, sems.at[SEM_W0]).wait()
        w_st[0:2 * WR, :] = w_0[...].astype(f32).reshape(2 * WR, D)
        for (wh, wb, rows, off) in wsets:
            wb[...] = jnp.concatenate([w_st[pl.ds(2 * off + hh, rows, stride=2), :] for hh in range(HP)], axis=1).astype(bf16)
        if P1 == 4:
            for cp in part_copies(1): cp.start()
        for cp in part_copies(0): cp.wait()
        if P1 == 5:
            for cp in part_copies(1): cp.start()

    early_wait()

    ct = step // 2
    half = step % 2
    ccol = pl.ds(pl.multiple_of(ct * 128, 128), 128)
    scale = (D ** -0.5) * LOG2E
    row = jax.lax.broadcasted_iota(jnp.int32, (128, 128), 0)
    col = jax.lax.broadcasted_iota(jnp.int32, (128, 128), 1)
    mask = col <= row
    never8 = f_ref[0, 0:8, :].astype(f32) > 2.0
    never = jnp.concatenate([never8] * 16, axis=0)

    side = collections.deque()
    budget = [0.0]

    def pin(arr, spacing):
        R = arr.shape[0]
        out, lastr = [], 0
        for g in range(R // 8):
            budget[0] = min(budget[0] + RATE * spacing, 80.0)
            if side and budget[0] >= side[0][0]:
                cost, fn = side.popleft()
                budget[0] -= cost
                v = fn()
                if g * 8 > lastr:
                    out.append(arr[lastr:g * 8])
                out.append(jnp.where(never8, v, arr[g * 8:(g + 1) * 8]))
                lastr = (g + 1) * 8
        if lastr == 0:
            return arr
        if lastr < R:
            out.append(arr[lastr:])
        return jnp.concatenate(out, axis=0)

    def flush():
        if side and CFG.get("dbg"): print("flush leftover", len(side))
        while side:
            side.popleft()[1]()

    def pq(i, hh):
        r0 = i * BQ; r1 = r0 + BQ
        hs = slice(hh * D, (hh + 1) * D)
        r = jnp.dot(x_v[r0:r1, :], wq_b[:, hs], preferred_element_type=f32)
        q_s[r0:r1, hs] = (pin(r, 8) * scale).astype(bf16)

    def pk(i, hh):
        r0 = i * BQ; r1 = r0 + BQ
        hs = slice(hh * D, (hh + 1) * D)
        r = jnp.dot(c_v[r0:r1, :], wk_b[:, hs], preferred_element_type=f32)
        k_s[r0:r1, hs] = pin(r, 8).astype(bf16)

    def pvv(i, hh):
        r0 = i * BQ; r1 = r0 + BQ
        hs = slice(hh * D, (hh + 1) * D)
        r = jnp.dot(c_v[r0:r1, :], wv_b[:, hs], preferred_element_type=f32)
        v_s[r0:r1, hs] = pin(r, 8).astype(bf16)

    def chunks(i):
        nt = 2 * i + 1
        out, t = [], 0
        while t < nt:
            n = min(KC, nt - t)
            out.append((0, t * 128, (t + n) * 128))
            t += n
        out.append((128, nt * 128, (nt + 1) * 128))
        return out

    st = {}

    def qk_atom(i, hh, ch):
        rl, kl, kh = ch
        r0 = i * BQ
        hs = slice(hh * D, (hh + 1) * D)
        s = jax.lax.dot_general(q_s[r0 + rl:r0 + BQ, hs], k_s[kl:kh, hs], NT, preferred_element_type=f32)
        nt = (kh - kl) // 128
        tiles = [s[:, t * 128:(t + 1) * 128] for t in range(nt)]
        if kh > r0 + rl:
            d = tiles[-1]
            dm = jnp.where(mask, d[:128], -1e30)
            tiles[-1] = dm if rl == 128 else jnp.concatenate([dm, d[128:]], axis=0)
        u = st.setdefault((i, hh), {"m": [None, None], "l": [None, None], "o": [None, None]})
        u[("s", ch)] = tiles
        if CFG.get("smem", 1):
            for t in range(nt):
                s_s[hh][rl:BQ, kl + t * 128:kl + (t + 1) * 128] = tiles[t]
        mm = functools.reduce(jnp.maximum, tiles)
        for g in range(rl // 128, 2):
            a = mm[g * 128 - rl:(g + 1) * 128 - rl]
            u["m"][g] = a if u["m"][g] is None else jnp.maximum(u["m"][g], a)

    def qk(i, hh, sel=None):
        chs = chunks(i)
        if sel == "head":
            for ch in chs[:-2]: qk_atom(i, hh, ch)
            return
        for ch in (chs[-2:] if sel == "tail" else chs): qk_atom(i, hh, ch)
        u = st[(i, hh)]
        u["M"] = [jnp.broadcast_to(jnp.max(u["m"][g], axis=1, keepdims=True), (128, 128)) for g in range(2)]
        if CFG.get("smem", 1):
            if CFG.get("mmem", 1):
                s_s[hh][0:BQ, S:S + 128] = jnp.concatenate(u["M"], axis=0)
            s_s[hh][pl.ds(pl.multiple_of(BQ + (step >> 8) * 8, 8), 8), 0:128] = u["m"][1][120:128]
            if CFG.get("mmem", 1):
                s_s[hh][pl.ds(pl.multiple_of(BQ + (step >> 8) * 8, 8), 8), S:S + 128] = u["m"][1][120:128]

    def pv_atom(i, hh, ch):
        rl, kl, kh = ch
        hs = slice(hh * D, (hh + 1) * D)
        u = st[(i, hh)]
        m = u["M"][1] if rl == 128 else jnp.concatenate(u["M"], axis=0)
        if CFG.get("mmem", 1):
            m = s_s[hh][rl:BQ, S:S + 128]
        if CFG.get("smem", 1):
            ps = [jnp.exp2(s_s[hh][rl:BQ, k0:k0 + 128] - m) for k0 in range(kl, kh, 128)]
        else:
            ps = [jnp.exp2(t - m) for t in u[("s", ch)]]
        lp = functools.reduce(jnp.add, ps)
        ls = []
        for g in range(rl // 128, 2):
            a = lp[g * 128 - rl:(g + 1) * 128 - rl]
            u["l"][g] = a if u["l"][g] is None else u["l"][g] + a
            ls.append(u["l"][g])
        ps[-1] = jnp.minimum(ps[-1], jnp.concatenate(ls, axis=0) if len(ls) > 1 else ls[0])
        pb = (jnp.concatenate(ps, axis=1) if len(ps) > 1 else ps[0]).astype(bf16)
        o = jnp.dot(pb, v_s[kl:kh, hs], preferred_element_type=f32)
        for g in range(rl // 128, 2):
            a = o[g * 128 - rl:(g + 1) * 128 - rl]
            u["o"][g] = a if u["o"][g] is None else u["o"][g] + a

    def recip(l):
        if CFG.get("exactdiv"):
            return 1.0 / l
        r = pl.reciprocal(l, approx=True)
        return r * (2.0 - l * r)

    def norm_piece(i, hh, g, r):
        u = st[(i, hh)]
        hs = slice(hh * D, (hh + 1) * D)
        o = u["o"][g][r:r + 16]
        c = o * recip(u["L"][g][r:r + 16])
        ctx_s[i, g * 128 + r:g * 128 + r + 16, hs] = c.astype(bf16)
        return jnp.maximum(c[:8], c[8:])

    def pv(i, hh, defer):
        for ch in chunks(i): pv_atom(i, hh, ch)
        u = st[(i, hh)]
        u["L"] = [jnp.sum(jnp.where(never, u["o"][g], u["l"][g]), axis=1, keepdims=True) for g in range(2)]
        pieces = [(CFG.get("normc", 32), P(norm_piece, i, hh, g, r)) for g in range(2) for r in range(0, 128, 16)]
        if defer:
            side.extendleft(reversed(pieces))
            u["left"] = len(side) - len(pieces)
        else:
            for _, fn in pieces: fn()

    def oproj(i, atoms=range(4), fine=0):
        r0 = i * BQ; r1 = r0 + BQ
        for a in atoms:
            cs = slice(a * 256, (a + 1) * 256)
            nsp = CFG.get("nsp", 4) if (fine and a >= 4 - fine) else 1
            for p in range(nsp):
                ra, rb = p * BQ // nsp, (p + 1) * BQ // nsp
                r = jnp.dot(ctx_s[i, ra:rb], wo_l[:, cs], preferred_element_type=f32)
                r = jnp.concatenate([pin(r[:, :128], 8), r[:, 128:]], axis=1)
                acc[r0 + ra:r0 + rb, cs] += r

    cv = {}

    UR = CFG.get("ur", 16)

    def u_piece(r):
        j = r // C
        par = cv["par"]
        if r == 0:
            kf = jnp.concatenate([jnp.zeros((8, 128), f32), kt_l[0:UR, :].astype(f32)], axis=0)
        else:
            kf = kt_l[r - 16:r + UR, :].astype(f32)[8:]
        ks = kf[8:] * par[0:1]
        for t in range(1, 4):
            ks = ks + kf[8 - t:8 - t + UR] * par[t:t + 1]
        u = ks * vt_l[r:r + UR, :].astype(f32)
        ub_s[r - j * C:r - j * C + UR, j * 128:(j + 1) * 128] = u.astype(bf16)
        b_s[r:r + UR, ccol] += u * par[4:5]
        return functools.reduce(jnp.maximum, [u[k:k + 8] for k in range(0, UR, 8)])

    def queue_u():
        cv["par"] = par_s[:, ccol]
        for r in range(0, S, UR):
            side.append((CFG.get("uc", 2.5) * UR, P(u_piece, r)))

    def split(T, j):
        t = T[:, j * 128:(j + 1) * 128]
        re = jnp.concatenate([t[16 * g:16 * g + 8] for g in range(8)], axis=0)
        im = jnp.concatenate([t[16 * g + 8:16 * g + 16] for g in range(8)], axis=0)
        return re, im

    def fwdu(hf):
        lo, hi = hf * NCH // 2, (hf + 1) * NCH // 2
        U = jnp.dot(f_ref[half], ub_s[:, lo * 128:hi * 128], preferred_element_type=f32)
        for j in range(lo, hi):
            re, im = split(U, j - lo)
            V_s[0, j] = re
            V_s[1, j] = im
            V_s[2, j] = re + im

    def fwdh(hf):
        lo, hi = hf * NCH // 2, (hf + 1) * NCH // 2
        hcat = jnp.concatenate([ht_l[:, j * C:(j + 1) * C] for j in range(lo, hi)], axis=0)
        Hf = jax.lax.dot_general(f_ref[half], hcat, NT, preferred_element_type=f32)
        for j in range(lo, hi):
            re, im = split(Hf, j - lo)
            H_s[0, j] = im - re
            H_s[1, j] = re + im
            H_s[2, j] = re

    def mac_piece(i, r, a):
        rs = slice(r, r + 8)
        s = functools.reduce(jnp.add, [H_s[a, i - j, rs, :] * V_s[a, j, rs, :] for j in range(i + 1)])
        cv[a] = s
        if a == 2:
            yr, yi = s - cv[1], s + cv[0]
            wr, wi = yr, yi
            if i > 0:
                pr, pi = cv[("y", r)]
                wr, wi = (yr - pi, yi + pr) if r < 32 else (yr + pi, yi - pr)
            cv[("y", r)] = (yr, yi)
            W_s[2 * r:2 * r + 16, i * 128:(i + 1) * 128] = jnp.concatenate([wr, wi], axis=0).astype(W_s.dtype)
        return s

    def queue_mac():
        for i2 in range(NCH):
            for r in range(0, 64, 8):
                for a in range(3):
                    side.append((MACW * (2 * (i2 + 1) + 3), P(mac_piece, i2, r, a)))

    def inv(hf):
        lo, hi = hf * NCH // 2, (hf + 1) * NCH // 2
        Y = jnp.dot(g_ref[half], W_s[:, lo * 128:hi * 128].astype(bf16), preferred_element_type=f32)
        for j in range(lo, hi):
            a, b = j * C, (j + 1) * C
            y = Y[:, (j - lo) * 128:(j - lo + 1) * 128]
            b_s[a:b, ccol] += y

    def gate_piece(r):
        rs = pl.ds(pl.multiple_of(step * GR + r, 8), 8)
        xs = x_v[rs, :].astype(f32) * par_s[5:6, :]
        z = functools.reduce(jnp.add, [xs[:, t * 128:(t + 1) * 128] for t in range(M // 128)])
        gate_s[rs, :] = z
        return z

    def stage_piece(t0):
        w = w_l[t0:t0 + 4].astype(f32).reshape(32, D)
        w_st[t0 * 8:t0 * 8 + 32, :] = w
        return functools.reduce(jnp.maximum, [w[k * 8:(k + 1) * 8] for k in range(4)])

    def extract_piece(wb, off, m0):
        ws = [w_st[pl.ds(2 * (off + m0) + hh, 8, stride=2), :] for hh in range(HP)]
        wb[m0:m0 + 8, :] = jnp.concatenate(ws, axis=1).astype(bf16)
        return ws[0]

    def queue_stage():
        for t0 in range(0, WR // 4, 4):
            side.append((12, P(stage_piece, t0)))

    def queue_extract():
        for (wh, wb, rows, off) in wsets:
            for m0 in range(0, rows, 8):
                side.append((8, P(extract_piece, wb, off, m0)))

    units = [(u // 2, u % 2) for u in range(NU)]

    queue_u()
    pq(0, 0); pk(0, 0); pq(0, 1); pk(0, 1)
    qk(0, 0)
    pvv(0, 0); pvv(0, 1)
    fwdh(0); fwdh(1)
    odone = 0
    ND = CFG.get("normdefer", 1)
    for s in range(NU):
        i, hh = units[s]
        if s == FW:
            flush()
            fwdu(0); fwdu(1)
            for cp in early_copies(step + 1): cp.start()
            late_wait()

            @pl.when(step == 0)
            def _():
                for cp in part_copies(1): cp.wait()
            if CFG.get("bal", 1): qk(i, hh, "tail")
            for r in range(0, GR, 8):
                side.append((32, P(gate_piece, r)))
            queue_mac()
            queue_stage()
        if s == NU - 2:
            flush()
            queue_extract()
        if i + 1 < NB:
            pk(i + 1, hh); pq(i + 1, hh); pvv(i + 1, hh)
            if s >= 1 and "left" in st[units[s - 1]]:
                assert len(side) <= max(st[units[s - 1]]["left"], 0) or s == FW, (s, len(side))
        if s >= FW and odone < i and s < NU - 2:
            oproj(odone); odone += 1
        if s == NU - 2:
            oproj(NB - 2, (0, 1))
        if s == NU - 1:
            oproj(NB - 2, (2, 3))
        pv(i, hh, ND and s + 1 < NU - 2 and s + 1 != FW)
        if s + 1 < NU:
            qk(*units[s + 1], "head" if (s + 1 == FW and CFG.get("bal", 1)) else None)
    inv(0); inv(1)
    assert odone == NB - 2
    oproj(NB - 1, fine=CFG.get('fine', 0))
    flush()

    @pl.when(step < pl.num_programs(0) - 1)
    def _():
        for cp in late_copies(step + 1): cp.start()

    @pl.when(step == NSTEP - 1)
    def _():
        RC = 128

        def fin(i, c):
            rs = pl.ds(pl.multiple_of(i * RC, RC), RC)
            g = jax.nn.sigmoid(jnp.sum(gate_s[rs, :], axis=1, keepdims=True))
            out_v[rs, :] = (g * acc[rs, :] + (1.0 - g) * (x_v[rs, :].astype(f32) * b_s[rs, :])).astype(bf16)
            pltpu.make_async_copy(out_v.at[rs, :], o_h.at[rs, :], sems.at[SEM_OUT]).start()
            return c
        jax.lax.fori_loop(0, S // RC, fin, 0)
        early_wait()
        pltpu.make_async_copy(out_v, o_h, sems.at[SEM_OUT]).wait()


@jax.jit
def pallas_gated_mix__compressed_kv_cla__ssm_conv_h3__prompt_kernel(A_x, A_c_kv, A_w_q, A_w_uk, A_w_uv, A_w_o, B_q, B_k, B_v, B_shift_k, B_ssm_k, B_ssm_D, gate_w):
    x = A_x.reshape(S, M)
    c = A_c_kv.reshape(S, DC)
    wo = A_w_o.reshape(H * D, M)
    k = B_k.reshape(S, M)
    v = B_v.reshape(S, M)
    Fc, Gc = _dft_consts()
    Fc = jnp.asarray(Fc, bf16); Gc = jnp.asarray(Gc, bf16)
    hbm = pl.BlockSpec(memory_space=pl.ANY)
    vm = pl.BlockSpec(memory_space=pltpu.VMEM)
    scratch = [
        pltpu.VMEM((4, M), bf16), pltpu.VMEM((M,), bf16), pltpu.VMEM((M,), bf16),
        pltpu.VMEM((2, 128, C), bf16), pltpu.VMEM((2, C, 128), bf16),
        pltpu.VMEM((S, M), bf16),
        pltpu.VMEM((S, DC), bf16),
        pltpu.VMEM((WR // 4, 8, D), bf16),
        pltpu.VMEM((WR // 4, 8, D), bf16),
        pltpu.VMEM((2 * WR + 8, D), f32),
        pltpu.VMEM((M, HP * D), bf16),
        pltpu.VMEM((DC, HP * D), bf16),
        pltpu.VMEM((DC, HP * D), bf16),
        pltpu.VMEM((HP * D, M), bf16),
        pltpu.VMEM((2, S, 128), bf16),
        pltpu.VMEM((128, S), bf16),
        pltpu.VMEM((S, M), f32),
        pltpu.VMEM((S, M), f32),
        pltpu.VMEM((S, M), bf16),
        pltpu.VMEM((S, HP * D), bf16),
        pltpu.VMEM((S, HP * D), bf16),
        pltpu.VMEM((S, HP * D), bf16),
        pltpu.VMEM((NB, BQ, HP * D), bf16),
        pltpu.VMEM((S, 128), f32),
        pltpu.VMEM((8, M), f32),
        pltpu.VMEM((C, NCH * 128), bf16),
        pltpu.VMEM((3, NCH, 64, 128), f32),
        pltpu.VMEM((3, NCH, 64, 128), f32),
        pltpu.VMEM((128, NCH * 128), bf16 if CFG.get('wbf', 1) else f32),
        pltpu.VMEM((BQ + 8, S + 128), f32),
        pltpu.VMEM((BQ + 8, S + 128), f32),
        pltpu.SemaphoreType.DMA((NSEM,)),
    ]
    out = pl.pallas_call(
        _kernel,
        out_shape=jax.ShapeDtypeStruct((S, M), bf16),
        grid=(NSTEP,),
        in_specs=[hbm] * 14,
        out_specs=hbm,
        scratch_shapes=scratch,
        compiler_params=pltpu.CompilerParams(vmem_limit_bytes=120 * 1024 * 1024, dimension_semantics=("arbitrary",),
                                             disable_bounds_checks=True),
    )(x, c, A_w_q.reshape(M // 4, 4, H, D), A_w_uk.reshape(DC // 4, 4, H, D), A_w_uv.reshape(DC // 4, 4, H, D), wo, k, v, B_ssm_k, B_shift_k.T, B_ssm_D, gate_w, Fc, Gc)
    return out.reshape(1, S, M)
```

```python
import collections
import functools
import numpy as np
import jax
import jax.numpy as jnp
import jax.experimental.pallas as pl
import jax.experimental.pallas.tpu as pltpu

f32, bf16 = jnp.float32, jnp.bfloat16
NT = (((1,), (1,)), ((), ()))

S = 2048
M = 1024
DC = 512
H = 32
D = 128
HP = 2
NSTEP = H // HP
BQ = 256
NB = S // BQ
NU = 2 * NB
C = 128
NCH = S // C
HB = 8
SPB = HB // HP
NBLK = H // HB
GR = S // NSTEP
WR = M + 2 * DC
LOG2E = 1.4426950408889634

CFG = {}
KC = CFG.get("kc", 4)
RATE = CFG.get("rate", 2.0)
MACW = CFG.get("macw", 2.0)
FW = CFG.get("fw", 4)
NP0 = (FW - 1) // 2 + 2

SEM_WQ, SEM_WK, SEM_WV, SEM_WO, SEM_KT, SEM_VT, SEM_HT = range(7)
SEM_W0 = 7
SEM_C = 10
SEM_OUT = 12
SEM_SM = 13
SEM_X = 18
NSEM = 26


def _dft_consts():
    n = np.arange(C)
    Fs, Gs = [], []
    for p in range(2):
        ks = np.arange(p * 64, (p + 1) * 64)
        ks = np.concatenate([ks[ks % 2 == 0], ks[ks % 2 == 1]])
        th = np.pi * (2 * ks[:, None] + 1) * n[None, :] / (2 * C)
        F = np.stack([np.cos(th).reshape(8, 8, C), -np.sin(th).reshape(8, 8, C)], axis=1).reshape(128, C)
        Fs.append(F); Gs.append(F.T / C)
    return np.stack(Fs).astype(np.float32), np.stack(Gs).astype(np.float32)


def _kernel(x_h, c_h, wq_h, wk_h, wv_h, wo_h, k_h, v_h, h_h,
            skt_h, dd_h, gw_h, f_h, g_h,
            o_h,
            skt_ref, dd_ref, gw_ref, f_ref, g_ref,
            x_v, c_v, w_l, w_0, w_st, wq_b, wk_b, wv_b, wo_l,
            kv_l, ht_l, acc, u_s, xg_s, out_v, q_s, k_s, v_s, ctx_s, gate_s, par_s, ub_s,
            V_s, H_s, W_s, s_a, s_b, sems):
    s_s = (s_a, s_b)
    kt_l, vt_l = kv_l.at[0], kv_l.at[1]
    step = pl.program_id(0)
    P = functools.partial
    wsets = ((wq_h, wq_b, M, 0), (wk_h, wk_b, DC, M), (wv_h, wv_b, DC, M + DC))

    def pair_copies(n, land, sem):
        h0 = pl.multiple_of(n * HP, HP)
        return [pltpu.make_async_copy(wh.at[:, j, pl.ds(h0, HP), :],
                                      land.at[off // 4:(off + rows) // 4, HP * j:HP * (j + 1), :], sems.at[sem])
                for (wh, wb, rows, off) in wsets for j in range(4)]

    def late_copies(n):
        return ([pltpu.make_async_copy(wo_h.at[pl.ds(pl.multiple_of(n * 256, 256), 256), :], wo_l, sems.at[SEM_WO])]
                + pair_copies(jnp.minimum(n + 1, NSTEP - 1), w_l, SEM_WQ))

    def late_wait():
        pltpu.make_async_copy(wo_l, wo_l, sems.at[SEM_WO]).wait()
        pltpu.make_async_copy(w_l, w_l, sems.at[SEM_WQ]).wait()

    def early_copies(n):
        col = pl.multiple_of((jnp.minimum(n, NSTEP - 1) // 2) * 128, 128)
        return [pltpu.make_async_copy(k_h.at[:, pl.ds(col, 128)], kt_l, sems.at[SEM_KT]),
                pltpu.make_async_copy(v_h.at[:, pl.ds(col, 128)], vt_l, sems.at[SEM_KT]),
                pltpu.make_async_copy(h_h.at[pl.ds(col, 128), :], ht_l, sems.at[SEM_HT])]

    def early_wait():
        pltpu.make_async_copy(kv_l, kv_l, sems.at[SEM_KT]).wait()
        pltpu.make_async_copy(ht_l, ht_l, sems.at[SEM_HT]).wait()

    def c_copy(p):
        a, b = (0, NP0 * BQ) if p == 0 else (NP0 * BQ, S)
        return pltpu.make_async_copy(c_h.at[a:b, :], c_v.at[a:b, :], sems.at[SEM_C + p])

    def x_copy(i):
        rs = pl.ds(i * BQ, BQ) if isinstance(i, int) else pl.ds(pl.multiple_of(i * BQ, BQ), BQ)
        return pltpu.make_async_copy(x_h.at[rs, :], x_v.at[rs, :], sems.at[SEM_X + i])

    def gate_blocks(lo, hi):
        def f(i, c):
            x_copy(i).wait()
            rs = pl.ds(pl.multiple_of(i * BQ, BQ), BQ)
            z = jnp.sum(x_v[rs, :].astype(f32) * par_s[5:6, :], axis=1, keepdims=True)
            gate_s[rs, :] = jnp.broadcast_to(jax.nn.sigmoid(z), (BQ, 128))
            return c
        jax.lax.fori_loop(lo, hi, f, 0)

    @pl.when(step == 0)
    def _():
        w0 = pair_copies(step, w_0, SEM_W0)
        sm = [pltpu.make_async_copy(a, b, sems.at[SEM_SM + n]) for n, (a, b) in enumerate(
            ((skt_h, skt_ref), (dd_h, dd_ref), (gw_h, gw_ref), (f_h, f_ref), (g_h, g_ref)))]
        for cp in (w0 + sm + [x_copy(i) for i in range(NP0)] + [c_copy(0)] + early_copies(step)
                   + [x_copy(i) for i in range(NP0, NB)] + [c_copy(1)] + late_copies(step)):
            cp.start()

        def zero(i, c):
            rs = pl.ds(pl.multiple_of(i * 64, 64), 64)
            acc[rs, :] = jnp.zeros((64, M), f32)
            return c
        jax.lax.fori_loop(0, S // 64, zero, 0)
        for cp in sm: cp.wait()
        par_s[0:4, :] = skt_ref[...].astype(f32)
        par_s[4:5, :] = 0.5 * dd_ref[...].astype(f32).reshape(1, M)
        par_s[5:6, :] = gw_ref[...].astype(f32).reshape(1, M)
        par_s[6:8, :] = jnp.zeros((2, M), f32)
        pltpu.make_async_copy(w_0, w_0, sems.at[SEM_W0]).wait()
        w_st[0:2 * WR, :] = w_0[...].astype(f32).reshape(2 * WR, D)
        for (wh, wb, rows, off) in wsets:
            wb[...] = jnp.concatenate([w_st[pl.ds(2 * off + hh, rows, stride=2), :] for hh in range(HP)], axis=1).astype(bf16)
        gate_blocks(0, NP0)
        c_copy(0).wait()

    early_wait()

    ct = step // 2
    half = step % 2
    ccol = pl.ds(pl.multiple_of(ct * 128, 128), 128)
    scale = (D ** -0.5) * LOG2E
    row = jax.lax.broadcasted_iota(jnp.int32, (128, 128), 0)
    col = jax.lax.broadcasted_iota(jnp.int32, (128, 128), 1)
    mask = col <= row
    never8 = f_ref[0, 0:8, :].astype(f32) > 2.0
    never = jnp.concatenate([never8] * 16, axis=0)

    side = collections.deque()
    budget = [0.0]

    lim = [32]

    def pin(arr, spacing):
        R = arr.shape[0]
        out, lastr = [], 0
        for g in range(min(R // 8, lim[0])):
            budget[0] = min(budget[0] + RATE * spacing, 80.0)
            if side and budget[0] >= side[0][0]:
                cost, fn = side.popleft()
                budget[0] -= cost
                v = fn()
                if g * 8 > lastr:
                    out.append(arr[lastr:g * 8])
                out.append(jnp.where(never8, v, arr[g * 8:(g + 1) * 8]))
                lastr = (g + 1) * 8
        if lastr == 0:
            return arr
        if lastr < R:
            out.append(arr[lastr:])
        return jnp.concatenate(out, axis=0)

    def flush():
        if side and CFG.get("dbg"): print("flush leftover", len(side))
        while side:
            side.popleft()[1]()

    def pq(i, hh):
        r0 = i * BQ; r1 = r0 + BQ
        hs = slice(hh * D, (hh + 1) * D)
        r = jnp.dot(x_v[r0:r1, :], wq_b[:, hs], preferred_element_type=f32)
        q_s[r0:r1, hs] = (pin(r, 8) * scale).astype(bf16)

    def pk(i, hh):
        r0 = i * BQ; r1 = r0 + BQ
        hs = slice(hh * D, (hh + 1) * D)
        r = jnp.dot(c_v[r0:r1, :], wk_b[:, hs], preferred_element_type=f32)
        k_s[r0:r1, hs] = pin(r, 8).astype(bf16)

    def pvv(i, hh):
        r0 = i * BQ; r1 = r0 + BQ
        hs = slice(hh * D, (hh + 1) * D)
        r = jnp.dot(c_v[r0:r1, :], wv_b[:, hs], preferred_element_type=f32)
        v_s[r0:r1, hs] = pin(r, 8).astype(bf16)

    def chunks(i):
        nt = 2 * i + 1
        out, t = [], 0
        while t < nt:
            n = min(KC, nt - t)
            out.append((0, t * 128, (t + n) * 128))
            t += n
        out.append((128, nt * 128, (nt + 1) * 128))
        return out

    st = {}

    def qk_atom(i, hh, ch):
        rl, kl, kh = ch
        r0 = i * BQ
        hs = slice(hh * D, (hh + 1) * D)
        s = jax.lax.dot_general(q_s[r0 + rl:r0 + BQ, hs], k_s[kl:kh, hs], NT, preferred_element_type=f32)
        nt = (kh - kl) // 128
        tiles = [s[:, t * 128:(t + 1) * 128] for t in range(nt)]
        if kh > r0 + rl:
            d = tiles[-1]
            dm = jnp.where(mask, d[:128], -1e30)
            tiles[-1] = dm if rl == 128 else jnp.concatenate([dm, d[128:]], axis=0)
        u = st.setdefault((i, hh), {"m": [None, None], "l": [None, None], "o": [None, None]})
        u[("s", ch)] = tiles
        if CFG.get("smem", 1):
            for t in range(nt):
                s_s[hh][rl:BQ, kl + t * 128:kl + (t + 1) * 128] = tiles[t]
        mm = functools.reduce(jnp.maximum, tiles)
        for g in range(rl // 128, 2):
            a = mm[g * 128 - rl:(g + 1) * 128 - rl]
            u["m"][g] = a if u["m"][g] is None else jnp.maximum(u["m"][g], a)

    def qk(i, hh, sel=None):
        chs = chunks(i)
        if sel == "head":
            for ch in chs[:-2]: qk_atom(i, hh, ch)
            return
        for ch in (chs[-2:] if sel == "tail" else chs): qk_atom(i, hh, ch)
        u = st[(i, hh)]
        u["M"] = [jnp.broadcast_to(jnp.max(u["m"][g], axis=1, keepdims=True), (128, 128)) for g in range(2)]
        if CFG.get("smem", 1):
            if CFG.get("mmem", 1):
                s_s[hh][0:BQ, S:S + 128] = jnp.concatenate(u["M"], axis=0)
            s_s[hh][pl.ds(pl.multiple_of(BQ + (step >> 8) * 8, 8), 8), 0:128] = u["m"][1][120:128]
            if CFG.get("mmem", 1):
                s_s[hh][pl.ds(pl.multiple_of(BQ + (step >> 8) * 8, 8), 8), S:S + 128] = u["m"][1][120:128]

    def pv_atom(i, hh, ch):
        rl, kl, kh = ch
        hs = slice(hh * D, (hh + 1) * D)
        u = st[(i, hh)]
        m = u["M"][1] if rl == 128 else jnp.concatenate(u["M"], axis=0)
        if CFG.get("mmem", 1):
            m = s_s[hh][rl:BQ, S:S + 128]
        if CFG.get("smem", 1):
            ps = [jnp.exp2(s_s[hh][rl:BQ, k0:k0 + 128] - m) for k0 in range(kl, kh, 128)]
        else:
            ps = [jnp.exp2(t - m) for t in u[("s", ch)]]
        lp = functools.reduce(jnp.add, ps)
        ls = []
        for g in range(rl // 128, 2):
            a = lp[g * 128 - rl:(g + 1) * 128 - rl]
            u["l"][g] = a if u["l"][g] is None else u["l"][g] + a
            ls.append(u["l"][g])
        ps[-1] = jnp.minimum(ps[-1], jnp.concatenate(ls, axis=0) if len(ls) > 1 else ls[0])
        pb = (jnp.concatenate(ps, axis=1) if len(ps) > 1 else ps[0]).astype(bf16)
        o = jnp.dot(pb, v_s[kl:kh, hs], preferred_element_type=f32)
        for g in range(rl // 128, 2):
            a = o[g * 128 - rl:(g + 1) * 128 - rl]
            u["o"][g] = a if u["o"][g] is None else u["o"][g] + a

    def recip(l):
        if CFG.get("exactdiv"):
            return 1.0 / l
        r = pl.reciprocal(l, approx=True)
        return r * (2.0 - l * r)

    def norm_piece(i, hh, g, r):
        u = st[(i, hh)]
        hs = slice(hh * D, (hh + 1) * D)
        o = u["o"][g][r:r + 16]
        r0 = i * BQ + g * 128 + r
        c = o * (gate_s[r0:r0 + 16, :] * recip(u["L"][g][r:r + 16]))
        ctx_s[i, g * 128 + r:g * 128 + r + 16, hs] = c.astype(bf16)
        return jnp.maximum(c[:8], c[8:])

    def pv(i, hh, defer):
        for ch in chunks(i): pv_atom(i, hh, ch)
        u = st[(i, hh)]
        u["L"] = [jnp.sum(jnp.where(never, u["o"][g], u["l"][g]), axis=1, keepdims=True) for g in range(2)]
        pieces = [(CFG.get("normc", 32), P(norm_piece, i, hh, g, r)) for g in range(2) for r in range(0, 128, 16)]
        if defer:
            side.extendleft(reversed(pieces))
            u["left"] = len(side) - len(pieces)
        else:
            for _, fn in pieces: fn()

    zdyn = (step >> 8) * 16

    def oproj(i, atoms=range(4), fine=0, lastlim=32):
        r0 = i * BQ; r1 = r0 + BQ
        for a in atoms:
            lim[0] = lastlim if a == atoms[-1] else 32
            cs = slice(a * 256, (a + 1) * 256)
            r = jnp.dot(ctx_s[i], wo_l[:, cs], preferred_element_type=f32)
            r = jnp.concatenate([pin(r[:, :128], 8), r[:, 128:]], axis=1)
            r = acc[r0:r1, cs] + r
            acc[r0:r1, cs] = r
            rb = r.astype(bf16)
            if a == atoms[0]:
                out_v[pl.ds(pl.multiple_of(r0 + zdyn, 16), 16), cs] = rb[:16]
                out_v[r0 + 16:r1, cs] = rb[16:]
            else:
                out_v[r0:r1, cs] = rb
        lim[0] = 32
        if atoms[-1] == 3 and i < NB - 1:
            @pl.when(step == pl.num_programs(0) - 1)
            def _():
                pltpu.make_async_copy(out_v.at[r0:r1, 0:M - 128], o_h.at[r0:r1, 0:M - 128], sems.at[SEM_OUT]).start()

    cv = {}

    UR = CFG.get("ur", 16)

    def u_piece(r):
        j = r // C
        par = cv["par"]
        if r == 0:
            kf = jnp.concatenate([jnp.zeros((8, 128), f32), kt_l[0:UR, :].astype(f32)], axis=0)
        else:
            kf = kt_l[r - 16:r + UR, :].astype(f32)[8:]
        ks = kf[8:] * par[0:1]
        for t in range(1, 4):
            ks = ks + kf[8 - t:8 - t + UR] * par[t:t + 1]
        u = ks * vt_l[r:r + UR, :].astype(f32)
        ub_s[r - j * C:r - j * C + UR, j * 128:(j + 1) * 128] = u.astype(bf16)
        u_s[r:r + UR, :] = u * par[4:5]
        return functools.reduce(jnp.maximum, [u[k:k + 8] for k in range(0, UR, 8)])

    def queue_u():
        cv["par"] = par_s[:, ccol]
        for r in range(0, S, UR):
            side.append((CFG.get("uc", 2.5) * UR, P(u_piece, r)))

    def split(T, j):
        t = T[:, j * 128:(j + 1) * 128]
        re = jnp.concatenate([t[16 * g:16 * g + 8] for g in range(8)], axis=0)
        im = jnp.concatenate([t[16 * g + 8:16 * g + 16] for g in range(8)], axis=0)
        return re, im

    def fwdu(hf):
        lo, hi = hf * NCH // 2, (hf + 1) * NCH // 2
        U = jnp.dot(f_ref[half], ub_s[:, lo * 128:hi * 128], preferred_element_type=f32)
        for j in range(lo, hi):
            re, im = split(U, j - lo)
            V_s[0, j] = re
            V_s[1, j] = im
            V_s[2, j] = re + im

    def fwdh(hf):
        lo, hi = hf * NCH // 2, (hf + 1) * NCH // 2
        hcat = jnp.concatenate([ht_l[:, j * C:(j + 1) * C] for j in range(lo, hi)], axis=0)
        Hf = jax.lax.dot_general(f_ref[half], hcat, NT, preferred_element_type=f32)
        for j in range(lo, hi):
            re, im = split(Hf, j - lo)
            H_s[0, j] = im - re
            H_s[1, j] = re + im
            H_s[2, j] = re

    def mac_piece(i, r, a):
        rs = slice(r, r + 8)
        s = functools.reduce(jnp.add, [H_s[a, i - j, rs, :] * V_s[a, j, rs, :] for j in range(i + 1)])
        cv[a] = s
        if a == 2:
            yr, yi = s - cv[1], s + cv[0]
            wr, wi = yr, yi
            if i > 0:
                pr, pi = cv[("y", r)]
                wr, wi = (yr - pi, yi + pr) if r < 32 else (yr + pi, yi - pr)
            cv[("y", r)] = (yr, yi)
            W_s[2 * r:2 * r + 16, i * 128:(i + 1) * 128] = jnp.concatenate([wr, wi], axis=0).astype(W_s.dtype)
        return s

    def queue_mac():
        for i2 in range(NCH):
            for r in range(0, 64, 8):
                for a in range(3):
                    side.append((MACW * (2 * (i2 + 1) + 3), P(mac_piece, i2, r, a)))

    def inv(hf):
        lo, hi = hf * NCH // 2, (hf + 1) * NCH // 2
        Y = jnp.dot(g_ref[half], W_s[:, lo * 128:hi * 128].astype(bf16), preferred_element_type=f32)
        for j in range(lo, hi):
            a, b = j * C, (j + 1) * C
            y = Y[:, (j - lo) * 128:(j - lo + 1) * 128]
            acc[a:b, ccol] += xg_s[a:b, :] * (y + u_s[a:b, :])

    def xg_piece(r):
        t = (1.0 - gate_s[r:r + 16, :]) * x_v[r:r + 16, ccol].astype(f32)
        xg_s[r:r + 16, :] = t
        return jnp.maximum(t[:8], t[8:])

    def stage_piece(t0):
        w = w_l[t0:t0 + 4].astype(f32).reshape(32, D)
        w_st[t0 * 8:t0 * 8 + 32, :] = w
        return functools.reduce(jnp.maximum, [w[k * 8:(k + 1) * 8] for k in range(4)])

    def extract_piece(wb, off, m0):
        ws = [w_st[pl.ds(2 * (off + m0) + hh, 8, stride=2), :] for hh in range(HP)]
        wb[m0:m0 + 8, :] = jnp.concatenate(ws, axis=1).astype(bf16)
        return ws[0]

    def queue_stage():
        for t0 in range(0, WR // 4, 4):
            side.append((12, P(stage_piece, t0)))

    def queue_extract():
        for (wh, wb, rows, off) in wsets:
            for m0 in range(0, rows, 8):
                side.append((8, P(extract_piece, wb, off, m0)))

    units = [(u // 2, u % 2) for u in range(NU)]

    queue_u()
    pq(0, 0); pk(0, 0); pq(0, 1); pk(0, 1)
    qk(0, 0)
    pvv(0, 0); pvv(0, 1)
    fwdh(0); fwdh(1)
    odone = 0
    ND = CFG.get("normdefer", 1)
    LL = CFG.get("ll", 16)
    for s in range(NU):
        i, hh = units[s]
        if s == FW:
            flush()
            fwdu(0); fwdu(1)
            for cp in early_copies(step + 1): cp.start()

            @pl.when(step == 0)
            def _():
                gate_blocks(NP0, NB)
                c_copy(1).wait()
            late_wait()
            if CFG.get("bal", 1): qk(i, hh, "tail")
            queue_mac()
            queue_stage()
            for r in range(0, S, 16):
                side.append((10, P(xg_piece, r)))
        if s == NU - 2:
            flush()
            queue_extract()
        if i + 1 < NB:
            pk(i + 1, hh); pq(i + 1, hh)
            if not (s >= FW and odone < i and s < NU - 2): lim[0] = LL
            pvv(i + 1, hh)
            lim[0] = 32
            if s >= 1 and "left" in st[units[s - 1]]:
                assert len(side) <= max(st[units[s - 1]]["left"], 0) or s == FW, (s, len(side))
        if s >= FW and odone < i and s < NU - 2:
            oproj(odone, lastlim=LL); odone += 1
        if s == NU - 2:
            oproj(NB - 2, (0, 1))
        if s == NU - 1:
            oproj(NB - 2, (2, 3))
        pv(i, hh, ND and s + 1 < NU - 2 and s + 1 != FW)
        if s + 1 < NU:
            qk(*units[s + 1], "head" if (s + 1 == FW and CFG.get("bal", 1)) else None)
    inv(0); inv(1)
    assert odone == NB - 2
    oproj(NB - 1, fine=CFG.get('fine', 0))
    flush()

    @pl.when(step < pl.num_programs(0) - 1)
    def _():
        for cp in late_copies(step + 1): cp.start()

    @pl.when(step == NSTEP - 1)
    def _():
        r7 = (NB - 1) * BQ
        pltpu.make_async_copy(out_v.at[r7:S, :], o_h.at[r7:S, :], sems.at[SEM_OUT]).start()
        for a, b in ((0, 512), (512, 1024), (1024, r7)):
            out_v[a:b, M - 128:M] = acc[a:b, M - 128:M].astype(bf16)
            pltpu.make_async_copy(out_v.at[a:b, M - 128:M], o_h.at[a:b, M - 128:M], sems.at[SEM_OUT]).start()
        early_wait()
        pltpu.make_async_copy(out_v, o_h, sems.at[SEM_OUT]).wait()


@jax.jit
def pallas_gated_mix__compressed_kv_cla__ssm_conv_h3__prompt_kernel(A_x, A_c_kv, A_w_q, A_w_uk, A_w_uv, A_w_o, B_q, B_k, B_v, B_shift_k, B_ssm_k, B_ssm_D, gate_w):
    x = A_x.reshape(S, M)
    c = A_c_kv.reshape(S, DC)
    wo = A_w_o.reshape(H * D, M)
    k = B_k.reshape(S, M)
    v = B_v.reshape(S, M)
    Fc, Gc = _dft_consts()
    Fc = jnp.asarray(Fc, bf16); Gc = jnp.asarray(Gc, bf16)
    hbm = pl.BlockSpec(memory_space=pl.ANY)
    vm = pl.BlockSpec(memory_space=pltpu.VMEM)
    scratch = [
        pltpu.VMEM((4, M), bf16), pltpu.VMEM((M,), bf16), pltpu.VMEM((M,), bf16),
        pltpu.VMEM((2, 128, C), bf16), pltpu.VMEM((2, C, 128), bf16),
        pltpu.VMEM((S, M), bf16),
        pltpu.VMEM((S, DC), bf16),
        pltpu.VMEM((WR // 4, 8, D), bf16),
        pltpu.VMEM((WR // 4, 8, D), bf16),
        pltpu.VMEM((2 * WR + 8, D), f32),
        pltpu.VMEM((M, HP * D), bf16),
        pltpu.VMEM((DC, HP * D), bf16),
        pltpu.VMEM((DC, HP * D), bf16),
        pltpu.VMEM((HP * D, M), bf16),
        pltpu.VMEM((2, S, 128), bf16),
        pltpu.VMEM((128, S), bf16),
        pltpu.VMEM((S, M), f32),
        pltpu.VMEM((S, 128), f32),
        pltpu.VMEM((S, 128), f32),
        pltpu.VMEM((S, M), bf16),
        pltpu.VMEM((S, HP * D), bf16),
        pltpu.VMEM((S, HP * D), bf16),
        pltpu.VMEM((S, HP * D), bf16),
        pltpu.VMEM((NB, BQ, HP * D), bf16),
        pltpu.VMEM((S, 128), f32),
        pltpu.VMEM((8, M), f32),
        pltpu.VMEM((C, NCH * 128), bf16),
        pltpu.VMEM((3, NCH, 64, 128), f32),
        pltpu.VMEM((3, NCH, 64, 128), f32),
        pltpu.VMEM((128, NCH * 128), bf16 if CFG.get('wbf', 1) else f32),
        pltpu.VMEM((BQ + 8, S + 128), f32),
        pltpu.VMEM((BQ + 8, S + 128), f32),
        pltpu.SemaphoreType.DMA((NSEM,)),
    ]
    out = pl.pallas_call(
        _kernel,
        out_shape=jax.ShapeDtypeStruct((S, M), bf16),
        grid=(NSTEP,),
        in_specs=[hbm] * 14,
        out_specs=hbm,
        scratch_shapes=scratch,
        compiler_params=pltpu.CompilerParams(vmem_limit_bytes=120 * 1024 * 1024, dimension_semantics=("arbitrary",),
                                             disable_bounds_checks=True),
    )(x, c, A_w_q.reshape(M // 4, 4, H, D), A_w_uk.reshape(DC // 4, 4, H, D), A_w_uv.reshape(DC // 4, 4, H, D), wo, k, v, B_ssm_k, B_shift_k.T, B_ssm_D, gate_w, Fc, Gc)
    return out.reshape(1, S, M)
```

```python
import collections
import functools

import numpy as np
import jax
import jax.numpy as jnp
import jax.experimental.pallas as pl
import jax.experimental.pallas.tpu as pltpu

f32, bf16 = jnp.float32, jnp.bfloat16
NT = (((1,), (1,)), ((), ()))

S = 2048
M = 1024
DC = 512
H = 32
D = 128
HP = 2
NSTEP = H // HP
BQ = 256
NB = S // BQ
NU = 2 * NB
C = 128
NCH = S // C
WR = M + 2 * DC
LOG2E = 1.4426950408889634

KC = 4
RATE = 2.0
MACW = 2.0
FW = 4
NP0 = (FW - 1) // 2 + 2
LL = 16

SEM_W, SEM_WO, SEM_KV, SEM_HT, SEM_W0, SEM_OUT = range(6)
SEM_C = 6
SEM_SM = 8
SEM_X = 13
NSEM = SEM_X + NB


def _dft_consts():
    n = np.arange(C)
    Fs, Gs = [], []
    for p in range(2):
        ks = np.arange(p * 64, (p + 1) * 64)
        ks = np.concatenate([ks[ks % 2 == 0], ks[ks % 2 == 1]])
        th = np.pi * (2 * ks[:, None] + 1) * n[None, :] / (2 * C)
        F = np.stack([np.cos(th).reshape(8, 8, C), -np.sin(th).reshape(8, 8, C)], axis=1).reshape(128, C)
        Fs.append(F)
        Gs.append(F.T / C)
    return np.stack(Fs).astype(bf16), np.stack(Gs).astype(bf16)


def _kernel(x_h, c_h, wq_h, wk_h, wv_h, wo_h, k_h, v_h, h_h,
            skt_h, dd_h, gw_h, f_h, g_h,
            o_h,
            skt_ref, dd_ref, gw_ref, f_ref, g_ref,
            x_v, c_v, w_l, w_0, w_st, wq_b, wk_b, wv_b, wo_l,
            kv_l, ht_l, acc, u_s, xg_s, out_v, q_s, k_s, v_s, ctx_s, gate_s, par_s, ub_s,
            V_s, H_s, W_s, s_a, s_b, sems):
    s_s = (s_a, s_b)
    kt_l, vt_l = kv_l.at[0], kv_l.at[1]
    step = pl.program_id(0)
    P = functools.partial
    wsets = ((wq_h, wq_b, M, 0), (wk_h, wk_b, DC, M), (wv_h, wv_b, DC, M + DC))

    def pair_copies(n, land, sem):
        h0 = pl.multiple_of(n * HP, HP)
        return [pltpu.make_async_copy(wh.at[:, j, pl.ds(h0, HP), :],
                                      land.at[off // 4:(off + rows) // 4, HP * j:HP * (j + 1), :], sems.at[sem])
                for (wh, wb, rows, off) in wsets for j in range(4)]

    def late_copies(n):
        return ([pltpu.make_async_copy(wo_h.at[pl.ds(pl.multiple_of(n * 256, 256), 256), :], wo_l, sems.at[SEM_WO])]
                + pair_copies(jnp.minimum(n + 1, NSTEP - 1), w_l, SEM_W))

    def late_wait():
        pltpu.make_async_copy(wo_l, wo_l, sems.at[SEM_WO]).wait()
        pltpu.make_async_copy(w_l, w_l, sems.at[SEM_W]).wait()

    def early_copies(n):
        col = pl.multiple_of((jnp.minimum(n, NSTEP - 1) // 2) * 128, 128)
        return [pltpu.make_async_copy(k_h.at[:, pl.ds(col, 128)], kt_l, sems.at[SEM_KV]),
                pltpu.make_async_copy(v_h.at[:, pl.ds(col, 128)], vt_l, sems.at[SEM_KV]),
                pltpu.make_async_copy(h_h.at[pl.ds(col, 128), :], ht_l, sems.at[SEM_HT])]

    def early_wait():
        pltpu.make_async_copy(kv_l, kv_l, sems.at[SEM_KV]).wait()
        pltpu.make_async_copy(ht_l, ht_l, sems.at[SEM_HT]).wait()

    def c_copy(p):
        a, b = (0, NP0 * BQ) if p == 0 else (NP0 * BQ, S)
        return pltpu.make_async_copy(c_h.at[a:b, :], c_v.at[a:b, :], sems.at[SEM_C + p])

    def x_copy(i):
        rs = pl.ds(i * BQ, BQ) if isinstance(i, int) else pl.ds(pl.multiple_of(i * BQ, BQ), BQ)
        return pltpu.make_async_copy(x_h.at[rs, :], x_v.at[rs, :], sems.at[SEM_X + i])

    def out_copy(r0, r1, c0, c1):
        return pltpu.make_async_copy(out_v.at[r0:r1, c0:c1], o_h.at[r0:r1, c0:c1], sems.at[SEM_OUT])

    def gate_blocks(lo, hi):
        def f(i, c):
            x_copy(i).wait()
            rs = pl.ds(pl.multiple_of(i * BQ, BQ), BQ)
            z = jnp.sum(x_v[rs, :].astype(f32) * par_s[5:6, :], axis=1, keepdims=True)
            gate_s[rs, :] = jnp.broadcast_to(jax.nn.sigmoid(z), (BQ, 128))
            return c
        jax.lax.fori_loop(lo, hi, f, 0)

    @pl.when(step == 0)
    def _():
        w0 = pair_copies(step, w_0, SEM_W0)
        sm = [pltpu.make_async_copy(a, b, sems.at[SEM_SM + n]) for n, (a, b) in enumerate(
            ((skt_h, skt_ref), (dd_h, dd_ref), (gw_h, gw_ref), (f_h, f_ref), (g_h, g_ref)))]
        for cp in (w0 + sm + [x_copy(i) for i in range(NP0)] + [c_copy(0)] + early_copies(step)
                   + [x_copy(i) for i in range(NP0, NB)] + [c_copy(1)] + late_copies(step)):
            cp.start()

        def zero(i, c):
            rs = pl.ds(pl.multiple_of(i * 64, 64), 64)
            acc[rs, :] = jnp.zeros((64, M), f32)
            return c
        jax.lax.fori_loop(0, S // 64, zero, 0)
        for cp in sm:
            cp.wait()
        par_s[0:4, :] = skt_ref[...].astype(f32)
        par_s[4:5, :] = 0.5 * dd_ref[...].astype(f32).reshape(1, M)
        par_s[5:6, :] = gw_ref[...].astype(f32).reshape(1, M)
        par_s[6:8, :] = jnp.zeros((2, M), f32)
        pltpu.make_async_copy(w_0, w_0, sems.at[SEM_W0]).wait()
        w_st[0:2 * WR, :] = w_0[...].astype(f32).reshape(2 * WR, D)
        for (wh, wb, rows, off) in wsets:
            wb[...] = jnp.concatenate(
                [w_st[pl.ds(2 * off + hh, rows, stride=2), :] for hh in range(HP)], axis=1).astype(bf16)
        gate_blocks(0, NP0)
        c_copy(0).wait()

    early_wait()

    ct = step // 2
    half = step % 2
    ccol = pl.ds(pl.multiple_of(ct * 128, 128), 128)
    scale = (D ** -0.5) * LOG2E
    row = jax.lax.broadcasted_iota(jnp.int32, (128, 128), 0)
    col = jax.lax.broadcasted_iota(jnp.int32, (128, 128), 1)
    mask = col <= row
    never8 = f_ref[0, 0:8, :].astype(f32) > 2.0
    never = jnp.concatenate([never8] * 16, axis=0)

    side = collections.deque()
    budget = [0.0]
    lim = [32]

    def pin(arr, spacing):
        R = arr.shape[0]
        out, lastr = [], 0
        for g in range(min(R // 8, lim[0])):
            budget[0] = min(budget[0] + RATE * spacing, 80.0)
            if side and budget[0] >= side[0][0]:
                cost, fn = side.popleft()
                budget[0] -= cost
                v = fn()
                if g * 8 > lastr:
                    out.append(arr[lastr:g * 8])
                out.append(jnp.where(never8, v, arr[g * 8:(g + 1) * 8]))
                lastr = (g + 1) * 8
        if lastr == 0:
            return arr
        if lastr < R:
            out.append(arr[lastr:])
        return jnp.concatenate(out, axis=0)

    def flush():
        while side:
            side.popleft()[1]()

    def pq(i, hh):
        r0, r1 = i * BQ, (i + 1) * BQ
        hs = slice(hh * D, (hh + 1) * D)
        r = jnp.dot(x_v[r0:r1, :], wq_b[:, hs], preferred_element_type=f32)
        q_s[r0:r1, hs] = (pin(r, 8) * scale).astype(bf16)

    def pk(i, hh):
        r0, r1 = i * BQ, (i + 1) * BQ
        hs = slice(hh * D, (hh + 1) * D)
        r = jnp.dot(c_v[r0:r1, :], wk_b[:, hs], preferred_element_type=f32)
        k_s[r0:r1, hs] = pin(r, 8).astype(bf16)

    def pvv(i, hh):
        r0, r1 = i * BQ, (i + 1) * BQ
        hs = slice(hh * D, (hh + 1) * D)
        r = jnp.dot(c_v[r0:r1, :], wv_b[:, hs], preferred_element_type=f32)
        v_s[r0:r1, hs] = pin(r, 8).astype(bf16)

    def chunks(i):
        nt = 2 * i + 1
        out, t = [], 0
        while t < nt:
            n = min(KC, nt - t)
            out.append((0, t * 128, (t + n) * 128))
            t += n
        out.append((128, nt * 128, (nt + 1) * 128))
        return out

    st = {}

    def qk_atom(i, hh, ch):
        rl, kl, kh = ch
        r0 = i * BQ
        hs = slice(hh * D, (hh + 1) * D)
        s = jax.lax.dot_general(q_s[r0 + rl:r0 + BQ, hs], k_s[kl:kh, hs], NT, preferred_element_type=f32)
        nt = (kh - kl) // 128
        tiles = [s[:, t * 128:(t + 1) * 128] for t in range(nt)]
        if kh > r0 + rl:
            d = tiles[-1]
            dm = jnp.where(mask, d[:128], -1e30)
            tiles[-1] = dm if rl == 128 else jnp.concatenate([dm, d[128:]], axis=0)
        u = st.setdefault((i, hh), {"m": [None, None], "l": [None, None], "o": [None, None]})
        for t in range(nt):
            s_s[hh][rl:BQ, kl + t * 128:kl + (t + 1) * 128] = tiles[t]
        mm = functools.reduce(jnp.maximum, tiles)
        for g in range(rl // 128, 2):
            a = mm[g * 128 - rl:(g + 1) * 128 - rl]
            u["m"][g] = a if u["m"][g] is None else jnp.maximum(u["m"][g], a)

    def qk(i, hh, sel=None):
        chs = chunks(i)
        if sel == "head":
            for ch in chs[:-2]:
                qk_atom(i, hh, ch)
            return
        for ch in (chs[-2:] if sel == "tail" else chs):
            qk_atom(i, hh, ch)
        u = st[(i, hh)]
        mx = [jnp.broadcast_to(jnp.max(u["m"][g], axis=1, keepdims=True), (128, 128)) for g in range(2)]
        s_s[hh][0:BQ, S:S + 128] = jnp.concatenate(mx, axis=0)
        s_s[hh][pl.ds(pl.multiple_of(BQ + (step >> 8) * 8, 8), 8), 0:128] = u["m"][1][120:128]
        s_s[hh][pl.ds(pl.multiple_of(BQ + (step >> 8) * 8, 8), 8), S:S + 128] = u["m"][1][120:128]

    def pv_atom(i, hh, ch):
        rl, kl, kh = ch
        hs = slice(hh * D, (hh + 1) * D)
        u = st[(i, hh)]
        m = s_s[hh][rl:BQ, S:S + 128]
        ps = [jnp.exp2(s_s[hh][rl:BQ, k0:k0 + 128] - m) for k0 in range(kl, kh, 128)]
        lp = functools.reduce(jnp.add, ps)
        ls = []
        for g in range(rl // 128, 2):
            a = lp[g * 128 - rl:(g + 1) * 128 - rl]
            u["l"][g] = a if u["l"][g] is None else u["l"][g] + a
            ls.append(u["l"][g])
        ps[-1] = jnp.minimum(ps[-1], jnp.concatenate(ls, axis=0) if len(ls) > 1 else ls[0])
        pb = (jnp.concatenate(ps, axis=1) if len(ps) > 1 else ps[0]).astype(bf16)
        o = jnp.dot(pb, v_s[kl:kh, hs], preferred_element_type=f32)
        for g in range(rl // 128, 2):
            a = o[g * 128 - rl:(g + 1) * 128 - rl]
            u["o"][g] = a if u["o"][g] is None else u["o"][g] + a

    def recip(l):
        r = pl.reciprocal(l, approx=True)
        return r * (2.0 - l * r)

    def norm_piece(i, hh, g, r):
        u = st[(i, hh)]
        hs = slice(hh * D, (hh + 1) * D)
        o = u["o"][g][r:r + 16]
        r0 = i * BQ + g * 128 + r
        c = o * (gate_s[r0:r0 + 16, :] * recip(u["L"][g][r:r + 16]))
        ctx_s[i, g * 128 + r:g * 128 + r + 16, hs] = c.astype(bf16)
        return jnp.maximum(c[:8], c[8:])

    def pv(i, hh, defer):
        for ch in chunks(i):
            pv_atom(i, hh, ch)
        u = st[(i, hh)]
        u["L"] = [jnp.sum(jnp.where(never, u["o"][g], u["l"][g]), axis=1, keepdims=True) for g in range(2)]
        pieces = [(32, P(norm_piece, i, hh, g, r)) for g in range(2) for r in range(0, 128, 16)]
        if defer:
            side.extendleft(reversed(pieces))
            u["left"] = len(side) - len(pieces)
        else:
            for _, fn in pieces:
                fn()

    def oproj(i, atoms=(0, 1, 2, 3), lastlim=32):
        r0, r1 = i * BQ, (i + 1) * BQ
        for a in atoms:
            lim[0] = lastlim if a == atoms[-1] else 32
            cs = slice(a * 256, (a + 1) * 256)
            r = jnp.dot(ctx_s[i], wo_l[:, cs], preferred_element_type=f32)
            r = jnp.concatenate([pin(r[:, :128], 8), r[:, 128:]], axis=1)
            r = acc[r0:r1, cs] + r
            acc[r0:r1, cs] = r
            out_v[r0:r1, cs] = r.astype(bf16)
            if i == NB - 1 and a < 3:
                @pl.when(step == NSTEP - 1)
                def _():
                    out_copy(r0, r1, a * 256, (a + 1) * 256).start()
        lim[0] = 32
        if atoms[-1] == 3 and i < NB - 1:
            @pl.when(step == NSTEP - 1)
            def _():
                out_copy(r0, r1, 0, M - 128).start()

    cv = {}

    def u_piece(r):
        j = r // C
        par = cv["par"]
        if r == 0:
            kf = jnp.concatenate([jnp.zeros((8, 128), f32), kt_l[0:16, :].astype(f32)], axis=0)
        else:
            kf = kt_l[r - 16:r + 16, :].astype(f32)[8:]
        ks = kf[8:] * par[0:1]
        for t in range(1, 4):
            ks = ks + kf[8 - t:24 - t] * par[t:t + 1]
        u = ks * vt_l[r:r + 16, :].astype(f32)
        ub_s[r - j * C:r - j * C + 16, j * 128:(j + 1) * 128] = u.astype(bf16)
        u_s[r:r + 16, :] = u * par[4:5]
        return jnp.maximum(u[:8], u[8:])

    def split(T, j):
        t = T[:, j * 128:(j + 1) * 128]
        re = jnp.concatenate([t[16 * g:16 * g + 8] for g in range(8)], axis=0)
        im = jnp.concatenate([t[16 * g + 8:16 * g + 16] for g in range(8)], axis=0)
        return re, im

    def fwdu(hf):
        lo, hi = hf * NCH // 2, (hf + 1) * NCH // 2
        U = jnp.dot(f_ref[half], ub_s[:, lo * 128:hi * 128], preferred_element_type=f32)
        for j in range(lo, hi):
            re, im = split(U, j - lo)
            V_s[0, j] = re
            V_s[1, j] = im
            V_s[2, j] = re + im

    def fwdh(hf):
        lo, hi = hf * NCH // 2, (hf + 1) * NCH // 2
        hcat = jnp.concatenate([ht_l[:, j * C:(j + 1) * C] for j in range(lo, hi)], axis=0)
        Hf = jax.lax.dot_general(f_ref[half], hcat, NT, preferred_element_type=f32)
        for j in range(lo, hi):
            re, im = split(Hf, j - lo)
            H_s[0, j] = im - re
            H_s[1, j] = re + im
            H_s[2, j] = re

    def mac_piece(i, r, a):
        rs = slice(r, r + 8)
        s = functools.reduce(jnp.add, [H_s[a, i - j, rs, :] * V_s[a, j, rs, :] for j in range(i + 1)])
        cv[a] = s
        if a == 2:
            yr, yi = s - cv[1], s + cv[0]
            wr, wi = yr, yi
            if i > 0:
                pr, pi = cv[("y", r)]
                wr, wi = (yr - pi, yi + pr) if r < 32 else (yr + pi, yi - pr)
            cv[("y", r)] = (yr, yi)
            W_s[2 * r:2 * r + 16, i * 128:(i + 1) * 128] = jnp.concatenate([wr, wi], axis=0).astype(bf16)
        return s

    def inv(hf):
        lo, hi = hf * NCH // 2, (hf + 1) * NCH // 2
        Y = jnp.dot(g_ref[half], W_s[:, lo * 128:hi * 128], preferred_element_type=f32)
        for j in range(lo, hi):
            a, b = j * C, (j + 1) * C
            y = Y[:, (j - lo) * 128:(j - lo + 1) * 128]
            acc[a:b, ccol] += xg_s[a:b, :] * (y + u_s[a:b, :])

    def xg_piece(r):
        t = (1.0 - gate_s[r:r + 16, :]) * x_v[r:r + 16, ccol].astype(f32)
        xg_s[r:r + 16, :] = t
        return jnp.maximum(t[:8], t[8:])

    def stage_piece(t0):
        w = w_l[t0:t0 + 4].astype(f32).reshape(32, D)
        w_st[t0 * 8:t0 * 8 + 32, :] = w
        return functools.reduce(jnp.maximum, [w[k * 8:(k + 1) * 8] for k in range(4)])

    def extract_piece(wb, off, m0):
        ws = [w_st[pl.ds(2 * (off + m0) + hh, 8, stride=2), :] for hh in range(HP)]
        wb[m0:m0 + 8, :] = jnp.concatenate(ws, axis=1).astype(bf16)
        return ws[0]

    units = [(u // 2, u % 2) for u in range(NU)]

    cv["par"] = par_s[:, ccol]
    for r in range(0, S, 16):
        side.append((40, P(u_piece, r)))
    pq(0, 0); pk(0, 0); pq(0, 1); pk(0, 1)
    qk(0, 0)
    pvv(0, 0); pvv(0, 1)
    fwdh(0); fwdh(1)
    odone = 0
    for s in range(NU):
        i, hh = units[s]
        if s == FW:
            flush()
            fwdu(0); fwdu(1)
            for cp in early_copies(step + 1):
                cp.start()

            @pl.when(step == 0)
            def _():
                gate_blocks(NP0, NB)
                c_copy(1).wait()
            late_wait()
            qk(i, hh, "tail")
            for i2 in range(NCH):
                for r in range(0, 64, 8):
                    for a in range(3):
                        side.append((MACW * (2 * (i2 + 1) + 3), P(mac_piece, i2, r, a)))
            for t0 in range(0, WR // 4, 4):
                side.append((12, P(stage_piece, t0)))
            for r in range(0, S, 16):
                side.append((10, P(xg_piece, r)))
        if s == NU - 2:
            flush()
            for (wh, wb, rows, off) in wsets:
                for m0 in range(0, rows, 8):
                    side.append((8, P(extract_piece, wb, off, m0)))
        do_o = s >= FW and odone < i and s < NU - 2
        if i + 1 < NB:
            pk(i + 1, hh); pq(i + 1, hh)
            if not do_o:
                lim[0] = LL
            pvv(i + 1, hh)
            lim[0] = 32
            if s >= 1 and "left" in st[units[s - 1]]:
                assert len(side) <= st[units[s - 1]]["left"]
        if do_o:
            oproj(odone, lastlim=LL)
            odone += 1
        if s == NU - 2:
            oproj(NB - 2, (0, 1))
        if s == NU - 1:
            oproj(NB - 2, (2, 3))
        pv(i, hh, s + 1 < NU - 2 and s + 1 != FW)
        if s + 1 < NU:
            qk(*units[s + 1], "head" if s + 1 == FW else None)
    inv(0); inv(1)
    assert odone == NB - 2
    oproj(NB - 1)
    flush()

    @pl.when(step < NSTEP - 1)
    def _():
        for cp in late_copies(step + 1):
            cp.start()

    @pl.when(step == NSTEP - 1)
    def _():
        r7 = (NB - 1) * BQ
        out_copy(r7, S, 768, M).start()
        for a, b in ((0, 512), (512, 1024), (1024, r7)):
            out_v[a:b, M - 128:M] = acc[a:b, M - 128:M].astype(bf16)
            out_copy(a, b, M - 128, M).start()
        early_wait()
        pltpu.make_async_copy(out_v, o_h, sems.at[SEM_OUT]).wait()


@jax.jit
def pallas_gated_mix__compressed_kv_cla__ssm_conv_h3__prompt_kernel(
    A_x: jax.Array,
    A_c_kv: jax.Array,
    A_w_q: jax.Array,
    A_w_uk: jax.Array,
    A_w_uv: jax.Array,
    A_w_o: jax.Array,
    B_q: jax.Array,
    B_k: jax.Array,
    B_v: jax.Array,
    B_shift_k: jax.Array,
    B_ssm_k: jax.Array,
    B_ssm_D: jax.Array,
    gate_w: jax.Array,
):
    del B_q
    Fc, Gc = _dft_consts()
    hbm = pl.BlockSpec(memory_space=pl.ANY)
    scratch = [
        pltpu.VMEM((4, M), bf16),
        pltpu.VMEM((M,), bf16),
        pltpu.VMEM((M,), bf16),
        pltpu.VMEM((2, 128, C), bf16),
        pltpu.VMEM((2, C, 128), bf16),
        pltpu.VMEM((S, M), bf16),
        pltpu.VMEM((S, DC), bf16),
        pltpu.VMEM((WR // 4, 8, D), bf16),
        pltpu.VMEM((WR // 4, 8, D), bf16),
        pltpu.VMEM((2 * WR + 8, D), f32),
        pltpu.VMEM((M, HP * D), bf16),
        pltpu.VMEM((DC, HP * D), bf16),
        pltpu.VMEM((DC, HP * D), bf16),
        pltpu.VMEM((HP * D, M), bf16),
        pltpu.VMEM((2, S, 128), bf16),
        pltpu.VMEM((128, S), bf16),
        pltpu.VMEM((S, M), f32),
        pltpu.VMEM((S, 128), f32),
        pltpu.VMEM((S, 128), f32),
        pltpu.VMEM((S, M), bf16),
        pltpu.VMEM((S, HP * D), bf16),
        pltpu.VMEM((S, HP * D), bf16),
        pltpu.VMEM((S, HP * D), bf16),
        pltpu.VMEM((NB, BQ, HP * D), bf16),
        pltpu.VMEM((S, 128), f32),
        pltpu.VMEM((8, M), f32),
        pltpu.VMEM((C, NCH * 128), bf16),
        pltpu.VMEM((3, NCH, 64, 128), f32),
        pltpu.VMEM((3, NCH, 64, 128), f32),
        pltpu.VMEM((128, NCH * 128), bf16),
        pltpu.VMEM((BQ + 8, S + 128), f32),
        pltpu.VMEM((BQ + 8, S + 128), f32),
        pltpu.SemaphoreType.DMA((NSEM,)),
    ]
    out = pl.pallas_call(
        _kernel,
        out_shape=jax.ShapeDtypeStruct((S, M), bf16),
        grid=(NSTEP,),
        in_specs=[hbm] * 14,
        out_specs=hbm,
        scratch_shapes=scratch,
        compiler_params=pltpu.CompilerParams(
            vmem_limit_bytes=100 * 1024 * 1024,
            dimension_semantics=("arbitrary",),
            disable_bounds_checks=True),
    )(A_x.reshape(S, M), A_c_kv.reshape(S, DC),
      A_w_q.reshape(M // 4, 4, H, D), A_w_uk.reshape(DC // 4, 4, H, D), A_w_uv.reshape(DC // 4, 4, H, D),
      A_w_o.reshape(H * D, M), B_k.reshape(S, M), B_v.reshape(S, M), B_ssm_k,
      B_shift_k.T, B_ssm_D, gate_w, jnp.asarray(Fc), jnp.asarray(Gc))
    return out.reshape(1, S, M)
```

```python
import collections
import functools

import numpy as np
import jax
import jax.numpy as jnp
import jax.experimental.pallas as pl
import jax.experimental.pallas.tpu as pltpu

f32, bf16 = jnp.float32, jnp.bfloat16
NT = (((1,), (1,)), ((), ()))

S = 2048
M = 1024
DC = 512
H = 32
D = 128
HP = 2
NSTEP = H // HP
BQ = 256
NB = S // BQ
NU = 2 * NB
C = 128
NCH = S // C
WR = M + 2 * DC
LOG2E = 1.4426950408889634

KC = 4
RATE = 2.0
MACW = 2.0
FW = 4
NP0 = (FW - 1) // 2 + 2
LL = 16

SEM_W, SEM_WO, SEM_KV, SEM_HT, SEM_W0, SEM_OUT = range(6)
SEM_C = 6
SEM_SM = 8
SEM_X = 13
NSEM = SEM_X + NB


def _dft_consts():
    n = np.arange(C)
    Fs, Gs = [], []
    for p in range(2):
        ks = np.arange(p * 64, (p + 1) * 64)
        ks = np.concatenate([ks[ks % 2 == 0], ks[ks % 2 == 1]])
        th = np.pi * (2 * ks[:, None] + 1) * n[None, :] / (2 * C)
        F = np.stack([np.cos(th).reshape(8, 8, C), -np.sin(th).reshape(8, 8, C)], axis=1).reshape(128, C)
        Fs.append(F)
        Gs.append(F.T / C)
    return np.stack(Fs).astype(bf16), np.stack(Gs).astype(bf16)


def _kernel(x_h, c_h, wq_h, wk_h, wv_h, wo_h, k_h, v_h, h_h,
            skt_h, dd_h, gw_h, f_h, g_h,
            o_h,
            skt_ref, dd_ref, gw_ref, f_ref, g_ref,
            x_v, c_v, w_l, w_0, w_st, wq_b, wk_b, wv_b, wo_l,
            kv_l, ht_l, acc, xg_s, out_v, q_s, k_s, v_s, ctx_s, gate_s, par_s, ub_s,
            V_s, H_s, W_s, s_a, s_b, sems):
    s_s = (s_a, s_b)
    kt_l, vt_l = kv_l.at[0], kv_l.at[1]
    step = pl.program_id(0)
    P = functools.partial
    wsets = ((wq_h, wq_b, M, 0), (wk_h, wk_b, DC, M), (wv_h, wv_b, DC, M + DC))

    def pair_copies(n, land, sem):
        h0 = pl.multiple_of(n * HP, HP)
        return [pltpu.make_async_copy(wh.at[:, j, pl.ds(h0, HP), :],
                                      land.at[off // 4:(off + rows) // 4, HP * j:HP * (j + 1), :], sems.at[sem])
                for (wh, wb, rows, off) in wsets for j in range(4)]

    def late_copies(n):
        return ([pltpu.make_async_copy(wo_h.at[pl.ds(pl.multiple_of(n * 256, 256), 256), :], wo_l, sems.at[SEM_WO])]
                + pair_copies(jnp.minimum(n + 1, NSTEP - 1), w_l, SEM_W))

    def late_wait():
        pltpu.make_async_copy(wo_l, wo_l, sems.at[SEM_WO]).wait()
        pltpu.make_async_copy(w_l, w_l, sems.at[SEM_W]).wait()

    def early_copies(n):
        col = pl.multiple_of((jnp.minimum(n, NSTEP - 1) // 2) * 128, 128)
        return [pltpu.make_async_copy(k_h.at[:, pl.ds(col, 128)], kt_l, sems.at[SEM_KV]),
                pltpu.make_async_copy(v_h.at[:, pl.ds(col, 128)], vt_l, sems.at[SEM_KV]),
                pltpu.make_async_copy(h_h.at[pl.ds(col, 128), :], ht_l, sems.at[SEM_HT])]

    def early_wait():
        pltpu.make_async_copy(kv_l, kv_l, sems.at[SEM_KV]).wait()
        pltpu.make_async_copy(ht_l, ht_l, sems.at[SEM_HT]).wait()

    def c_copy(p):
        a, b = (0, NP0 * BQ) if p == 0 else (NP0 * BQ, S)
        return pltpu.make_async_copy(c_h.at[a:b, :], c_v.at[a:b, :], sems.at[SEM_C + p])

    def x_copy(i):
        rs = pl.ds(i * BQ, BQ) if isinstance(i, int) else pl.ds(pl.multiple_of(i * BQ, BQ), BQ)
        return pltpu.make_async_copy(x_h.at[rs, :], x_v.at[rs, :], sems.at[SEM_X + i])

    def out_copy(r0, r1, c0, c1):
        return pltpu.make_async_copy(out_v.at[r0:r1, c0:c1], o_h.at[r0:r1, c0:c1], sems.at[SEM_OUT])

    def gate_blocks(lo, hi):
        def f(i, c):
            x_copy(i).wait()
            rs = pl.ds(pl.multiple_of(i * BQ, BQ), BQ)
            z = jnp.sum(x_v[rs, :].astype(f32) * par_s[5:6, :], axis=1, keepdims=True)
            gate_s[rs, :] = jnp.broadcast_to(jax.nn.sigmoid(z), (BQ, 128))
            return c
        jax.lax.fori_loop(lo, hi, f, 0)

    @pl.when(step == 0)
    def _():
        w0 = pair_copies(step, w_0, SEM_W0)
        sm = [pltpu.make_async_copy(a, b, sems.at[SEM_SM + n]) for n, (a, b) in enumerate(
            ((skt_h, skt_ref), (dd_h, dd_ref), (gw_h, gw_ref), (f_h, f_ref), (g_h, g_ref)))]
        for cp in (w0 + sm + [x_copy(i) for i in range(NP0)] + [c_copy(0)] + early_copies(step)
                   + [x_copy(i) for i in range(NP0, NB)] + [c_copy(1)] + late_copies(step)):
            cp.start()

        def zero(i, c):
            rs = pl.ds(pl.multiple_of(i * 64, 64), 64)
            acc[rs, :] = jnp.zeros((64, M), f32)
            return c
        jax.lax.fori_loop(0, S // 64, zero, 0)
        for cp in sm:
            cp.wait()
        par_s[0:4, :] = skt_ref[...].astype(f32)
        par_s[4:5, :] = dd_ref[...].astype(f32).reshape(1, M)
        par_s[5:6, :] = gw_ref[...].astype(f32).reshape(1, M)
        par_s[6:8, :] = jnp.zeros((2, M), f32)
        pltpu.make_async_copy(w_0, w_0, sems.at[SEM_W0]).wait()
        w_st[0:2 * WR, :] = w_0[...].astype(f32).reshape(2 * WR, D)
        for (wh, wb, rows, off) in wsets:
            wb[...] = jnp.concatenate(
                [w_st[pl.ds(2 * off + hh, rows, stride=2), :] for hh in range(HP)], axis=1).astype(bf16)
        gate_blocks(0, NP0)
        c_copy(0).wait()

    early_wait()

    ct = step // 2
    half = step % 2
    ccol = pl.ds(pl.multiple_of(ct * 128, 128), 128)
    scale = (D ** -0.5) * LOG2E
    row = jax.lax.broadcasted_iota(jnp.int32, (128, 128), 0)
    col = jax.lax.broadcasted_iota(jnp.int32, (128, 128), 1)
    mask = col <= row
    never8 = f_ref[0, 0:8, :].astype(f32) > 2.0
    never = jnp.concatenate([never8] * 16, axis=0)

    side = collections.deque()
    budget = [0.0]
    lim = [32]

    def pin(arr, spacing):
        R = arr.shape[0]
        out, lastr = [], 0
        for g in range(min(R // 8, lim[0])):
            budget[0] = min(budget[0] + RATE * spacing, 80.0)
            if side and budget[0] >= side[0][0]:
                cost, fn = side.popleft()
                budget[0] -= cost
                v = fn()
                if g * 8 > lastr:
                    out.append(arr[lastr:g * 8])
                out.append(jnp.where(never8, v, arr[g * 8:(g + 1) * 8]))
                lastr = (g + 1) * 8
        if lastr == 0:
            return arr
        if lastr < R:
            out.append(arr[lastr:])
        return jnp.concatenate(out, axis=0)

    def flush():
        while side:
            side.popleft()[1]()

    def pq(i, hh):
        r0, r1 = i * BQ, (i + 1) * BQ
        hs = slice(hh * D, (hh + 1) * D)
        r = jnp.dot(x_v[r0:r1, :], wq_b[:, hs], preferred_element_type=f32)
        q_s[r0:r1, hs] = (pin(r, 8) * scale).astype(bf16)

    def pk(i, hh):
        r0, r1 = i * BQ, (i + 1) * BQ
        hs = slice(hh * D, (hh + 1) * D)
        r = jnp.dot(c_v[r0:r1, :], wk_b[:, hs], preferred_element_type=f32)
        k_s[r0:r1, hs] = pin(r, 8).astype(bf16)

    def pvv(i, hh):
        r0, r1 = i * BQ, (i + 1) * BQ
        hs = slice(hh * D, (hh + 1) * D)
        r = jnp.dot(c_v[r0:r1, :], wv_b[:, hs], preferred_element_type=f32)
        v_s[r0:r1, hs] = pin(r, 8).astype(bf16)

    def chunks(i):
        nt = 2 * i + 1
        out, t = [], 0
        while t < nt:
            n = min(KC, nt - t)
            out.append((0, t * 128, (t + n) * 128))
            t += n
        out.append((128, nt * 128, (nt + 1) * 128))
        return out

    st = {}

    def qk_atom(i, hh, ch):
        rl, kl, kh = ch
        r0 = i * BQ
        hs = slice(hh * D, (hh + 1) * D)
        s = jax.lax.dot_general(q_s[r0 + rl:r0 + BQ, hs], k_s[kl:kh, hs], NT, preferred_element_type=f32)
        nt = (kh - kl) // 128
        tiles = [s[:, t * 128:(t + 1) * 128] for t in range(nt)]
        if kh > r0 + rl:
            d = tiles[-1]
            dm = jnp.where(mask, d[:128], -1e30)
            tiles[-1] = dm if rl == 128 else jnp.concatenate([dm, d[128:]], axis=0)
        u = st.setdefault((i, hh), {"m": [None, None], "l": [None, None], "o": [None, None]})
        for t in range(nt):
            s_s[hh][rl:BQ, kl + t * 128:kl + (t + 1) * 128] = tiles[t]
        mm = functools.reduce(jnp.maximum, tiles)
        for g in range(rl // 128, 2):
            a = mm[g * 128 - rl:(g + 1) * 128 - rl]
            u["m"][g] = a if u["m"][g] is None else jnp.maximum(u["m"][g], a)

    def qk(i, hh, sel=None):
        chs = chunks(i)
        if sel == "head":
            for ch in chs[:-2]:
                qk_atom(i, hh, ch)
            return
        for ch in (chs[-2:] if sel == "tail" else chs):
            qk_atom(i, hh, ch)
        u = st[(i, hh)]
        mx = [jnp.broadcast_to(jnp.max(u["m"][g], axis=1, keepdims=True), (128, 128)) for g in range(2)]
        s_s[hh][0:BQ, S:S + 128] = jnp.concatenate(mx, axis=0)
        s_s[hh][pl.ds(pl.multiple_of(BQ + (step >> 8) * 8, 8), 8), 0:128] = u["m"][1][120:128]
        s_s[hh][pl.ds(pl.multiple_of(BQ + (step >> 8) * 8, 8), 8), S:S + 128] = u["m"][1][120:128]

    def pv_atom(i, hh, ch):
        rl, kl, kh = ch
        hs = slice(hh * D, (hh + 1) * D)
        u = st[(i, hh)]
        m = s_s[hh][rl:BQ, S:S + 128]
        ps = [jnp.exp2(s_s[hh][rl:BQ, k0:k0 + 128] - m) for k0 in range(kl, kh, 128)]
        lp = functools.reduce(jnp.add, ps)
        ls = []
        for g in range(rl // 128, 2):
            a = lp[g * 128 - rl:(g + 1) * 128 - rl]
            u["l"][g] = a if u["l"][g] is None else u["l"][g] + a
            ls.append(u["l"][g])
        ps[-1] = jnp.minimum(ps[-1], jnp.concatenate(ls, axis=0) if len(ls) > 1 else ls[0])
        pb = (jnp.concatenate(ps, axis=1) if len(ps) > 1 else ps[0]).astype(bf16)
        o = jnp.dot(pb, v_s[kl:kh, hs], preferred_element_type=f32)
        for g in range(rl // 128, 2):
            a = o[g * 128 - rl:(g + 1) * 128 - rl]
            u["o"][g] = a if u["o"][g] is None else u["o"][g] + a

    def recip(l):
        r = pl.reciprocal(l, approx=True)
        return r * (2.0 - l * r)

    def norm_piece(i, hh, g, r):
        u = st[(i, hh)]
        hs = slice(hh * D, (hh + 1) * D)
        o = u["o"][g][r:r + 16]
        r0 = i * BQ + g * 128 + r
        c = o * (gate_s[r0:r0 + 16, :] * recip(u["L"][g][r:r + 16]))
        ctx_s[i, g * 128 + r:g * 128 + r + 16, hs] = c.astype(bf16)
        return jnp.maximum(c[:8], c[8:])

    def pv(i, hh, defer):
        for ch in chunks(i):
            pv_atom(i, hh, ch)
        u = st[(i, hh)]
        u["L"] = [jnp.sum(jnp.where(never, u["o"][g], u["l"][g]), axis=1, keepdims=True) for g in range(2)]
        pieces = [(32, P(norm_piece, i, hh, g, r)) for g in range(2) for r in range(0, 128, 16)]
        if defer:
            side.extendleft(reversed(pieces))
            u["left"] = len(side) - len(pieces)
        else:
            for _, fn in pieces:
                fn()

    def oproj(i, atoms=(0, 1, 2, 3), lastlim=32):
        r0, r1 = i * BQ, (i + 1) * BQ
        for a in atoms:
            lim[0] = lastlim if a == atoms[-1] else 32
            cs = slice(a * 256, (a + 1) * 256)
            r = jnp.dot(ctx_s[i], wo_l[:, cs], preferred_element_type=f32)
            r = jnp.concatenate([pin(r[:, :128], 8), r[:, 128:]], axis=1)
            r = acc[r0:r1, cs] + r
            acc[r0:r1, cs] = r
            out_v[r0:r1, cs] = r.astype(bf16)
            if i == NB - 1 and a < 3:
                @pl.when(step == NSTEP - 1)
                def _():
                    out_copy(r0, r1, a * 256, (a + 1) * 256).start()
        lim[0] = 32
        if atoms[-1] == 3 and i < NB - 1:
            @pl.when(step == NSTEP - 1)
            def _():
                out_copy(r0, r1, 0, M - 128).start()

    cv = {}

    def u_piece(r):
        j = r // C
        par = cv["par"]
        if r == 0:
            kf = jnp.concatenate([jnp.zeros((8, 128), f32), kt_l[0:16, :].astype(f32)], axis=0)
        else:
            kf = kt_l[r - 16:r + 16, :].astype(f32)[8:]
        ks = kf[8:] * par[0:1]
        for t in range(1, 4):
            ks = ks + kf[8 - t:24 - t] * par[t:t + 1]
        u = ks * vt_l[r:r + 16, :].astype(f32)
        ub_s[r - j * C:r - j * C + 16, j * 128:(j + 1) * 128] = u.astype(bf16)
        return jnp.maximum(u[:8], u[8:])

    def split(T, j):
        t = T[:, j * 128:(j + 1) * 128]
        re = jnp.concatenate([t[16 * g:16 * g + 8] for g in range(8)], axis=0)
        im = jnp.concatenate([t[16 * g + 8:16 * g + 16] for g in range(8)], axis=0)
        return re, im

    def fwdu(hf):
        lo, hi = hf * NCH // 2, (hf + 1) * NCH // 2
        U = jnp.dot(f_ref[half], ub_s[:, lo * 128:hi * 128], preferred_element_type=f32)
        for j in range(lo, hi):
            re, im = split(U, j - lo)
            V_s[0, j] = re
            V_s[1, j] = im
            V_s[2, j] = re + im

    def fwdh(hf):
        lo, hi = hf * NCH // 2, (hf + 1) * NCH // 2
        hcat = jnp.concatenate([ht_l[:, j * C:(j + 1) * C] for j in range(lo, hi)], axis=0)
        Hf = jax.lax.dot_general(f_ref[half], hcat, NT, preferred_element_type=f32)
        for j in range(lo, hi):
            re, im = split(Hf, j - lo)
            if j == 0:
                re = re + cv["par"][4:5]
            H_s[0, j] = im - re
            H_s[1, j] = re + im
            H_s[2, j] = re

    def mac_piece(i, r, a):
        rs = slice(r, r + 8)
        s = functools.reduce(jnp.add, [H_s[a, i - j, rs, :] * V_s[a, j, rs, :] for j in range(i + 1)])
        cv[a] = s
        if a == 2:
            yr, yi = s - cv[1], s + cv[0]
            wr, wi = yr, yi
            if i > 0:
                pr, pi = cv[("y", r)]
                wr, wi = (yr - pi, yi + pr) if r < 32 else (yr + pi, yi - pr)
            cv[("y", r)] = (yr, yi)
            W_s[2 * r:2 * r + 16, i * 128:(i + 1) * 128] = jnp.concatenate([wr, wi], axis=0).astype(bf16)
        return s

    def inv(hf):
        lo, hi = hf * NCH // 2, (hf + 1) * NCH // 2
        Y = jnp.dot(g_ref[half], W_s[:, lo * 128:hi * 128], preferred_element_type=f32)
        for j in range(lo, hi):
            a, b = j * C, (j + 1) * C
            y = Y[:, (j - lo) * 128:(j - lo + 1) * 128]
            acc[a:b, ccol] += xg_s[a:b, :] * y

    def xg_piece(r):
        t = (1.0 - gate_s[r:r + 16, :]) * x_v[r:r + 16, ccol].astype(f32)
        xg_s[r:r + 16, :] = t
        return jnp.maximum(t[:8], t[8:])

    def stage_piece(t0):
        w = w_l[t0:t0 + 4].astype(f32).reshape(32, D)
        w_st[t0 * 8:t0 * 8 + 32, :] = w
        return functools.reduce(jnp.maximum, [w[k * 8:(k + 1) * 8] for k in range(4)])

    def extract_piece(wb, off, m0):
        ws = [w_st[pl.ds(2 * (off + m0) + hh, 8, stride=2), :] for hh in range(HP)]
        wb[m0:m0 + 8, :] = jnp.concatenate(ws, axis=1).astype(bf16)
        return ws[0]

    units = [(u // 2, u % 2) for u in range(NU)]

    cv["par"] = par_s[:, ccol]
    for r in range(0, S, 16):
        side.append((40, P(u_piece, r)))
    pq(0, 0); pk(0, 0); pq(0, 1); pk(0, 1)
    qk(0, 0)
    pvv(0, 0); pvv(0, 1)
    fwdh(0); fwdh(1)
    odone = 0
    for s in range(NU):
        i, hh = units[s]
        if s == FW:
            flush()
            fwdu(0); fwdu(1)
            for cp in early_copies(step + 1):
                cp.start()

            @pl.when(step == 0)
            def _():
                gate_blocks(NP0, NB)
                c_copy(1).wait()
            late_wait()
            qk(i, hh, "tail")
            for i2 in range(NCH):
                for r in range(0, 64, 8):
                    for a in range(3):
                        side.append((MACW * (2 * (i2 + 1) + 3), P(mac_piece, i2, r, a)))
            for t0 in range(0, WR // 4, 4):
                side.append((12, P(stage_piece, t0)))
            for r in range(0, S, 16):
                side.append((10, P(xg_piece, r)))
        if s == NU - 2:
            flush()
            for (wh, wb, rows, off) in wsets:
                for m0 in range(0, rows, 8):
                    side.append((8, P(extract_piece, wb, off, m0)))
        do_o = s >= FW and odone < i and s < NU - 2
        if i + 1 < NB:
            pk(i + 1, hh); pq(i + 1, hh)
            if not do_o:
                lim[0] = LL
            pvv(i + 1, hh)
            lim[0] = 32
            if s >= 1 and "left" in st[units[s - 1]]:
                assert len(side) <= st[units[s - 1]]["left"]
        if do_o:
            oproj(odone, lastlim=LL)
            odone += 1
        if s == NU - 2:
            oproj(NB - 2, (0, 1))
        if s == NU - 1:
            oproj(NB - 2, (2, 3))
        pv(i, hh, s + 1 < NU - 2 and s + 1 != FW)
        if s + 1 < NU:
            qk(*units[s + 1], "head" if s + 1 == FW else None)
    inv(0); inv(1)
    assert odone == NB - 2
    oproj(NB - 1)
    flush()

    @pl.when(step < NSTEP - 1)
    def _():
        for cp in late_copies(step + 1):
            cp.start()

    @pl.when(step == NSTEP - 1)
    def _():
        r7 = (NB - 1) * BQ
        out_copy(r7, S, 768, M).start()
        for a, b in ((0, 512), (512, 1024), (1024, r7)):
            out_v[a:b, M - 128:M] = acc[a:b, M - 128:M].astype(bf16)
            out_copy(a, b, M - 128, M).start()
        early_wait()
        pltpu.make_async_copy(out_v, o_h, sems.at[SEM_OUT]).wait()


@jax.jit
def pallas_gated_mix__compressed_kv_cla__ssm_conv_h3__prompt_kernel(
    A_x: jax.Array,
    A_c_kv: jax.Array,
    A_w_q: jax.Array,
    A_w_uk: jax.Array,
    A_w_uv: jax.Array,
    A_w_o: jax.Array,
    B_q: jax.Array,
    B_k: jax.Array,
    B_v: jax.Array,
    B_shift_k: jax.Array,
    B_ssm_k: jax.Array,
    B_ssm_D: jax.Array,
    gate_w: jax.Array,
):
    del B_q
    Fc, Gc = _dft_consts()
    hbm = pl.BlockSpec(memory_space=pl.ANY)
    scratch = [
        pltpu.VMEM((4, M), bf16),
        pltpu.VMEM((M,), bf16),
        pltpu.VMEM((M,), bf16),
        pltpu.VMEM((2, 128, C), bf16),
        pltpu.VMEM((2, C, 128), bf16),
        pltpu.VMEM((S, M), bf16),
        pltpu.VMEM((S, DC), bf16),
        pltpu.VMEM((WR // 4, 8, D), bf16),
        pltpu.VMEM((WR // 4, 8, D), bf16),
        pltpu.VMEM((2 * WR + 8, D), f32),
        pltpu.VMEM((M, HP * D), bf16),
        pltpu.VMEM((DC, HP * D), bf16),
        pltpu.VMEM((DC, HP * D), bf16),
        pltpu.VMEM((HP * D, M), bf16),
        pltpu.VMEM((2, S, 128), bf16),
        pltpu.VMEM((128, S), bf16),
        pltpu.VMEM((S, M), f32),
        pltpu.VMEM((S, 128), f32),
        pltpu.VMEM((S, M), bf16),
        pltpu.VMEM((S, HP * D), bf16),
        pltpu.VMEM((S, HP * D), bf16),
        pltpu.VMEM((S, HP * D), bf16),
        pltpu.VMEM((NB, BQ, HP * D), bf16),
        pltpu.VMEM((S, 128), f32),
        pltpu.VMEM((8, M), f32),
        pltpu.VMEM((C, NCH * 128), bf16),
        pltpu.VMEM((3, NCH, 64, 128), f32),
        pltpu.VMEM((3, NCH, 64, 128), f32),
        pltpu.VMEM((128, NCH * 128), bf16),
        pltpu.VMEM((BQ + 8, S + 128), f32),
        pltpu.VMEM((BQ + 8, S + 128), f32),
        pltpu.SemaphoreType.DMA((NSEM,)),
    ]
    out = pl.pallas_call(
        _kernel,
        out_shape=jax.ShapeDtypeStruct((S, M), bf16),
        grid=(NSTEP,),
        in_specs=[hbm] * 14,
        out_specs=hbm,
        scratch_shapes=scratch,
        compiler_params=pltpu.CompilerParams(
            vmem_limit_bytes=100 * 1024 * 1024,
            dimension_semantics=("arbitrary",),
            disable_bounds_checks=True),
    )(A_x.reshape(S, M), A_c_kv.reshape(S, DC),
      A_w_q.reshape(M // 4, 4, H, D), A_w_uk.reshape(DC // 4, 4, H, D), A_w_uv.reshape(DC // 4, 4, H, D),
      A_w_o.reshape(H * D, M), B_k.reshape(S, M), B_v.reshape(S, M), B_ssm_k,
      B_shift_k.T, B_ssm_D, gate_w, jnp.asarray(Fc), jnp.asarray(Gc))
    return out.reshape(1, S, M)
```

```python
import collections
import functools

import numpy as np
import jax
import jax.numpy as jnp
import jax.experimental.pallas as pl
import jax.experimental.pallas.tpu as pltpu

f32, bf16 = jnp.float32, jnp.bfloat16
NT = (((1,), (1,)), ((), ()))

S = 2048
M = 1024
DC = 512
H = 32
D = 128
HP = 2
NSTEP = H // HP
BQ = 256
NB = S // BQ
NU = 2 * NB
C = 128
NCH = S // C
WR = M + 2 * DC
LOG2E = 1.4426950408889634

XO = 256
KC = 4
RATE = 2.0
MACW = 2.0
FW = 4
NP0 = (FW - 1) // 2 + 2
LL = 16

SEM_W, SEM_WO, SEM_KV, SEM_HT, SEM_W0, SEM_OUT = range(6)
SEM_C = 6
SEM_SM = 8
SEM_X = 13
NSEM = SEM_X + NB


def _dft_consts():
    n = np.arange(C)
    Fs, Gs = [], []
    for p in range(2):
        ks = np.arange(p * 64, (p + 1) * 64)
        ks = np.concatenate([ks[ks % 2 == 0], ks[ks % 2 == 1]])
        th = np.pi * (2 * ks[:, None] + 1) * n[None, :] / (2 * C)
        F = np.stack([np.cos(th).reshape(8, 8, C), -np.sin(th).reshape(8, 8, C)], axis=1).reshape(128, C)
        Fs.append(F)
        Gs.append(F.T / C)
    return np.stack(Fs).astype(bf16), np.stack(Gs).astype(bf16)


def _kernel(x_h, c_h, wq_h, wk_h, wv_h, wo_h, k_h, v_h, h_h,
            skt_h, dd_h, gw_h, f_h, g_h,
            o_h,
            skt_ref, dd_ref, gw_ref, f_ref, g_ref,
            x_v, c_v, w_l, w_0, w_st, wq_b, wk_b, wv_b, wo_l,
            kv_l, ht_l, acc, xg_s, out_v, q_s, k_s, v_s, ctx_s, gate_s, par_s, ub_s,
            V_s, H_s, W_s, s_a, s_b, sems):
    s_s = (s_a, s_b)
    kt_l, vt_l = kv_l.at[0], kv_l.at[1]
    step = pl.program_id(0)
    P = functools.partial
    wsets = ((wq_h, wq_b, M, 0), (wk_h, wk_b, DC, M), (wv_h, wv_b, DC, M + DC))

    def pair_copies(n, land, sem):
        h0 = pl.multiple_of(n * HP, HP)
        return [pltpu.make_async_copy(wh.at[:, j, pl.ds(h0, HP), :],
                                      land.at[off // 4:(off + rows) // 4, HP * j:HP * (j + 1), :], sems.at[sem])
                for (wh, wb, rows, off) in wsets for j in range(4)]

    def late_copies(n):
        return ([pltpu.make_async_copy(wo_h.at[pl.ds(pl.multiple_of(n * 256, 256), 256), :], wo_l, sems.at[SEM_WO])]
                + pair_copies(jnp.minimum(n + 1, NSTEP - 1), w_l, SEM_W))

    def late_wait():
        pltpu.make_async_copy(wo_l, wo_l, sems.at[SEM_WO]).wait()
        pltpu.make_async_copy(w_l, w_l, sems.at[SEM_W]).wait()

    def early_copies(n):
        col = pl.multiple_of((jnp.minimum(n, NSTEP - 1) // 2) * 128, 128)
        return [pltpu.make_async_copy(k_h.at[:, pl.ds(col, 128)], kt_l, sems.at[SEM_KV]),
                pltpu.make_async_copy(v_h.at[:, pl.ds(col, 128)], vt_l, sems.at[SEM_KV]),
                pltpu.make_async_copy(h_h.at[pl.ds(col, 128), :], ht_l, sems.at[SEM_HT])]

    def early_wait():
        pltpu.make_async_copy(kv_l, kv_l, sems.at[SEM_KV]).wait()
        pltpu.make_async_copy(ht_l, ht_l, sems.at[SEM_HT]).wait()

    def c_copy(p):
        a, b = (0, NP0 * BQ) if p == 0 else (NP0 * BQ, S)
        return pltpu.make_async_copy(c_h.at[a:b, :], c_v.at[a:b, :], sems.at[SEM_C + p])

    def x_copy(i):
        rs = pl.ds(i * BQ, BQ) if isinstance(i, int) else pl.ds(pl.multiple_of(i * BQ, BQ), BQ)
        return pltpu.make_async_copy(x_h.at[rs, :], x_v.at[rs, :], sems.at[SEM_X + i])

    def out_copy(r0, r1, c0, c1):
        return pltpu.make_async_copy(out_v.at[r0:r1, c0:c1], o_h.at[r0:r1, c0:c1], sems.at[SEM_OUT])

    def gate_blocks(lo, hi):
        def f(i, c):
            x_copy(i).wait()
            rs = pl.ds(pl.multiple_of(i * BQ, BQ), BQ)
            xf = x_v[rs, :].astype(f32)
            z = jnp.sum(xf * par_s[5:6, :], axis=1, keepdims=True)
            g = jax.nn.sigmoid(z)
            gate_s[rs, :] = jnp.broadcast_to(g, (BQ, 128))
            xg_s[rs, XO:XO + M] = (1.0 - g) * xf
            return c
        jax.lax.fori_loop(lo, hi, f, 0)

    @pl.when(step == 0)
    def _():
        w0 = pair_copies(step, w_0, SEM_W0)
        sm = [pltpu.make_async_copy(a, b, sems.at[SEM_SM + n]) for n, (a, b) in enumerate(
            ((skt_h, skt_ref), (dd_h, dd_ref), (gw_h, gw_ref), (f_h, f_ref), (g_h, g_ref)))]
        for cp in (w0 + sm + [x_copy(i) for i in range(NP0)] + [c_copy(0)] + early_copies(step)
                   + [x_copy(i) for i in range(NP0, NB)] + [c_copy(1)] + late_copies(step)):
            cp.start()

        def zero(i, c):
            rs = pl.ds(pl.multiple_of(i * 64, 64), 64)
            acc[rs, :] = jnp.zeros((64, M), f32)
            return c
        jax.lax.fori_loop(0, S // 64, zero, 0)
        for cp in sm:
            cp.wait()
        par_s[0:4, :] = skt_ref[...].astype(f32)
        par_s[4:5, :] = dd_ref[...].astype(f32).reshape(1, M)
        par_s[5:6, :] = gw_ref[...].astype(f32).reshape(1, M)
        par_s[6:8, :] = jnp.zeros((2, M), f32)
        pltpu.make_async_copy(w_0, w_0, sems.at[SEM_W0]).wait()
        w_st[0:2 * WR, :] = w_0[...].astype(f32).reshape(2 * WR, D)
        for (wh, wb, rows, off) in wsets:
            wb[...] = jnp.concatenate(
                [w_st[pl.ds(2 * off + hh, rows, stride=2), :] for hh in range(HP)], axis=1).astype(bf16)
        gate_blocks(0, NP0)
        c_copy(0).wait()

    early_wait()

    ct = step // 2
    half = step % 2
    ccol = pl.ds(pl.multiple_of(ct * 128, 128), 128)
    scale = (D ** -0.5) * LOG2E
    row = jax.lax.broadcasted_iota(jnp.int32, (128, 128), 0)
    col = jax.lax.broadcasted_iota(jnp.int32, (128, 128), 1)
    mask = col <= row
    never8 = f_ref[0, 0:8, :].astype(f32) > 2.0
    never = jnp.concatenate([never8] * 16, axis=0)

    side = collections.deque()
    budget = [0.0]
    lim = [32]

    def pin(arr, spacing):
        R = arr.shape[0]
        out, lastr = [], 0
        for g in range(min(R // 8, lim[0])):
            budget[0] = min(budget[0] + RATE * spacing, 80.0)
            if side and budget[0] >= side[0][0]:
                cost, fn = side.popleft()
                budget[0] -= cost
                v = fn()
                if g * 8 > lastr:
                    out.append(arr[lastr:g * 8])
                out.append(jnp.where(never8, v, arr[g * 8:(g + 1) * 8]))
                lastr = (g + 1) * 8
        if lastr == 0:
            return arr
        if lastr < R:
            out.append(arr[lastr:])
        return jnp.concatenate(out, axis=0)

    def flush():
        while side:
            side.popleft()[1]()

    def pq(i, hh):
        r0, r1 = i * BQ, (i + 1) * BQ
        hs = slice(hh * D, (hh + 1) * D)
        r = jnp.dot(x_v[r0:r1, :], wq_b[:, hs], preferred_element_type=f32)
        q_s[r0:r1, hs] = (pin(r, 8) * scale).astype(bf16)

    def pk(i, hh):
        r0, r1 = i * BQ, (i + 1) * BQ
        hs = slice(hh * D, (hh + 1) * D)
        r = jnp.dot(c_v[r0:r1, :], wk_b[:, hs], preferred_element_type=f32)
        k_s[r0:r1, hs] = pin(r, 8).astype(bf16)

    def pvv(i, hh):
        r0, r1 = i * BQ, (i + 1) * BQ
        hs = slice(hh * D, (hh + 1) * D)
        r = jnp.dot(c_v[r0:r1, :], wv_b[:, hs], preferred_element_type=f32)
        v_s[r0:r1, hs] = pin(r, 8).astype(bf16)

    def chunks(i):
        nt = 2 * i + 1
        out, t = [], 0
        while t < nt:
            n = min(KC, nt - t)
            out.append((0, t * 128, (t + n) * 128))
            t += n
        out.append((128, nt * 128, (nt + 1) * 128))
        return out

    st = {}

    def qk_atom(i, hh, ch):
        rl, kl, kh = ch
        r0 = i * BQ
        hs = slice(hh * D, (hh + 1) * D)
        s = jax.lax.dot_general(q_s[r0 + rl:r0 + BQ, hs], k_s[kl:kh, hs], NT, preferred_element_type=f32)
        nt = (kh - kl) // 128
        tiles = [s[:, t * 128:(t + 1) * 128] for t in range(nt)]
        if kh > r0 + rl:
            d = tiles[-1]
            dm = jnp.where(mask, d[:128], -1e30)
            tiles[-1] = dm if rl == 128 else jnp.concatenate([dm, d[128:]], axis=0)
        u = st.setdefault((i, hh), {"m": [None, None], "l": [None, None], "o": [None, None]})
        for t in range(nt):
            s_s[hh][rl:BQ, kl + t * 128:kl + (t + 1) * 128] = tiles[t]
        mm = functools.reduce(jnp.maximum, tiles)
        for g in range(rl // 128, 2):
            a = mm[g * 128 - rl:(g + 1) * 128 - rl]
            u["m"][g] = a if u["m"][g] is None else jnp.maximum(u["m"][g], a)

    def qk(i, hh, sel=None):
        chs = chunks(i)
        if sel == "head":
            for ch in chs[:-2]:
                qk_atom(i, hh, ch)
            return
        for ch in (chs[-2:] if sel == "tail" else chs):
            qk_atom(i, hh, ch)
        u = st[(i, hh)]
        mx = [jnp.broadcast_to(jnp.max(u["m"][g], axis=1, keepdims=True), (128, 128)) for g in range(2)]
        s_s[hh][0:BQ, S:S + 128] = jnp.concatenate(mx, axis=0)
        s_s[hh][pl.ds(pl.multiple_of(BQ + (step >> 8) * 8, 8), 8), 0:128] = u["m"][1][120:128]
        s_s[hh][pl.ds(pl.multiple_of(BQ + (step >> 8) * 8, 8), 8), S:S + 128] = u["m"][1][120:128]

    def pv_atom(i, hh, ch):
        rl, kl, kh = ch
        hs = slice(hh * D, (hh + 1) * D)
        u = st[(i, hh)]
        m = s_s[hh][rl:BQ, S:S + 128]
        ps = [jnp.exp2(s_s[hh][rl:BQ, k0:k0 + 128] - m) for k0 in range(kl, kh, 128)]
        lp = functools.reduce(jnp.add, ps)
        ls = []
        for g in range(rl // 128, 2):
            a = lp[g * 128 - rl:(g + 1) * 128 - rl]
            u["l"][g] = a if u["l"][g] is None else u["l"][g] + a
            ls.append(u["l"][g])
        ps[-1] = jnp.minimum(ps[-1], jnp.concatenate(ls, axis=0) if len(ls) > 1 else ls[0])
        pb = (jnp.concatenate(ps, axis=1) if len(ps) > 1 else ps[0]).astype(bf16)
        o = jnp.dot(pb, v_s[kl:kh, hs], preferred_element_type=f32)
        for g in range(rl // 128, 2):
            a = o[g * 128 - rl:(g + 1) * 128 - rl]
            u["o"][g] = a if u["o"][g] is None else u["o"][g] + a

    def recip(l):
        r = pl.reciprocal(l, approx=True)
        return r * (2.0 - l * r)

    def norm_piece(i, hh, g, r):
        u = st[(i, hh)]
        hs = slice(hh * D, (hh + 1) * D)
        o = u["o"][g][r:r + 16]
        r0 = i * BQ + g * 128 + r
        c = o * (gate_s[r0:r0 + 16, :] * recip(u["L"][g][r:r + 16]))
        ctx_s[i, g * 128 + r:g * 128 + r + 16, hs] = c.astype(bf16)
        return jnp.maximum(c[:8], c[8:])

    def pv(i, hh, defer):
        for ch in chunks(i):
            pv_atom(i, hh, ch)
        u = st[(i, hh)]
        u["L"] = [jnp.sum(jnp.where(never, u["o"][g], u["l"][g]), axis=1, keepdims=True) for g in range(2)]
        pieces = [(32, P(norm_piece, i, hh, g, r)) for g in range(2) for r in range(0, 128, 16)]
        if defer:
            side.extendleft(reversed(pieces))
            u["left"] = len(side) - len(pieces)
        else:
            for _, fn in pieces:
                fn()

    def oproj(i, atoms=(0, 1, 2, 3), lastlim=32):
        r0, r1 = i * BQ, (i + 1) * BQ
        for a in atoms:
            lim[0] = lastlim if a == atoms[-1] else 32
            cs = slice(a * 256, (a + 1) * 256)
            r = jnp.dot(ctx_s[i], wo_l[:, cs], preferred_element_type=f32)
            r = jnp.concatenate([pin(r[:, :128], 8), r[:, 128:]], axis=1)
            r = acc[r0:r1, cs] + r
            acc[r0:r1, cs] = r
            out_v[r0:r1, cs] = r.astype(bf16)
            if i == NB - 1 and a < 3:
                @pl.when(step == NSTEP - 1)
                def _():
                    out_copy(r0, r1, a * 256, (a + 1) * 256).start()
        lim[0] = 32
        if atoms[-1] == 3 and i < NB - 1:
            @pl.when(step == NSTEP - 1)
            def _():
                out_copy(r0, r1, 0, M - 128).start()

    cv = {}

    def u_piece(r):
        j = r // C
        par = cv["par"]
        if r == 0:
            kf = jnp.concatenate([jnp.zeros((8, 128), f32), kt_l[0:16, :].astype(f32)], axis=0)
        else:
            kf = kt_l[r - 16:r + 16, :].astype(f32)[8:]
        ks = kf[8:] * par[0:1]
        for t in range(1, 4):
            ks = ks + kf[8 - t:24 - t] * par[t:t + 1]
        u = ks * vt_l[r:r + 16, :].astype(f32)
        ub_s[r - j * C:r - j * C + 16, j * 128:(j + 1) * 128] = u.astype(bf16)
        return jnp.maximum(u[:8], u[8:])

    def split(T, j):
        t = T[:, j * 128:(j + 1) * 128]
        re = jnp.concatenate([t[16 * g:16 * g + 8] for g in range(8)], axis=0)
        im = jnp.concatenate([t[16 * g + 8:16 * g + 16] for g in range(8)], axis=0)
        return re, im

    def fwdu(hf):
        lo, hi = hf * NCH // 2, (hf + 1) * NCH // 2
        U = jnp.dot(f_ref[half], ub_s[:, lo * 128:hi * 128], preferred_element_type=f32)
        for j in range(lo, hi):
            re, im = split(U, j - lo)
            V_s[0, j] = re
            V_s[1, j] = im
            V_s[2, j] = re + im

    def fwdh(hf):
        lo, hi = hf * NCH // 2, (hf + 1) * NCH // 2
        hcat = jnp.concatenate([ht_l[:, j * C:(j + 1) * C] for j in range(lo, hi)], axis=0)
        Hf = jax.lax.dot_general(f_ref[half], hcat, NT, preferred_element_type=f32)
        for j in range(lo, hi):
            re, im = split(Hf, j - lo)
            if j == 0:
                re = re + cv["par"][4:5]
            H_s[0, j] = im - re
            H_s[1, j] = re + im
            H_s[2, j] = re

    def mac_piece(i, r, a):
        rs = slice(r, r + 8)
        s = functools.reduce(jnp.add, [H_s[a, i - j, rs, :] * V_s[a, j, rs, :] for j in range(i + 1)])
        cv[a] = s
        if a == 2:
            yr, yi = s - cv[1], s + cv[0]
            wr, wi = yr, yi
            if i > 0:
                pr, pi = cv[("y", r)]
                wr, wi = (yr - pi, yi + pr) if r < 32 else (yr + pi, yi - pr)
            cv[("y", r)] = (yr, yi)
            W_s[2 * r:2 * r + 16, i * 128:(i + 1) * 128] = jnp.concatenate([wr, wi], axis=0).astype(bf16)
        return s

    def inv(hf):
        lo, hi = hf * NCH // 2, (hf + 1) * NCH // 2
        Y = jnp.dot(g_ref[half], W_s[:, lo * 128:hi * 128], preferred_element_type=f32)
        for j in range(lo, hi):
            a, b = j * C, (j + 1) * C
            y = Y[:, (j - lo) * 128:(j - lo + 1) * 128]
            acc[a:b, ccol] += xg_s[a:b, pl.ds(pl.multiple_of(ct * 128 + XO, 128), 128)] * y

    def stage_piece(t0):
        w = w_l[t0:t0 + 4].astype(f32).reshape(32, D)
        w_st[t0 * 8:t0 * 8 + 32, :] = w
        return functools.reduce(jnp.maximum, [w[k * 8:(k + 1) * 8] for k in range(4)])

    def extract_piece(wb, off, m0):
        ws = [w_st[pl.ds(2 * (off + m0) + hh, 8, stride=2), :] for hh in range(HP)]
        wb[m0:m0 + 8, :] = jnp.concatenate(ws, axis=1).astype(bf16)
        return ws[0]

    units = [(u // 2, u % 2) for u in range(NU)]

    cv["par"] = par_s[:, ccol]
    for r in range(0, S, 16):
        side.append((40, P(u_piece, r)))
    pq(0, 0); pk(0, 0); pq(0, 1); pk(0, 1)
    qk(0, 0)
    pvv(0, 0); pvv(0, 1)
    fwdh(0); fwdh(1)
    odone = 0
    for s in range(NU):
        i, hh = units[s]
        if s == FW:
            flush()
            fwdu(0); fwdu(1)
            for cp in early_copies(step + 1):
                cp.start()

            @pl.when(step == 0)
            def _():
                gate_blocks(NP0, NB)
                c_copy(1).wait()
            late_wait()
            qk(i, hh, "tail")
            for i2 in range(NCH):
                for r in range(0, 64, 8):
                    for a in range(3):
                        side.append((MACW * (2 * (i2 + 1) + 3), P(mac_piece, i2, r, a)))
            for t0 in range(0, WR // 4, 4):
                side.append((12, P(stage_piece, t0)))
        if s == NU - 2:
            flush()
            for (wh, wb, rows, off) in wsets:
                for m0 in range(0, rows, 8):
                    side.append((8, P(extract_piece, wb, off, m0)))
        do_o = s >= FW and odone < i and s < NU - 2
        if i + 1 < NB:
            pk(i + 1, hh); pq(i + 1, hh)
            if not do_o:
                lim[0] = LL
            pvv(i + 1, hh)
            lim[0] = 32
            if s >= 1 and "left" in st[units[s - 1]]:
                assert len(side) <= st[units[s - 1]]["left"]
        if do_o:
            oproj(odone, lastlim=LL)
            odone += 1
        if s == NU - 2:
            oproj(NB - 2, (0, 1))
        if s == NU - 1:
            oproj(NB - 2, (2, 3))
        pv(i, hh, s + 1 < NU - 2 and s + 1 != FW)
        if s + 1 < NU:
            qk(*units[s + 1], "head" if s + 1 == FW else None)
    inv(0); inv(1)
    assert odone == NB - 2
    oproj(NB - 1)
    flush()

    @pl.when(step < NSTEP - 1)
    def _():
        for cp in late_copies(step + 1):
            cp.start()

    @pl.when(step == NSTEP - 1)
    def _():
        r7 = (NB - 1) * BQ
        out_copy(r7, S, 768, M).start()
        for a, b in ((0, 512), (512, 1024), (1024, r7)):
            out_v[a:b, M - 128:M] = acc[a:b, M - 128:M].astype(bf16)
            out_copy(a, b, M - 128, M).start()
        early_wait()
        pltpu.make_async_copy(out_v, o_h, sems.at[SEM_OUT]).wait()


@jax.jit
def pallas_gated_mix__compressed_kv_cla__ssm_conv_h3__prompt_kernel(
    A_x: jax.Array,
    A_c_kv: jax.Array,
    A_w_q: jax.Array,
    A_w_uk: jax.Array,
    A_w_uv: jax.Array,
    A_w_o: jax.Array,
    B_q: jax.Array,
    B_k: jax.Array,
    B_v: jax.Array,
    B_shift_k: jax.Array,
    B_ssm_k: jax.Array,
    B_ssm_D: jax.Array,
    gate_w: jax.Array,
):
    del B_q
    Fc, Gc = _dft_consts()
    hbm = pl.BlockSpec(memory_space=pl.ANY)
    scratch = [
        pltpu.VMEM((4, M), bf16),
        pltpu.VMEM((M,), bf16),
        pltpu.VMEM((M,), bf16),
        pltpu.VMEM((2, 128, C), bf16),
        pltpu.VMEM((2, C, 128), bf16),
        pltpu.VMEM((S, M), bf16),
        pltpu.VMEM((S, DC), bf16),
        pltpu.VMEM((WR // 4, 8, D), bf16),
        pltpu.VMEM((WR // 4, 8, D), bf16),
        pltpu.VMEM((2 * WR + 8, D), f32),
        pltpu.VMEM((M, HP * D), bf16),
        pltpu.VMEM((DC, HP * D), bf16),
        pltpu.VMEM((DC, HP * D), bf16),
        pltpu.VMEM((HP * D, M), bf16),
        pltpu.VMEM((2, S, 128), bf16),
        pltpu.VMEM((128, S), bf16),
        pltpu.VMEM((S, M), f32),
        pltpu.VMEM((S, M + 512), f32),
        pltpu.VMEM((S, M), bf16),
        pltpu.VMEM((S, HP * D), bf16),
        pltpu.VMEM((S, HP * D), bf16),
        pltpu.VMEM((S, HP * D), bf16),
        pltpu.VMEM((NB, BQ, HP * D), bf16),
        pltpu.VMEM((S, 128), f32),
        pltpu.VMEM((8, M), f32),
        pltpu.VMEM((C, NCH * 128), bf16),
        pltpu.VMEM((3, NCH, 64, 128), f32),
        pltpu.VMEM((3, NCH, 64, 128), f32),
        pltpu.VMEM((128, NCH * 128), bf16),
        pltpu.VMEM((BQ + 8, S + 128), f32),
        pltpu.VMEM((BQ + 8, S + 128), f32),
        pltpu.SemaphoreType.DMA((NSEM,)),
    ]
    out = pl.pallas_call(
        _kernel,
        out_shape=jax.ShapeDtypeStruct((S, M), bf16),
        grid=(NSTEP,),
        in_specs=[hbm] * 14,
        out_specs=hbm,
        scratch_shapes=scratch,
        compiler_params=pltpu.CompilerParams(
            vmem_limit_bytes=100 * 1024 * 1024,
            dimension_semantics=("arbitrary",),
            disable_bounds_checks=True),
    )(A_x.reshape(S, M), A_c_kv.reshape(S, DC),
      A_w_q.reshape(M // 4, 4, H, D), A_w_uk.reshape(DC // 4, 4, H, D), A_w_uv.reshape(DC // 4, 4, H, D),
      A_w_o.reshape(H * D, M), B_k.reshape(S, M), B_v.reshape(S, M), B_ssm_k,
      B_shift_k.T, B_ssm_D, gate_w, jnp.asarray(Fc), jnp.asarray(Gc))
    return out.reshape(1, S, M)
```

```python
import collections
import functools

import numpy as np
import jax
import jax.numpy as jnp
import jax.experimental.pallas as pl
import jax.experimental.pallas.tpu as pltpu

f32, bf16 = jnp.float32, jnp.bfloat16
NT = (((1,), (1,)), ((), ()))

S = 2048
M = 1024
DC = 512
H = 32
D = 128
HP = 2
NSTEP = H // HP
BQ = 256
NB = S // BQ
NU = 2 * NB
C = 128
NCH = S // C
WR = M + 2 * DC
LOG2E = 1.4426950408889634

XO = 256
KC = 4
RATE = 2.0
MACW = 2.0
FW = 4
NP0 = (FW - 1) // 2 + 2
LL = 16

SEM_W, SEM_WO, SEM_KV, SEM_HT, SEM_W0, SEM_OUT = range(6)
SEM_C = 6
SEM_SM = 8
SEM_X = 13
NSEM = SEM_X + NB


def _dft_consts():
    n = np.arange(C)
    Fs, Gs = [], []
    for p in range(2):
        ks = np.arange(p * 64, (p + 1) * 64)
        ks = np.concatenate([ks[ks % 2 == 0], ks[ks % 2 == 1]])
        th = np.pi * (2 * ks[:, None] + 1) * n[None, :] / (2 * C)
        F = np.stack([np.cos(th).reshape(8, 8, C), -np.sin(th).reshape(8, 8, C)], axis=1).reshape(128, C)
        Fs.append(F)
        Gs.append(F.T / C)
    return np.stack(Fs).astype(bf16), np.stack(Gs).astype(bf16)


def _kernel(x_h, c_h, wq_h, wk_h, wv_h, wo_h, k_h, v_h, h_h,
            skt_h, dd_h, gw_h, f_h, g_h,
            o_h,
            skt_ref, dd_ref, gw_ref, f_ref, g_ref,
            x_v, c_v, w_l, w_0, w_st, wq_b, wk_b, wv_b, wo_l,
            kv_l, ht_l, acc, xg_s, out_v, q_s, k_s, v_s, ctx_s, gate_s, par_s, ub_s,
            V_s, H_s, W_s, s_a, s_b, sems):
    s_s = (s_a, s_b)
    kt_l, vt_l = kv_l.at[0], kv_l.at[1]
    step = pl.program_id(0)
    P = functools.partial
    wsets = ((wq_h, wq_b, M, 0), (wk_h, wk_b, DC, M), (wv_h, wv_b, DC, M + DC))

    def pair_copies(n, land, sem):
        h0 = pl.multiple_of(n * HP, HP)
        return [pltpu.make_async_copy(wh.at[:, j, pl.ds(h0, HP), :],
                                      land.at[off // 4:(off + rows) // 4, HP * j:HP * (j + 1), :], sems.at[sem])
                for (wh, wb, rows, off) in wsets for j in range(4)]

    def late_copies(n):
        return ([pltpu.make_async_copy(wo_h.at[pl.ds(pl.multiple_of(n * 256, 256), 256), :], wo_l, sems.at[SEM_WO])]
                + pair_copies(jnp.minimum(n + 1, NSTEP - 1), w_l, SEM_W))

    def late_wait():
        pltpu.make_async_copy(wo_l, wo_l, sems.at[SEM_WO]).wait()
        pltpu.make_async_copy(w_l, w_l, sems.at[SEM_W]).wait()

    def early_copies(n):
        col = pl.multiple_of((jnp.minimum(n, NSTEP - 1) // 2) * 128, 128)
        return [pltpu.make_async_copy(k_h.at[:, pl.ds(col, 128)], kt_l, sems.at[SEM_KV]),
                pltpu.make_async_copy(v_h.at[:, pl.ds(col, 128)], vt_l, sems.at[SEM_KV]),
                pltpu.make_async_copy(h_h.at[pl.ds(col, 128), :], ht_l, sems.at[SEM_HT])]

    def early_wait():
        pltpu.make_async_copy(kv_l, kv_l, sems.at[SEM_KV]).wait()
        pltpu.make_async_copy(ht_l, ht_l, sems.at[SEM_HT]).wait()

    def c_copy(p):
        a, b = (0, NP0 * BQ) if p == 0 else (NP0 * BQ, S)
        return pltpu.make_async_copy(c_h.at[a:b, :], c_v.at[a:b, :], sems.at[SEM_C + p])

    def x_copy(i):
        rs = pl.ds(i * BQ, BQ) if isinstance(i, int) else pl.ds(pl.multiple_of(i * BQ, BQ), BQ)
        return pltpu.make_async_copy(x_h.at[rs, :], x_v.at[rs, :], sems.at[SEM_X + i])

    def out_copy(r0, r1, c0, c1):
        return pltpu.make_async_copy(out_v.at[r0:r1, c0:c1], o_h.at[r0:r1, c0:c1], sems.at[SEM_OUT])

    def gate_blocks(lo, hi):
        def f(i, c):
            x_copy(i).wait()
            rs = pl.ds(pl.multiple_of(i * BQ, BQ), BQ)
            xf = x_v[rs, :].astype(f32)
            z = jnp.sum(xf * par_s[5:6, :], axis=1, keepdims=True)
            g = jax.nn.sigmoid(z)
            gate_s[rs, :] = jnp.broadcast_to(g, (BQ, 128))
            xg_s[rs, XO:XO + M] = (1.0 - g) * xf
            return c
        jax.lax.fori_loop(lo, hi, f, 0)

    @pl.when(step == 0)
    def _():
        w0 = pair_copies(step, w_0, SEM_W0)
        sm = [pltpu.make_async_copy(a, b, sems.at[SEM_SM + n]) for n, (a, b) in enumerate(
            ((skt_h, skt_ref), (dd_h, dd_ref), (gw_h, gw_ref), (f_h, f_ref), (g_h, g_ref)))]
        for cp in (w0 + sm + [x_copy(i) for i in range(NP0)] + [c_copy(0)] + early_copies(step)
                   + [x_copy(i) for i in range(NP0, NB)] + [c_copy(1)] + late_copies(step)):
            cp.start()

        def zero(i, c):
            rs = pl.ds(pl.multiple_of(i * 64, 64), 64)
            acc[rs, :] = jnp.zeros((64, M), f32)
            return c
        jax.lax.fori_loop(0, S // 64, zero, 0)
        for cp in sm:
            cp.wait()
        par_s[0:4, :] = skt_ref[...].astype(f32)
        par_s[4:5, :] = dd_ref[...].astype(f32).reshape(1, M)
        par_s[5:6, :] = gw_ref[...].astype(f32).reshape(1, M)
        par_s[6:8, :] = jnp.zeros((2, M), f32)
        pltpu.make_async_copy(w_0, w_0, sems.at[SEM_W0]).wait()
        w_st[0:2 * WR, :] = w_0[...].astype(f32).reshape(2 * WR, D)
        for (wh, wb, rows, off) in wsets:
            wb[...] = jnp.concatenate(
                [w_st[pl.ds(2 * off + hh, rows, stride=2), :] for hh in range(HP)], axis=1).astype(bf16)
        gate_blocks(0, NP0)
        c_copy(0).wait()

    early_wait()

    ct = step // 2
    half = step % 2
    ccol = pl.ds(pl.multiple_of(ct * 128, 128), 128)
    scale = (D ** -0.5) * LOG2E
    row = jax.lax.broadcasted_iota(jnp.int32, (128, 128), 0)
    col = jax.lax.broadcasted_iota(jnp.int32, (128, 128), 1)
    mask = col <= row
    never8 = f_ref[0, 0:8, :].astype(f32) > 2.0
    never = jnp.concatenate([never8] * 16, axis=0)

    side = collections.deque()
    budget = [0.0]
    lim = [32]

    def pin(arr, spacing):
        R = arr.shape[0]
        out, lastr = [], 0
        for g in range(min(R // 8, lim[0])):
            budget[0] = min(budget[0] + RATE * spacing, 80.0)
            if side and budget[0] >= side[0][0]:
                cost, fn = side.popleft()
                budget[0] -= cost
                v = fn()
                if g * 8 > lastr:
                    out.append(arr[lastr:g * 8])
                out.append(jnp.where(never8, v, arr[g * 8:(g + 1) * 8]))
                lastr = (g + 1) * 8
        if lastr == 0:
            return arr
        if lastr < R:
            out.append(arr[lastr:])
        return jnp.concatenate(out, axis=0)

    def flush():
        while side:
            side.popleft()[1]()

    def pq(i, hh):
        r0, r1 = i * BQ, (i + 1) * BQ
        hs = slice(hh * D, (hh + 1) * D)
        r = jnp.dot(x_v[r0:r1, :], wq_b[:, hs], preferred_element_type=f32)
        q_s[r0:r1, hs] = (pin(r, 8) * scale).astype(bf16)

    def pk(i, hh):
        r0, r1 = i * BQ, (i + 1) * BQ
        hs = slice(hh * D, (hh + 1) * D)
        r = jnp.dot(c_v[r0:r1, :], wk_b[:, hs], preferred_element_type=f32)
        k_s[r0:r1, hs] = pin(r, 8).astype(bf16)

    def pvv(i, hh):
        r0, r1 = i * BQ, (i + 1) * BQ
        hs = slice(hh * D, (hh + 1) * D)
        r = jnp.dot(c_v[r0:r1, :], wv_b[:, hs], preferred_element_type=f32)
        v_s[r0:r1, hs] = pin(r, 8).astype(bf16)

    def chunks(i):
        nt = 2 * i + 1
        out, t = [], 0
        while t < nt:
            n = min(KC, nt - t)
            out.append((0, t * 128, (t + n) * 128))
            t += n
        out.append((128, nt * 128, (nt + 1) * 128))
        return out

    st = {}

    def qk_atom(i, hh, ch):
        rl, kl, kh = ch
        r0 = i * BQ
        hs = slice(hh * D, (hh + 1) * D)
        s = jax.lax.dot_general(q_s[r0 + rl:r0 + BQ, hs], k_s[kl:kh, hs], NT, preferred_element_type=f32)
        nt = (kh - kl) // 128
        tiles = [s[:, t * 128:(t + 1) * 128] for t in range(nt)]
        if kh > r0 + rl:
            d = tiles[-1]
            dm = jnp.where(mask, d[:128], -1e30)
            tiles[-1] = dm if rl == 128 else jnp.concatenate([dm, d[128:]], axis=0)
        u = st.setdefault((i, hh), {"m": [None, None], "l": [None, None], "o": [None, None]})
        for t in range(nt):
            s_s[hh][rl:BQ, kl + t * 128:kl + (t + 1) * 128] = tiles[t]
        mm = functools.reduce(jnp.maximum, tiles)
        for g in range(rl // 128, 2):
            a = mm[g * 128 - rl:(g + 1) * 128 - rl]
            u["m"][g] = a if u["m"][g] is None else jnp.maximum(u["m"][g], a)

    def qk(i, hh, sel=None):
        chs = chunks(i)
        if sel == "head":
            for ch in chs[:-2]:
                qk_atom(i, hh, ch)
            return
        for ch in (chs[-2:] if sel == "tail" else chs):
            qk_atom(i, hh, ch)
        u = st[(i, hh)]
        mx = [jnp.broadcast_to(jnp.max(u["m"][g], axis=1, keepdims=True), (128, 128)) for g in range(2)]
        s_s[hh][0:BQ, S:S + 128] = jnp.concatenate(mx, axis=0)
        s_s[hh][pl.ds(pl.multiple_of(BQ + (step >> 8) * 8, 8), 8), 0:128] = u["m"][1][120:128]
        s_s[hh][pl.ds(pl.multiple_of(BQ + (step >> 8) * 8, 8), 8), S:S + 128] = u["m"][1][120:128]

    def pv_atom(i, hh, ch):
        rl, kl, kh = ch
        hs = slice(hh * D, (hh + 1) * D)
        u = st[(i, hh)]
        m = s_s[hh][rl:BQ, S:S + 128]
        ps = [jnp.exp2(s_s[hh][rl:BQ, k0:k0 + 128] - m) for k0 in range(kl, kh, 128)]
        lp = functools.reduce(jnp.add, ps)
        ls = []
        for g in range(rl // 128, 2):
            a = lp[g * 128 - rl:(g + 1) * 128 - rl]
            u["l"][g] = a if u["l"][g] is None else u["l"][g] + a
            ls.append(u["l"][g])
        ps[-1] = jnp.minimum(ps[-1], jnp.concatenate(ls, axis=0) if len(ls) > 1 else ls[0])
        pb = (jnp.concatenate(ps, axis=1) if len(ps) > 1 else ps[0]).astype(bf16)
        o = jnp.dot(pb, v_s[kl:kh, hs], preferred_element_type=f32)
        for g in range(rl // 128, 2):
            a = o[g * 128 - rl:(g + 1) * 128 - rl]
            u["o"][g] = a if u["o"][g] is None else u["o"][g] + a

    def recip(l):
        r = pl.reciprocal(l, approx=True)
        return r * (2.0 - l * r)

    def norm_piece(i, hh, g, r):
        u = st[(i, hh)]
        hs = slice(hh * D, (hh + 1) * D)
        o = u["o"][g][r:r + 16]
        r0 = i * BQ + g * 128 + r
        c = o * (gate_s[r0:r0 + 16, :] * recip(u["L"][g][r:r + 16]))
        ctx_s[i, g * 128 + r:g * 128 + r + 16, hs] = c.astype(bf16)
        return jnp.maximum(c[:8], c[8:])

    def pv(i, hh, defer):
        for ch in chunks(i):
            pv_atom(i, hh, ch)
        u = st[(i, hh)]
        u["L"] = [jnp.sum(jnp.where(never, u["o"][g], u["l"][g]), axis=1, keepdims=True) for g in range(2)]
        pieces = [(32, P(norm_piece, i, hh, g, r)) for g in range(2) for r in range(0, 128, 16)]
        if defer:
            side.extendleft(reversed(pieces))
            u["left"] = len(side) - len(pieces)
        else:
            for _, fn in pieces:
                fn()

    def oproj(i, atoms=(0, 1, 2, 3), lastlim=32):
        r0, r1 = i * BQ, (i + 1) * BQ
        for a in atoms:
            lim[0] = lastlim if a == atoms[-1] else 32
            cs = slice(a * 256, (a + 1) * 256)
            r = jnp.dot(ctx_s[i], wo_l[:, cs], preferred_element_type=f32)
            r = jnp.concatenate([pin(r[:, :128], 8), r[:, 128:]], axis=1)
            r = acc[r0:r1, cs] + r
            acc[r0:r1, cs] = r
            out_v[r0:r1, cs] = r.astype(bf16)
            if i == NB - 1 and a < 3:
                @pl.when(step == NSTEP - 1)
                def _():
                    out_copy(r0, r1, a * 256, (a + 1) * 256).start()
        lim[0] = 32
        if atoms[-1] == 3 and i < NB - 1:
            @pl.when(step == NSTEP - 1)
            def _():
                out_copy(r0, r1, 0, M - 128).start()

    cv = {}

    def u_piece(r):
        j = r // C
        par = cv["par"]
        if r == 0:
            kf = jnp.concatenate([jnp.zeros((8, 128), f32), kt_l[0:16, :].astype(f32)], axis=0)
        else:
            kf = kt_l[r - 16:r + 16, :].astype(f32)[8:]
        ks = kf[8:] * par[0:1]
        for t in range(1, 4):
            ks = ks + kf[8 - t:24 - t] * par[t:t + 1]
        u = ks * vt_l[r:r + 16, :].astype(f32)
        ub_s[r - j * C:r - j * C + 16, j * 128:(j + 1) * 128] = u.astype(bf16)
        return jnp.maximum(u[:8], u[8:])

    def split(T, j):
        t = T[:, j * 128:(j + 1) * 128]
        re = jnp.concatenate([t[16 * g:16 * g + 8] for g in range(8)], axis=0)
        im = jnp.concatenate([t[16 * g + 8:16 * g + 16] for g in range(8)], axis=0)
        return re, im

    def fwdu(hf):
        lo, hi = hf * NCH // 2, (hf + 1) * NCH // 2
        U = jnp.dot(f_ref[half], ub_s[:, lo * 128:hi * 128], preferred_element_type=f32)
        for j in range(lo, hi):
            re, im = split(U, j - lo)
            V_s[0, j] = re
            V_s[1, j] = im
            V_s[2, j] = re + im

    def fwdh(hf):
        lo, hi = hf * NCH // 2, (hf + 1) * NCH // 2
        hcat = jnp.concatenate([ht_l[:, j * C:(j + 1) * C] for j in range(lo, hi)], axis=0)
        Hf = jax.lax.dot_general(f_ref[half], hcat, NT, preferred_element_type=f32)
        for j in range(lo, hi):
            re, im = split(Hf, j - lo)
            if j == 0:
                re = re + cv["par"][4:5]
            H_s[0, NCH - 1 - j] = im - re
            H_s[1, NCH - 1 - j] = re + im
            H_s[2, NCH - 1 - j] = re

    def mac_piece(i, r, a):
        rs = slice(r, r + 8)
        s = jnp.sum(H_s[a, NCH - 1 - i:NCH, rs, :] * V_s[a, 0:i + 1, rs, :], axis=0)
        cv[a] = s
        if a == 2:
            yr, yi = s - cv[1], s + cv[0]
            wr, wi = yr, yi
            if i > 0:
                pr, pi = cv[("y", r)]
                wr, wi = (yr - pi, yi + pr) if r < 32 else (yr + pi, yi - pr)
            cv[("y", r)] = (yr, yi)
            W_s[2 * r:2 * r + 16, i * 128:(i + 1) * 128] = jnp.concatenate([wr, wi], axis=0).astype(bf16)
        return s

    def inv(hf):
        lo, hi = hf * NCH // 2, (hf + 1) * NCH // 2
        Y = jnp.dot(g_ref[half], W_s[:, lo * 128:hi * 128], preferred_element_type=f32)
        for j in range(lo, hi):
            a, b = j * C, (j + 1) * C
            y = Y[:, (j - lo) * 128:(j - lo + 1) * 128]
            acc[a:b, ccol] += xg_s[a:b, pl.ds(pl.multiple_of(ct * 128 + XO, 128), 128)] * y

    def stage_piece(t0):
        w = w_l[t0:t0 + 4].astype(f32).reshape(32, D)
        w_st[t0 * 8:t0 * 8 + 32, :] = w
        return functools.reduce(jnp.maximum, [w[k * 8:(k + 1) * 8] for k in range(4)])

    def extract_piece(wb, off, m0):
        ws = [w_st[pl.ds(2 * (off + m0) + hh, 8, stride=2), :] for hh in range(HP)]
        wb[m0:m0 + 8, :] = jnp.concatenate(ws, axis=1).astype(bf16)
        return ws[0]

    units = [(u // 2, u % 2) for u in range(NU)]

    cv["par"] = par_s[:, ccol]
    for r in range(0, S, 16):
        side.append((40, P(u_piece, r)))
    pq(0, 0); pk(0, 0); pq(0, 1); pk(0, 1)
    qk(0, 0)
    pvv(0, 0); pvv(0, 1)
    fwdh(0); fwdh(1)
    odone = 0
    for s in range(NU):
        i, hh = units[s]
        if s == FW:
            flush()
            fwdu(0); fwdu(1)
            for cp in early_copies(step + 1):
                cp.start()

            @pl.when(step == 0)
            def _():
                gate_blocks(NP0, NB)
                c_copy(1).wait()
            late_wait()
            qk(i, hh, "tail")
            for i2 in range(NCH):
                for r in range(0, 64, 8):
                    for a in range(3):
                        side.append((MACW * (2 * (i2 + 1) + 3), P(mac_piece, i2, r, a)))
            for t0 in range(0, WR // 4, 4):
                side.append((12, P(stage_piece, t0)))
        if s == NU - 2:
            flush()
            for (wh, wb, rows, off) in wsets:
                for m0 in range(0, rows, 8):
                    side.append((8, P(extract_piece, wb, off, m0)))
        do_o = s >= FW and odone < i and s < NU - 2
        if i + 1 < NB:
            pk(i + 1, hh); pq(i + 1, hh)
            if not do_o:
                lim[0] = LL
            pvv(i + 1, hh)
            lim[0] = 32
            if s >= 1 and "left" in st[units[s - 1]]:
                assert len(side) <= st[units[s - 1]]["left"]
        if do_o:
            oproj(odone, lastlim=LL)
            odone += 1
        if s == NU - 2:
            oproj(NB - 2, (0, 1))
        if s == NU - 1:
            oproj(NB - 2, (2, 3))
        pv(i, hh, s + 1 < NU - 2 and s + 1 != FW)
        if s + 1 < NU:
            qk(*units[s + 1], "head" if s + 1 == FW else None)
    inv(0); inv(1)
    assert odone == NB - 2
    oproj(NB - 1)
    flush()

    @pl.when(step < NSTEP - 1)
    def _():
        for cp in late_copies(step + 1):
            cp.start()

    @pl.when(step == NSTEP - 1)
    def _():
        r7 = (NB - 1) * BQ
        out_copy(r7, S, 768, M).start()
        for a, b in ((0, 512), (512, 1024), (1024, r7)):
            out_v[a:b, M - 128:M] = acc[a:b, M - 128:M].astype(bf16)
            out_copy(a, b, M - 128, M).start()
        early_wait()
        pltpu.make_async_copy(out_v, o_h, sems.at[SEM_OUT]).wait()


@jax.jit
def pallas_gated_mix__compressed_kv_cla__ssm_conv_h3__prompt_kernel(
    A_x: jax.Array,
    A_c_kv: jax.Array,
    A_w_q: jax.Array,
    A_w_uk: jax.Array,
    A_w_uv: jax.Array,
    A_w_o: jax.Array,
    B_q: jax.Array,
    B_k: jax.Array,
    B_v: jax.Array,
    B_shift_k: jax.Array,
    B_ssm_k: jax.Array,
    B_ssm_D: jax.Array,
    gate_w: jax.Array,
):
    del B_q
    Fc, Gc = _dft_consts()
    hbm = pl.BlockSpec(memory_space=pl.ANY)
    scratch = [
        pltpu.VMEM((4, M), bf16),
        pltpu.VMEM((M,), bf16),
        pltpu.VMEM((M,), bf16),
        pltpu.VMEM((2, 128, C), bf16),
        pltpu.VMEM((2, C, 128), bf16),
        pltpu.VMEM((S, M), bf16),
        pltpu.VMEM((S, DC), bf16),
        pltpu.VMEM((WR // 4, 8, D), bf16),
        pltpu.VMEM((WR // 4, 8, D), bf16),
        pltpu.VMEM((2 * WR + 8, D), f32),
        pltpu.VMEM((M, HP * D), bf16),
        pltpu.VMEM((DC, HP * D), bf16),
        pltpu.VMEM((DC, HP * D), bf16),
        pltpu.VMEM((HP * D, M), bf16),
        pltpu.VMEM((2, S, 128), bf16),
        pltpu.VMEM((128, S), bf16),
        pltpu.VMEM((S, M), f32),
        pltpu.VMEM((S, M + 512), f32),
        pltpu.VMEM((S, M), bf16),
        pltpu.VMEM((S, HP * D), bf16),
        pltpu.VMEM((S, HP * D), bf16),
        pltpu.VMEM((S, HP * D), bf16),
        pltpu.VMEM((NB, BQ, HP * D), bf16),
        pltpu.VMEM((S, 128), f32),
        pltpu.VMEM((8, M), f32),
        pltpu.VMEM((C, NCH * 128), bf16),
        pltpu.VMEM((3, NCH, 64, 128), f32),
        pltpu.VMEM((3, NCH, 64, 128), f32),
        pltpu.VMEM((128, NCH * 128), bf16),
        pltpu.VMEM((BQ + 8, S + 128), f32),
        pltpu.VMEM((BQ + 8, S + 128), f32),
        pltpu.SemaphoreType.DMA((NSEM,)),
    ]
    out = pl.pallas_call(
        _kernel,
        out_shape=jax.ShapeDtypeStruct((S, M), bf16),
        grid=(NSTEP,),
        in_specs=[hbm] * 14,
        out_specs=hbm,
        scratch_shapes=scratch,
        compiler_params=pltpu.CompilerParams(
            vmem_limit_bytes=100 * 1024 * 1024,
            dimension_semantics=("arbitrary",),
            disable_bounds_checks=True),
    )(A_x.reshape(S, M), A_c_kv.reshape(S, DC),
      A_w_q.reshape(M // 4, 4, H, D), A_w_uk.reshape(DC // 4, 4, H, D), A_w_uv.reshape(DC // 4, 4, H, D),
      A_w_o.reshape(H * D, M), B_k.reshape(S, M), B_v.reshape(S, M), B_ssm_k,
      B_shift_k.T, B_ssm_D, gate_w, jnp.asarray(Fc), jnp.asarray(Gc))
    return out.reshape(1, S, M)
```
